```python
import jax
import jax.numpy as jnp

def _softmax(x, axis=-1):
    return jax.nn.softmax(x, axis=axis)

def _gelu(x):
    return jax.nn.gelu(x, approximate=True)

def _silu(x):
    return jax.nn.silu(x)

def _sigmoid(x):
    return jax.nn.sigmoid(x)

def _layernorm(x, axis=-1, eps=1e-05):
    m = jnp.mean(x, axis=axis, keepdims=True)
    v = jnp.var(x, axis=axis, keepdims=True)
    return (x - m) / jnp.sqrt(v + eps)

def _scatter_add(tgt, idx, src, axis=0):
    return tgt.at[idx].add(src)

def _segment_sum(src, seg, n):
    return jax.ops.segment_sum(src, seg, n)

class _Rng:

    def __init__(self, key):
        self._k = key

    def _next(self):
        self._k, sub = jax.random.split(self._k)
        return sub

    def normal(self, shape):
        return jax.random.normal(self._next(), shape, dtype=jnp.bfloat16)

    def randint(self, lo, hi, shape):
        return jax.random.randint(self._next(), shape, lo, hi, dtype=jnp.int32)

    def uniform(self, shape, lo=0.0, hi=1.0):
        return jax.random.uniform(self._next(), shape, jnp.bfloat16, lo, hi)

    def permutation(self, n):
        return jax.random.permutation(self._next(), n)
kernel_name = 'adaLN_cond__ssm_conv_h3__mixer_gmlp__prompt'

def setup_inputs():
    _rng = _Rng(jax.random.key(int.from_bytes(__import__("os").urandom(4), "little")))
    _w = lambda a: (lambda t: t.astype(jnp.bfloat16) if jnp.issubdtype(t.dtype, jnp.floating) else t)(jnp.asarray(a))

    def _A_setup():
        B, S, D = (1, 2048, 640)
        ks = 4
        return {'q': _w((lambda *s: _rng.normal(s) * 0.05)(B, S, D)), 'k': _w((lambda *s: _rng.normal(s) * 0.05)(B, S, D)), 'v': _w((lambda *s: _rng.normal(s) * 0.05)(B, S, D)), 'shift_k': _w((lambda *s: _rng.normal(s) * 0.05)(D, ks) * 0.5), 'ssm_k': _w((lambda *s: _rng.normal(s) * 0.05)(D, S) * (1.0 / S ** 0.5)), 'ssm_D': _w((lambda *s: _rng.normal(s) * 0.05)(D))}
    _A_in = _A_setup()

    def _B_setup():
        B, S, D, F = (1, 2048, 640, 1728)
        Fh = F // 2
        return {'x': _w((lambda *s: _rng.normal(s) * 0.05)(B, S, D)), 'w_in': _w((lambda *s: _rng.normal(s) * 0.05)(D, 2 * Fh)), 'w_sp': _w(0.01 * (lambda *s: _rng.normal(s) * 0.05)(S, S)), 'b_sp': _w(1.0 + 0.01 * (lambda *s: _rng.normal(s) * 0.05)(S)), 'w_out': _w((lambda *s: _rng.normal(s) * 0.05)(Fh, D))}
    _B_in = _B_setup()
    return {'A_q': _A_in['q'], 'A_k': _A_in['k'], 'A_v': _A_in['v'], 'A_shift_k': _A_in['shift_k'], 'A_ssm_k': _A_in['ssm_k'], 'A_ssm_D': _A_in['ssm_D'], 'B_x': _B_in['x'], 'B_w_in': _B_in['w_in'], 'B_w_sp': _B_in['w_sp'], 'B_b_sp': _B_in['b_sp'], 'B_w_out': _B_in['w_out'], 'c': _w((lambda *s: _rng.normal(s) * 0.05)(1, 640)), 'w_mod': _w((lambda *s: _rng.normal(s) * 0.05)(640, 6 * 640) * 640 ** (-0.5))}

def reference(A_q, A_k, A_v, A_shift_k, A_ssm_k, A_ssm_D, B_x, B_w_in, B_w_sp, B_b_sp, B_w_out, c, w_mod):

    def _A_ref(q, k, v, shift_k, ssm_k, ssm_D):
        B, S, D = q.shape
        ks = shift_k.shape[-1]
        k_pad = jnp.pad(k, ((0, 0), (ks - 1, 0), (0, 0)))
        k_shift = jnp.zeros_like(k)
        for t in range(ks):
            k_shift = k_shift + k_pad[:, t:t + S, :] * shift_k[:, ks - 1 - t][None, None, :]
        kv = k_shift * v
        L = 2 * S
        kv_pad = jnp.pad(kv, ((0, 0), (0, S), (0, 0)))
        kf_pad = jnp.pad(ssm_k, ((0, 0), (0, S)))
        kv_f = (lambda x, axes=(-2, -1): jnp.fft.rfft2(x.astype(jnp.float32), axes=axes))(kv_pad[:, None, :, :], axes=(1, 2))
        kf_f = (lambda x, axes=(-2, -1): jnp.fft.rfft2(x.astype(jnp.float32), axes=axes))(kf_pad[:, None, :], axes=(1, 2))
        kf_f = (lambda x, *d: x.transpose(*d))(kf_f, 1, 2, 0)
        y_f = kv_f * kf_f[None, :, :, :]
        y = (lambda x, s, axes=(-2, -1): jnp.fft.irfft2(x, s=s, axes=axes).astype(jnp.bfloat16))(y_f, (1, L), axes=(1, 2))[:, 0, :S, :]
        y = y + kv * ssm_D[None, None, :]
        return q * y

    def _B_ref(x, w_in, w_sp, b_sp, w_out):
        B, S, D = x.shape
        F = w_in.shape[-1]
        Fh = F // 2
        z = _gelu(jnp.einsum('bsd,df->bsf', x, w_in))
        z1 = z[..., :Fh].copy()
        z2 = _layernorm(z[..., Fh:], axis=-1)
        g = jnp.einsum('ts,bsf->btf', w_sp, z2) + b_sp[None, :, None]
        return jnp.einsum('bsf,fd->bsd', z1 * g, w_out)
    x = A_q
    mod = (_silu(c) @ w_mod).reshape(c.shape[0], 6, 1, -1)
    sa, ca, ga, sb, cb, gb = (mod[:, 0].copy(), mod[:, 1].copy(), mod[:, 2].copy(), mod[:, 3].copy(), mod[:, 4].copy(), mod[:, 5].copy())
    h = _layernorm(x, axis=-1) * (1 + ca) + sa
    x = x + ga * _A_ref(h, A_k, A_v, A_shift_k, A_ssm_k, A_ssm_D)
    h = _layernorm(x, axis=-1) * (1 + cb) + sb
    x = x + gb * _B_ref(h, B_w_in, B_w_sp, B_b_sp, B_w_out)
    return x
```

```python
import numpy as np

import jax
import jax.numpy as jnp
from jax import lax
import jax.experimental.pallas as pl
import jax.experimental.pallas.tpu as pltpu

LANES = 128
R = 4
M = 128
C = R * M
HIST = 16
EPS = 1e-5
GELU_C1 = float(np.sqrt(2.0 / np.pi))
GELU_C3 = float(np.sqrt(2.0 / np.pi) * 0.044715)
TB = 256
TC = 256

F32 = jnp.float32
BF16 = jnp.bfloat16
NT = (((1,), (1,)), ((), ()))


def _dft_matrices():
    f0 = np.arange(M)[:, None]
    m = np.arange(M)[None, :]
    fwd = np.zeros((R, 2 * M, M), np.float64)
    for r in range(R):
        n = R * m + r
        ph = -np.pi * ((n * (1 + 4 * f0)) % (4 * C)) / (2 * C)
        re = np.cos(ph).reshape(M // 8, 8, M)
        im = np.sin(ph).reshape(M // 8, 8, M)
        fwd[r] = np.stack([re, im], 1).reshape(2 * M, M)
    inv = np.transpose(fwd, (0, 2, 1)) / C
    return fwd.astype(np.float32), np.ascontiguousarray(inv).astype(np.float32)


def _dot(a, b):
    return jnp.dot(a, b, preferred_element_type=F32)


def _dot_nt(a, b):
    return lax.dot_general(a, b, NT, preferred_element_type=F32)


def _gelu2(x):
    t = jnp.tanh(x * (x * x * GELU_C3 + GELU_C1))
    return x * t + x


def _ln_rows(x):
    n = x.shape[-1]
    d = x - jnp.sum(x, axis=-1, keepdims=True) * (1.0 / n)
    var = jnp.sum(d * d, axis=-1, keepdims=True) * (1.0 / n)
    return d * lax.rsqrt(var + EPS)


def _butterfly(x, inverse):
    (r0, i0), (r1, i1), (r2, i2), (r3, i3) = x
    ar, ai, br, bi = r0 + r2, i0 + i2, r0 - r2, i0 - i2
    cr, ci, dr, di = r1 + r3, i1 + i3, r1 - r3, i1 - i3
    lo, hi = (br + di, bi - dr), (br - di, bi + dr)
    if inverse:
        lo, hi = hi, lo
    return [(ar + cr, ai + ci), lo, (ar - cr, ai - ci), hi]


def _forward(f_v, phases):
    es = []
    for r in range(R):
        e = _dot(f_v[r], phases[r].astype(BF16)).reshape(M // 8, 2, 8, LANES)
        es.append((e[:, 0], e[:, 1]))
    return _butterfly(es, inverse=False)


def _kernel(q_h, k_h, v_h, sk_h, g_h, sd_h, win_h, wsp_h, bsp_h, wout_h, c_h, wmod_h, f_h, fi_h,
            out_h,
            q_v, k_v, v_v, sk_v, g_v, sd_v, win_v, wsp_v, bsp_v, wout_v, c_v, wmod_v, f_v, fi_v,
            gs_v, us_v, gt_v, kf_v, vf_v, y_v, row_v, h_v, z1_v, z2_v, woutt_v, out_v, sems):
    S, D = q_v.shape
    FH = wout_v.shape[0]
    NA, NJ = S // C, D // LANES
    KS = sk_v.shape[0]

    n_sem = [0]

    def fetch(src, dst):
        cp = pltpu.make_async_copy(src, dst, sems.at[n_sem[0]])
        n_sem[0] += 1
        cp.start()
        return cp

    def rows(ref, i, n):
        return ref.at[pl.ds(i * n, n)]

    cp_f = fetch(f_h, f_v)
    cp_g = [fetch(rows(g_h, j, LANES), rows(g_v, j, LANES)) for j in range(NJ)]
    cp_small = [fetch(sd_h, sd_v), fetch(sk_h, sk_v), fetch(fi_h, fi_v)]
    cp_kv = [(fetch(rows(k_h, a, C), rows(k_v, a, C)), fetch(rows(v_h, a, C), rows(v_v, a, C)))
             for a in range(NA)]
    cp_c = fetch(c_h, c_v)
    cp_win = fetch(win_h, win_v)
    cp_q0 = fetch(rows(q_h, 0, C), rows(q_v, 0, C))
    cp_wmod = fetch(wmod_h, wmod_v)
    cp_q1 = fetch(q_h.at[pl.ds(C, S - C)], q_v.at[pl.ds(C, S - C)])
    cp_rest = [fetch(bsp_h, bsp_v), fetch(wout_h, wout_v), fetch(wsp_h, wsp_v)]

    cp_f.wait()
    for cp in cp_small:
        cp.wait()
    sd_row = sd_v[...].astype(F32).reshape(1, D)
    sk = sk_v[...].astype(F32)
    row_v[0:1, :] = sd_row
    row_v[8:8 + KS, :] = sk

    for j in range(NJ):
        cp_g[j].wait()
        prev = None
        for a in range(NA):
            gt_v[a] = g_v[j * LANES:(j + 1) * LANES, a * C:(a + 1) * C].T.astype(F32)
            spec = _forward(f_v, [gt_v[a, pl.ds(r, M, stride=R), :] for r in range(R)])
            for qq in range(R):
                re, im = spec[qq]
                if a == 0:
                    re = re + row_v[0:1, j * LANES:(j + 1) * LANES]
                else:
                    re, im = re - prev[qq][1], im + prev[qq][0]
                gs_v[j, a, 2 * qq] = re
                gs_v[j, a, 2 * qq + 1] = im
            prev = spec

    for a in range(NA):
        cp_kv[a][0].wait()
        cp_kv[a][1].wait()

        def conv_tile(j, carry, a=a):
            lanes = pl.ds(pl.multiple_of(j * LANES, LANES), LANES)
            if a == 0:
                kf_v[0:HIST, :] = jnp.zeros((HIST, LANES), F32)
                kf_v[HIST:, :] = k_v[0:C, lanes].astype(F32)
            else:
                kf_v[...] = k_v[a * C - HIST:(a + 1) * C, lanes].astype(F32)
            vf_v[...] = v_v[a * C:(a + 1) * C, lanes].astype(F32)
            kp = {s: kf_v[pl.ds(HIST + s, M, stride=R), :] for s in range(1 - KS, R)}
            taps = [row_v[8 + t:9 + t, lanes] for t in range(KS)]
            phases = []
            for r in range(R):
                acc = kp[r] * taps[0]
                for t in range(1, KS):
                    acc = acc + kp[r - t] * taps[t]
                phases.append(acc * vf_v[pl.ds(r, M, stride=R), :])
            spec = _forward(f_v, phases)
            ys = []
            for qq in range(R):
                ur, ui = spec[qq]
                if a + 1 < NA:
                    us_v[j, a, 2 * qq] = ur
                    us_v[j, a, 2 * qq + 1] = ui
                yr = yi = None
                for b in range(a + 1):
                    if b > 0:
                        ur, ui = us_v[j, a - b, 2 * qq], us_v[j, a - b, 2 * qq + 1]
                    gr, gi = gs_v[j, b, 2 * qq], gs_v[j, b, 2 * qq + 1]
                    tr, ti = gr * ur - gi * ui, gr * ui + gi * ur
                    yr, yi = (tr, ti) if b == 0 else (yr + tr, yi + ti)
                ys.append((yr, yi))
            bs = _butterfly(ys, inverse=True)
            for r in range(R):
                bm = jnp.stack(bs[r], axis=1).reshape(2 * M, LANES).astype(BF16)
                y_v[j, pl.ds(a * C + r, M, stride=R), :] = _dot(fi_v[r], bm)
            return carry

        lax.fori_loop(0, NJ, conv_tile, None)

    cp_c.wait()
    cp_wmod.wait()
    cc = c_v[...].astype(F32)
    sc = jnp.broadcast_to(cc * jax.nn.sigmoid(cc), (16, D)).astype(BF16)
    mod = _dot(sc, wmod_v[...])[0:1]
    sa, ca, ga, sb, cb, gb = (mod[:, i * D:(i + 1) * D] for i in range(6))
    row_v[1:2, :] = ga * (1.0 + ca)
    row_v[2:3, :] = ga * sa
    row_v[3:4, :] = 1.0 + cb
    row_v[4:5, :] = sb
    row_v[5:6, :] = 0.5 * gb

    def prepare(i, slot):
        rs = pl.ds(pl.multiple_of(i * TB, TB), TB)
        x = q_v[rs, :].astype(F32)
        y = jnp.concatenate([y_v[j, rs, :] for j in range(NJ)], axis=1)
        x1 = x + (_ln_rows(x) * row_v[1:2, :] + row_v[2:3, :]) * y
        for j in range(NJ):
            y_v[j, rs, :] = x1[:, j * LANES:(j + 1) * LANES]
        h_v[slot] = (_ln_rows(x1) * row_v[3:4, :] + row_v[4:5, :]).astype(BF16)

    def project(i, slot):
        cs = pl.ds(pl.multiple_of(i * TB, TB), TB)
        h = h_v[slot]
        a2 = _gelu2(_dot_nt(win_v[FH:, :], h))
        d = a2 - jnp.sum(a2, axis=0, keepdims=True) * (1.0 / FH)
        var = jnp.sum(d * d, axis=0, keepdims=True) * (1.0 / FH)
        z2_v[:, cs] = (d * lax.rsqrt(var + 4.0 * EPS)).astype(BF16)
        z1_v[:, cs] = _dot_nt(win_v[:FH, :], h)

    cp_win.wait()
    cp_q0.wait()
    prepare(0, 0)
    cp_q1.wait()

    def phase_b(i, carry):
        project(i, i % 2)
        prepare(i + 1, (i + 1) % 2)
        return carry

    nb = S // TB
    lax.fori_loop(0, nb - 1, phase_b, None)
    project(nb - 1, (nb - 1) % 2)

    for cp in cp_rest:
        cp.wait()
    woutt_v[...] = wout_v[...].T
    brow = bsp_v[...].astype(F32).reshape(1, S)
    nc = S // TC
    out_sem0 = n_sem[0]

    def out_copy(i):
        rs = pl.ds(pl.multiple_of(i * TC, TC), TC)
        return pltpu.make_async_copy(out_v.at[rs], out_h.at[rs], sems.at[out_sem0 + i])

    def scoped(brow_v):
        brow_v[...] = brow

        def phase_c(i, carry):
            rs = pl.ds(pl.multiple_of(i * TC, TC), TC)
            gate = _dot_nt(z2_v[...], wsp_v[rs, :]) + brow_v[:, rs]
            p = (_gelu2(z1_v[:, rs]) * gate).astype(BF16)
            o = _dot(woutt_v[...], p).T
            x1 = jnp.concatenate([y_v[j, rs, :] for j in range(NJ)], axis=1)
            out_v[rs, :] = (x1 + row_v[5:6, :] * o).astype(out_v.dtype)
            out_copy(i).start()
            return carry

        lax.fori_loop(0, nc, phase_c, None)

    pl.run_scoped(scoped, pltpu.VMEM((1, S), F32))
    for i in range(nc):
        out_copy(i).wait()


@jax.jit
def pallas_adaLN_cond__ssm_conv_h3__mixer_gmlp__prompt_kernel(
    A_q: jax.Array,
    A_k: jax.Array,
    A_v: jax.Array,
    A_shift_k: jax.Array,
    A_ssm_k: jax.Array,
    A_ssm_D: jax.Array,
    B_x: jax.Array,
    B_w_in: jax.Array,
    B_w_sp: jax.Array,
    B_b_sp: jax.Array,
    B_w_out: jax.Array,
    c: jax.Array,
    w_mod: jax.Array,
):
    del B_x
    B, S, D = A_q.shape
    FH = B_w_out.shape[0]
    assert B == 1 and S % C == 0 and D % LANES == 0 and B_w_in.shape[1] == 2 * FH
    NA, NJ = S // C, D // LANES
    fwd, inv = _dft_matrices()
    operands = (
        A_q.reshape(S, D), A_k.reshape(S, D), A_v.reshape(S, D), A_shift_k.T, A_ssm_k, A_ssm_D,
        B_w_in.T, B_w_sp, B_b_sp, B_w_out, c, w_mod,
        fwd.astype(BF16), inv.astype(BF16),
    )
    spectrum = (2 * R, M // 8, 8, LANES)
    scratch = [pltpu.VMEM(o.shape, o.dtype) for o in operands] + [
        pltpu.VMEM((NJ, NA) + spectrum, F32),
        pltpu.VMEM((NJ, NA - 1) + spectrum, F32),
        pltpu.VMEM((NA, C, LANES), F32),
        pltpu.VMEM((HIST + C, LANES), F32),
        pltpu.VMEM((C, LANES), F32),
        pltpu.VMEM((NJ, S, LANES), F32),
        pltpu.VMEM((16, D), F32),
        pltpu.VMEM((2, TB, D), BF16),
        pltpu.VMEM((FH, S), F32),
        pltpu.VMEM((FH, S), BF16),
        pltpu.VMEM((D, FH), BF16),
        pltpu.VMEM((S, D), A_q.dtype),
        pltpu.SemaphoreType.DMA((48,)),
    ]
    out = pl.pallas_call(
        _kernel,
        out_shape=jax.ShapeDtypeStruct((S, D), A_q.dtype),
        in_specs=[pl.BlockSpec(memory_space=pl.ANY)] * len(operands),
        out_specs=pl.BlockSpec(memory_space=pl.ANY),
        scratch_shapes=scratch,
        compiler_params=pltpu.CompilerParams(vmem_limit_bytes=110 * 2**20),
    )(*operands)
    return out.reshape(B, S, D)
```

```python
import functools

import numpy as np

import jax
import jax.numpy as jnp
from jax import lax
import jax.experimental.pallas as pl
import jax.experimental.pallas.tpu as pltpu

LANES = 128
R = 4
M = 128
C = R * M
HIST = 16
EPS = 1e-5
GELU_C1 = float(np.sqrt(2.0 / np.pi))
GELU_C3 = float(np.sqrt(2.0 / np.pi) * 0.044715)
T = 128
PR = 16
MB = 288
NR = 96
NO = 16
FLAGS = None
PH = 'ABC'
S1 = 1
S2 = 1

F32 = jnp.float32
BF16 = jnp.bfloat16
NT = (((1,), (1,)), ((), ()))
QUADS = ((0, 0), (0, 1), (1, 0), (1, 1))


def _dft_matrices():
    f0 = np.arange(M)[:, None]
    m = np.arange(M)[None, :]
    fwd = np.zeros((R, 2 * M, M), np.float64)
    for r in range(R):
        n = R * m + r
        ph = -np.pi * ((n * (1 + 4 * f0)) % (4 * C)) / (2 * C)
        re = np.cos(ph).reshape(M // 8, 8, M)
        im = np.sin(ph).reshape(M // 8, 8, M)
        fwd[r] = np.stack([re, im], 1).reshape(2 * M, M)
    inv = np.transpose(fwd, (0, 2, 1)) / C
    return fwd.astype(np.float32), np.ascontiguousarray(inv).astype(np.float32)


def _dot(a, b):
    return jnp.dot(a, b, preferred_element_type=F32)


def _dot_nt(a, b):
    return lax.dot_general(a, b, NT, preferred_element_type=F32)


def _gelu2(x):
    t = jnp.tanh(x * (x * x * GELU_C3 + GELU_C1))
    return x * t + x


def _ln_rows(x):
    n = x.shape[-1]
    d = x - jnp.sum(x, axis=-1, keepdims=True) * (1.0 / n)
    var = jnp.sum(d * d, axis=-1, keepdims=True) * (1.0 / n)
    return d * lax.rsqrt(var + EPS)


def _interleave(*streams):
    order = sorted(((n + (0.5 if k else 0.0)) / len(st), k, n)
                   for k, st in enumerate(streams) for n in range(len(st)))
    for _, k, n in order:
        streams[k][n]()


def _strassen_left(a11, a12, a21, a22):
    return (a11 + a22, a21 + a22, a11, a22, a11 + a12, a21 - a11, a12 - a22)


def _strassen(dot, left, b11, b12, b21, b22):
    f11, f12, f21, f22 = (b.astype(F32) for b in (b11, b12, b21, b22))
    m2 = dot(left[1], b11.astype(BF16))
    m5 = dot(left[4], b22.astype(BF16))
    m3 = dot(left[2], (f12 - f22).astype(BF16))
    m4 = dot(left[3], (f21 - f11).astype(BF16))
    m1 = dot(left[0], (f11 + f22).astype(BF16))
    m7 = dot(left[6], (f21 + f22).astype(BF16))
    m6 = dot(left[5], (f11 + f12).astype(BF16))
    return (m4 - m5) + m1 + m7, m3 + m5, m2 + m4, (m3 - m2) + m1 + m6


def _butterfly(x, inverse):
    (r0, i0), (r1, i1), (r2, i2), (r3, i3) = x
    ar, ai, br, bi = r0 + r2, i0 + i2, r0 - r2, i0 - i2
    cr, ci, dr, di = r1 + r3, i1 + i3, r1 - r3, i1 - i3
    lo, hi = (br + di, bi - dr), (br - di, bi + dr)
    if inverse:
        lo, hi = hi, lo
    return [(ar + cr, ai + ci), lo, (ar - cr, ai - ci), hi]


def _forward(f_v, phases):
    es = []
    for r in range(R):
        e = _dot(f_v[r], phases[r].astype(BF16)).reshape(M // 8, 2, 8, LANES)
        es.append((e[:, 0], e[:, 1]))
    return _butterfly(es, inverse=False)


def _kernel(q_h, k_h, v_h, sk_h, g_h, sd_h, win_h, wsp_h, bsp_h, wout_h, c_h, wmod_h, f_h, fi_h,
            out_h,
            q_v, k_v, v_v, sk_v, g_v, sd_v, win_v, wsp_v, bsp_v, wout_v, c_v, wmod_v, f_v, fi_v,
            gs_v, us_v, gt_v, kf_v, vf_v, y_v, x1_v, row_v, mod_v, h_v, hb_v, a2_v, mean_v, zs_v,
            wis_v, wos_v, p_v, o_v, woutt_v, brow_v, out_v, sems):
    S, D = q_v.shape
    FH = wout_v.shape[0]
    NA, NJ = S // C, D // LANES
    KS = sk_v.shape[0]

    n_sem = [0]

    def fetch(src, dst):
        cp = pltpu.make_async_copy(src, dst, sems.at[n_sem[0]])
        n_sem[0] += 1
        cp.start()
        return cp

    def rows(ref, i, n):
        return ref.at[pl.ds(i * n, n)]

    cp_g = [fetch(rows(g_h, 0, LANES), rows(g_v, 0, LANES))]
    cp_small = [fetch(f_h, f_v), fetch(sd_h, sd_v), fetch(sk_h, sk_v), fetch(c_h, c_v)]
    cp_g += [fetch(rows(g_h, j, LANES), rows(g_v, j, LANES)) for j in range(1, NJ)]
    cp_fi = fetch(fi_h, fi_v)
    cp_kv = [(fetch(rows(k_h, a, C), rows(k_v, a, C)), fetch(rows(v_h, a, C), rows(v_v, a, C)))
             for a in range(NA)]
    def mod_cols(n):
        return fetch(wmod_h.at[:, pl.ds(n * D, D)], wmod_v.at[:, pl.ds(n * D, D)])

    cp_q0 = [fetch(q_h.at[pl.ds(s, T)], q_v.at[pl.ds(s, T)]) for s in (0, S // 2)]
    cp_wmod = [mod_cols(n) for n in range(5)]
    cp_win2 = fetch(rows(win_h, 1, FH), rows(win_v, 1, FH))
    cp_q1 = [fetch(q_h.at[pl.ds(s + T, S // 2 - T)], q_v.at[pl.ds(s + T, S // 2 - T)])
             for s in (0, S // 2)]
    cp_wmod += [mod_cols(5)]
    cp_rest = [fetch(rows(win_h, 0, FH), rows(win_v, 0, FH)), fetch(bsp_h, bsp_v),
               fetch(wout_h, wout_v), fetch(wsp_h, wsp_v)]

    for cp in cp_small:
        cp.wait()
    sd_row = sd_v[...].astype(F32).reshape(1, D)
    sk = sk_v[...].astype(F32)
    row_v[0:1, :] = sd_row
    row_v[8:8 + KS, :] = sk

    for j in range(NJ):
        cp_g[j].wait()
        prev = None
        for a in range(NA if 'A' in PH else 0):
            gt_v[a] = g_v[j * LANES:(j + 1) * LANES, a * C:(a + 1) * C].T.astype(F32)
            spec = _forward(f_v, [gt_v[a, pl.ds(r, M, stride=R), :] for r in range(R)])
            for qq in range(R):
                re, im = spec[qq]
                if a == 0:
                    re = re + row_v[0:1, j * LANES:(j + 1) * LANES]
                else:
                    re, im = re - prev[qq][1], im + prev[qq][0]
                gs_v[j, a, 2 * qq] = re
                gs_v[j, a, 2 * qq + 1] = im
            prev = spec

    cp_fi.wait()
    for a in range(NA):
        cp_kv[a][0].wait()
        cp_kv[a][1].wait()

        def conv_tile(j, carry, a=a):
            lanes = pl.ds(pl.multiple_of(j * LANES, LANES), LANES)
            if a == 0:
                kf_v[0:HIST, :] = jnp.zeros((HIST, LANES), F32)
                kf_v[HIST:, :] = k_v[0:C, lanes].astype(F32)
            else:
                kf_v[...] = k_v[a * C - HIST:(a + 1) * C, lanes].astype(F32)
            vf_v[...] = v_v[a * C:(a + 1) * C, lanes].astype(F32)
            kp = {s: kf_v[pl.ds(HIST + s, M, stride=R), :] for s in range(1 - KS, R)}
            taps = [row_v[8 + t:9 + t, lanes] for t in range(KS)]
            phases = []
            for r in range(R):
                acc = kp[r] * taps[0]
                for t in range(1, KS):
                    acc = acc + kp[r - t] * taps[t]
                phases.append(acc * vf_v[pl.ds(r, M, stride=R), :])
            spec = _forward(f_v, phases)
            ys = []
            for qq in range(R):
                ur, ui = spec[qq]
                if a + 1 < NA:
                    us_v[j, a, 2 * qq] = ur
                    us_v[j, a, 2 * qq + 1] = ui
                yr = yi = None
                for b in range(a + 1):
                    if b > 0:
                        ur, ui = us_v[j, a - b, 2 * qq], us_v[j, a - b, 2 * qq + 1]
                    gr, gi = gs_v[j, b, 2 * qq], gs_v[j, b, 2 * qq + 1]
                    tr, ti = gr * ur - gi * ui, gr * ui + gi * ur
                    yr, yi = (tr, ti) if b == 0 else (yr + tr, yi + ti)
                ys.append((yr, yi))
            bs = _butterfly(ys, inverse=True)
            for r in range(R):
                bm = jnp.stack(bs[r], axis=1).reshape(2 * M, LANES).astype(BF16)
                y_v[j, pl.ds(a * C + r, M, stride=R), :] = _dot(fi_v[r], bm)
            return carry

        if 'A' in PH:
            lax.fori_loop(0, NJ, conv_tile, None)

    def modulation(n):
        cp_wmod[n].wait()
        return _dot(sc, wmod_v[:, n * D:(n + 1) * D])[0:8]

    cc = c_v[...].astype(F32)
    sc = jnp.broadcast_to(cc * jax.nn.sigmoid(cc), (16, D)).astype(BF16)
    sa, ca, ga, sb, cb = (modulation(n) for n in range(5))
    mod_v[0] = ga * (1.0 + ca)
    mod_v[1] = ga * sa
    mod_v[2] = 1.0 + cb
    mod_v[3] = sb

    def scale(x, n):
        return (x.reshape(x.shape[0] // 8, 8, D) * mod_v[n]).reshape(x.shape)

    def shift(x, n):
        return (x.reshape(x.shape[0] // 8, 8, D) + mod_v[n]).reshape(x.shape)

    HS, HF, HD = S // 2, FH // 2, D // 2
    nb = HS // T

    def halves(i, off=0, n=T):
        return [pl.ds(pl.multiple_of(hh * HS + i * T + off, n), n) for hh in range(2)]

    def prepare(i):
        def piece(hh, off):
            rs = halves(i, off, PR)[hh]
            x = q_v[rs, :].astype(F32)
            y = jnp.concatenate([y_v[j, rs, :] for j in range(NJ)], axis=1)
            x1 = x + shift(scale(_ln_rows(x), 0), 1) * y
            x1_v[rs, :] = x1
            h_v[rs, :] = shift(scale(_ln_rows(x1), 2), 3).astype(BF16)

        return [functools.partial(piece, hh, off) for hh in range(2) for off in range(0, T, PR)]

    def project2(slot):
        tot = {}

        def piece(r0):
            a2 = _gelu2(_dot_nt(win_v[FH + r0:FH + r0 + MB, :], hb_v[slot]))
            a2_v[slot, r0:r0 + MB, :] = a2
            part = jnp.sum(a2.reshape(MB // 8, 8, 2 * T), axis=0)
            tot[0] = part if r0 == 0 else tot[0] + part
            if r0 + MB == FH:
                mean = jnp.sum(tot[0], axis=0, keepdims=True) * (1.0 / FH)
                mean_v[slot] = jnp.broadcast_to(mean, (8, 2 * T))

        return [functools.partial(piece, r0) for r0 in range(0, FH, MB)]

    def normalize(i, slot):
        state = {}

        def centred(r0, n):
            return a2_v[slot, r0:r0 + n, :].reshape(n // 8, 8, 2 * T) - mean_v[slot]

        def var_piece(r0):
            d = centred(r0, NR)
            part = jnp.sum(d * d, axis=0)
            state["ss"] = part if r0 == 0 else state["ss"] + part
            if r0 + NR == FH:
                var = jnp.sum(state["ss"], axis=0, keepdims=True) * (1.0 / FH)
                state["rstd"] = jnp.broadcast_to(lax.rsqrt(var + 4.0 * EPS), (8, 2 * T))

        def out_piece(r0):
            za = (centred(r0, NO) * state["rstd"]).reshape(NO, 2 * T)
            zb = (centred(HF + r0, NO) * state["rstd"]).reshape(NO, 2 * T)
            cs = pl.ds(pl.multiple_of(i * T, T), T)
            for n, val in enumerate(_strassen_left(za[:, :T], za[:, T:], zb[:, :T], zb[:, T:])):
                zs_v[n, r0:r0 + NO, cs] = val.astype(BF16)

        return ([functools.partial(var_piece, r0) for r0 in range(0, FH, NR)]
                + [functools.partial(out_piece, r0) for r0 in range(0, HF, NO)])

    def stage(i, slot):
        for hh, rs in enumerate(halves(i)):
            hb_v[slot, hh * T:(hh + 1) * T, :] = h_v[rs, :]

    def step_b(i, slot, first=False, last=False):
        side = [] if first else [normalize(i - 1, 1 - slot)]
        side += [] if last else [prepare(i + 1)]
        _interleave(project2(slot), *side)
        if not last:
            stage(i + 1, 1 - slot)

    def two_steps_b(n, carry):
        step_b(2 * n + 1, 1)
        step_b(2 * n + 2, 0)
        return carry

    for cp in cp_q0:
        cp.wait()
    if 'C' in PH:
        _interleave(prepare(0))
        stage(0, 0)
    cp_win2.wait()
    for cp in cp_q1:
        cp.wait()
    if 'C' in PH:
        step_b(0, 0, first=True)
    if 'B' in PH:
        lax.fori_loop(0, (nb - 2) // 2, two_steps_b, None)
    for cp in cp_rest:
        cp.wait()
    if 'C' not in PH:
        out_v[0:16, 0:128] = (x1_v[0:16, 0:128]).astype(BF16) + zs_v[1, 0:16, 0:128] + h_v[0:16, 0:128]
        pltpu.sync_copy(out_v, out_h)
        return
    step_b(nb - 1, 1, last=True)
    mod_v[4] = 0.5 * modulation(5)
    brow_v[...] = jnp.broadcast_to(bsp_v[...].astype(F32).reshape(1, S), (8, S))

    KI, KO = (NJ // 2) * LANES, (FH // (2 * LANES)) * LANES
    woutt_v[...] = wout_v[...].T
    for r0 in range(0, HF, NO):
        blk = [win_v[r:r + NO, k:k + KI].astype(F32) for r in (r0, HF + r0) for k in (0, KI)]
        for n, val in enumerate(_strassen_left(*blk)):
            wis_v[n, r0:r0 + NO, :] = val.astype(BF16)
    for r0 in range(0, HD, NO):
        blk = [woutt_v[r:r + NO, k:k + KO].astype(F32) for r in (r0, HD + r0) for k in (0, KO)]
        for n, val in enumerate(_strassen_left(*blk)):
            wos_v[n, r0:r0 + NO, :] = val.astype(BF16)
    _interleave(normalize(nb - 1, 1))

    out_sem0 = n_sem[0]

    def out_copies(i):
        return [pltpu.make_async_copy(out_v.at[rs], out_h.at[rs], sems.at[out_sem0 + 2 * i + hh])
                for hh, rs in enumerate(halves(i))]

    def project1(i):
        t1, t2 = halves(i)
        if not S1:
            h = jnp.concatenate([h_v[t1, :], h_v[t2, :]], axis=0)
            z = _dot_nt(win_v[:FH, :], h)
            return z[:HF, :T], z[:HF, T:], z[HF:, :T], z[HF:, T:]
        quads = _strassen(_dot_nt, wis_v, h_v[t1, :KI], h_v[t2, :KI], h_v[t1, KI:2 * KI], h_v[t2, KI:2 * KI])
        return [z + _dot_nt(win_v[fh * HF:(fh + 1) * HF, 2 * KI:], h_v[(t1, t2)[hh], 2 * KI:])
                for z, (fh, hh) in zip(quads, QUADS)]

    def mix(i):
        t1, t2 = halves(i)
        return _strassen(_dot_nt, zs_v, wsp_v[t1, :HS], wsp_v[t2, :HS], wsp_v[t1, HS:], wsp_v[t2, HS:])

    def gate(i, slot, acts, gates):
        for a, g, (fh, hh) in zip(acts, gates, QUADS):
            g = (g.reshape(HF // 8, 8, T) + brow_v[:, halves(i)[hh]]).reshape(HF, T)
            p_v[slot, fh * HF:(fh + 1) * HF, hh * T:(hh + 1) * T] = (a * g).astype(p_v.dtype)

    def project_out(slot):
        if not S2:
            o_v[slot] = _dot(woutt_v[...], p_v[slot].astype(BF16))
            return
        quads = _strassen(_dot, wos_v, p_v[slot, :KO, :T], p_v[slot, :KO, T:],
                          p_v[slot, KO:2 * KO, :T], p_v[slot, KO:2 * KO, T:])
        for o, (dh, hh) in zip(quads, QUADS):
            rest = p_v[slot, 2 * KO:, hh * T:(hh + 1) * T].astype(BF16)
            o_v[slot, dh * HD:(dh + 1) * HD, hh * T:(hh + 1) * T] = (
                o + _dot(woutt_v[dh * HD:(dh + 1) * HD, 2 * KO:], rest))

    def finish(i, slot):
        for hh, rs in enumerate(halves(i)):
            o = o_v[slot, :, hh * T:(hh + 1) * T].T
            out_v[rs, :] = (x1_v[rs, :] + scale(o, 4)).astype(out_v.dtype)
        for cp in out_copies(i):
            cp.start()

    def step_c(i, slot, n_done):
        acts = [_gelu2(z) for z in project1(i)]
        gates = mix(i)
        if n_done >= 2:
            finish(i - 2, slot)
        if n_done >= 1:
            project_out(1 - slot)
        gate(i, slot, acts, gates)

    def two_steps_c(n, carry):
        step_c(2 * n, 0, 2)
        step_c(2 * n + 1, 1, 2)
        return carry

    step_c(0, 0, 0)
    step_c(1, 1, 1)
    lax.fori_loop(1, nb // 2, two_steps_c, None)
    project_out((nb - 1) % 2)
    finish(nb - 2, nb % 2)
    finish(nb - 1, (nb - 1) % 2)
    for i in range(nb):
        for cp in out_copies(i):
            cp.wait()


@jax.jit
def pallas_adaLN_cond__ssm_conv_h3__mixer_gmlp__prompt_kernel(
    A_q: jax.Array,
    A_k: jax.Array,
    A_v: jax.Array,
    A_shift_k: jax.Array,
    A_ssm_k: jax.Array,
    A_ssm_D: jax.Array,
    B_x: jax.Array,
    B_w_in: jax.Array,
    B_w_sp: jax.Array,
    B_b_sp: jax.Array,
    B_w_out: jax.Array,
    c: jax.Array,
    w_mod: jax.Array,
):
    del B_x
    B, S, D = A_q.shape
    FH = B_w_out.shape[0]
    assert B == 1 and S % C == 0 and D % LANES == 0 and B_w_in.shape[1] == 2 * FH
    NA, NJ = S // C, D // LANES
    fwd, inv = _dft_matrices()
    operands = (
        A_q.reshape(S, D), A_k.reshape(S, D), A_v.reshape(S, D), A_shift_k.T, A_ssm_k, A_ssm_D,
        B_w_in.T, B_w_sp, B_b_sp, B_w_out, c, w_mod,
        fwd.astype(BF16), inv.astype(BF16),
    )
    spectrum = (2 * R, M // 8, 8, LANES)
    scratch = [pltpu.VMEM(o.shape, o.dtype) for o in operands] + [
        pltpu.VMEM((NJ, NA) + spectrum, F32),
        pltpu.VMEM((NJ, NA - 1) + spectrum, F32),
        pltpu.VMEM((NA, C, LANES), F32),
        pltpu.VMEM((HIST + C, LANES), F32),
        pltpu.VMEM((C, LANES), F32),
        pltpu.VMEM((NJ, S, LANES), F32),
        pltpu.VMEM((S, D), F32),
        pltpu.VMEM((16, D), F32),
        pltpu.VMEM((5, 8, D), F32),
        pltpu.VMEM((S, D), BF16),
        pltpu.VMEM((2, 2 * T, D), BF16),
        pltpu.VMEM((2, FH, 2 * T), F32),
        pltpu.VMEM((2, 8, 2 * T), F32),
        pltpu.VMEM((7, FH // 2, S // 2), BF16),
        pltpu.VMEM((7, FH // 2, (NJ // 2) * LANES), BF16),
        pltpu.VMEM((7, D // 2, (FH // (2 * LANES)) * LANES), BF16),
        pltpu.VMEM((2, FH, 2 * T), F32 if S2 else BF16),
        pltpu.VMEM((2, D, 2 * T), F32),
        pltpu.VMEM((D, FH), BF16),
        pltpu.VMEM((8, S), F32),
        pltpu.VMEM((S, D), A_q.dtype),
        pltpu.SemaphoreType.DMA((64,)),
    ]
    out = pl.pallas_call(
        _kernel,
        out_shape=jax.ShapeDtypeStruct((S, D), A_q.dtype),
        in_specs=[pl.BlockSpec(memory_space=pl.ANY)] * len(operands),
        out_specs=pl.BlockSpec(memory_space=pl.ANY),
        scratch_shapes=scratch,
        compiler_params=pltpu.CompilerParams(vmem_limit_bytes=110 * 2**20, flags=FLAGS),
    )(*operands)
    return out.reshape(B, S, D)
```

```python
import functools

import numpy as np

import jax
import jax.numpy as jnp
from jax import lax
import jax.experimental.pallas as pl
import jax.experimental.pallas.tpu as pltpu

LANES = 128
R = 4
M = 128
C = R * M
HIST = 16
EPS = 1e-5
GELU_C1 = float(np.sqrt(2.0 / np.pi))
GELU_C3 = float(np.sqrt(2.0 / np.pi) * 0.044715)
T = 128
PR = 32
MB = 288
NR = 288
NO = 16
FLAGS = None
PH = 'ABC'
GL = 3
TW = 4
SYNC = (1, 2, 4)
ORD = (1, 4, 2, 3, 0, 6, 5)
PAD = 0
XC = 1
CP = 0
DL = -1
CO = 1
NP = 8
KM = 128
KG = 16

F32 = jnp.float32
BF16 = jnp.bfloat16
U32 = jnp.uint32
NT = (((1,), (1,)), ((), ()))
QUADS = ((0, 0), (0, 1), (1, 0), (1, 1))


def _dft_matrix():
    f0 = np.arange(M)[:, None]
    m = np.arange(M)[None, :]
    fwd = np.zeros((R, 2 * M, M), np.float64)
    for r in range(R):
        n = R * m + r
        ph = -np.pi * ((n * (1 + 4 * f0)) % (4 * C)) / (2 * C)
        re = np.cos(ph).reshape(M // 8, 8, M)
        im = np.sin(ph).reshape(M // 8, 8, M)
        fwd[r] = np.stack([re, im], 1).reshape(2 * M, M)
    return fwd.astype(np.float32)


def _pack(x):
    return pltpu.bitcast(x.astype(BF16), U32)


def _unpack(w):
    return pltpu.bitcast(w, BF16)


def _join_rows(even, odd):
    return pltpu.pack_elementwise([even, odd], packed_dtype=BF16)


def _split_rows(w):
    return [pltpu.unpack_elementwise(w, index=n, packed_dtype=BF16, unpacked_dtype=F32) for n in range(2)]


def _np_pack(x):
    bits = x.astype(BF16).view(np.uint16).astype(np.uint32)
    return bits[..., 0::2, :] | (bits[..., 1::2, :] << 16)


def _dot(a, b):
    return jnp.dot(a, b, preferred_element_type=F32)


def _dot_nt(a, b):
    return lax.dot_general(a, b, NT, preferred_element_type=F32)


def _gelu2(x):
    t = jnp.tanh(x * (x * x * GELU_C3 + GELU_C1))
    return x * t + x


def _ln_rows(x):
    n = x.shape[-1]
    d = x - jnp.sum(x, axis=-1, keepdims=True) * (1.0 / n)
    var = jnp.sum(d * d, axis=-1, keepdims=True) * (1.0 / n)
    return d * lax.rsqrt(var + EPS)


def _interleave(*streams):
    order = sorted(((n + (0.5 if k else 0.0)) / len(st), k, n)
                   for k, st in enumerate(streams) for n in range(len(st)))
    for _, k, n in order:
        streams[k][n]()


def _strassen_left(a11, a12, a21, a22):
    return (a11 + a22, a21 + a22, a11, a22, a11 + a12, a21 - a11, a12 - a22)


def _strassen_right(b11, b12, b21, b22):
    f11, f12, f21, f22 = (b.astype(F32) for b in (b11, b12, b21, b22))
    return [b.astype(BF16) for b in (f11 + f22, b11, f12 - f22, f21 - f11, b22, f11 + f12, f21 + f22)]


def _strassen(product, rest):
    m2, m4 = product(1), product(3)
    yield (1, 0), m2 + m4 + rest(1, 0)
    m5, m3 = product(4), product(2)
    yield (0, 1), m3 + m5 + rest(0, 1)
    m1, m7 = product(0), product(6)
    yield (0, 0), (m4 - m5) + m1 + m7 + rest(0, 0)
    yield (1, 1), (m3 - m2) + m1 + product(5) + rest(1, 1)


def _strassen_sum(products):
    m1, m2, m3, m4, m5, m6, m7 = products
    return (m4 - m5) + m1 + m7, m3 + m5, m2 + m4, (m3 - m2) + m1 + m6


def _butterfly(x, inverse):
    (r0, i0), (r1, i1), (r2, i2), (r3, i3) = x
    ar, ai, br, bi = r0 + r2, i0 + i2, r0 - r2, i0 - i2
    cr, ci, dr, di = r1 + r3, i1 + i3, r1 - r3, i1 - i3
    lo, hi = (br + di, bi - dr), (br - di, bi + dr)
    if inverse:
        lo, hi = hi, lo
    return [(ar + cr, ai + ci), lo, (ar - cr, ai - ci), hi]


def _forward(f_v, phases):
    es = []
    for r in range(R):
        e = _dot(_unpack(f_v[r]), phases[r].astype(BF16)).reshape(M // 8, 2, 8, LANES)
        es.append((e[:, 0], e[:, 1]))
    return _butterfly(es, inverse=False)


def _kernel(q_h, k_h, v_h, sk_h, g_h, sd_h, win_h, wsp_h, bsp_h, wout_h, c_h, wmod_h, f_h,
            out_h,
            q_v, k_v, v_v, sk_v, g_v, sd_v, win_v, wsp_v, bsp_v, wout_v, c_v, wmod_v, f_v, fi_v,
            gs_v, us_v, gt_v, kf_v, vf_v, y_v, x1_v, flag_v, row_v, tap_v, mod_v, h_v, w_v, acc_v, a2_v, mean_v, zs_v,
            wis_v, wos_v, p_v, pr_v, o_v, woutt_v, brow_v, out_v, sems):
    S, D = q_v.shape
    FH = wout_v.shape[0]
    NA, NJ = S // C, D // LANES
    KS = sk_v.shape[0]
    HS, HF, HD = S // 2, FH // 2, D // 2
    nb = S // (2 * T)

    n_sem = [NJ + nb]

    def fetch(src, dst):
        cp = pltpu.make_async_copy(src, dst, sems.at[n_sem[0]])
        n_sem[0] += 1
        cp.start()
        return cp

    def rows(ref, i, n):
        return ref.at[pl.ds(i * n, n)]

    def cols(ref, i, n):
        return ref.at[:, pl.ds(i * n, n)]

    def filter_rows(j):
        rs = pl.ds(pl.multiple_of(j * LANES, LANES), LANES)
        return pltpu.make_async_copy(g_h.at[rs], g_v.at[rs], sems.at[j])

    def mix_cols(i):
        cs = pl.ds(pl.multiple_of(i * 2 * T, 2 * T), 2 * T)
        return pltpu.make_async_copy(wsp_h.at[:, cs], wsp_v.at[i], sems.at[NJ + i])

    filter_rows(0).start()
    cp_small = [fetch(f_h, f_v), fetch(sd_h, sd_v), fetch(sk_h, sk_v), fetch(c_h, c_v)]
    for j in range(1, NJ):
        filter_rows(j).start()
    cp_kv = [(fetch(rows(k_h, a, C), rows(k_v, a, C)), fetch(rows(v_h, a, C), rows(v_v, a, C)))
             for a in range(NA)]

    def q_block(i):
        return fetch(rows(q_h, i, 2 * T), rows(q_v, i, 2 * T))

    cp_q = [q_block(0)]
    cp_wmod = {n: fetch(cols(wmod_h, n, D), cols(wmod_v, n, D)) for n in (2, 1, 0, 4, 3)}
    cp_win = {1: fetch(rows(win_h, 1, FH), rows(win_v, 1, FH))}
    cp_q += [q_block(1)]
    cp_rest = []

    def fetch_group(i):
        later = [n for n in SYNC if n > i]
        for n in range(i, (later + [nb + 1])[0]):
            if n + 1 < nb:
                cp_q.append(q_block(n + 1))
            mix_cols(n - 1).start()
        if not later:
            cp_wmod[5] = fetch(cols(wmod_h, 5, D), cols(wmod_v, 5, D))
            cp_win[0] = fetch(rows(win_h, 0, FH), rows(win_v, 0, FH))
            cp_rest.extend([fetch(bsp_h, bsp_v), fetch(wout_h, wout_v)])

    fetch_group(SYNC[0])
    flag_v[0] = 0

    def clear(n):
        acc_v[n, :7 * HF] = jnp.zeros((7 * HF, T), F32)

    pl.loop(0, nb - NJ)(clear)

    for cp in cp_small:
        cp.wait()
    sd_row = sd_v[...].astype(F32).reshape(1, D)
    sk = sk_v[...].astype(F32)
    tap_v[KS] = jnp.broadcast_to(sd_row, (8, D))
    for t in range(KS):
        tap_v[t] = jnp.broadcast_to(sk[t:t + 1] * (1.0 / C), (8, D))

    for r in range(R):
        fi_v[r] = _pack(_unpack(f_v[r]).T)

    def filter_spectrum(j, carry):
        filter_rows(j).wait()
        rs = pl.ds(pl.multiple_of(j * LANES, LANES), LANES)
        prev = None
        for a in range(NA):
            gt_v[a] = g_v[rs, a * C:(a + 1) * C].T.astype(F32)
            spec = _forward(f_v, [gt_v[a, pl.ds(r, M, stride=R), :] for r in range(R)])
            for qq in range(R):
                re, im = spec[qq]
                if a == 0:
                    re = re + tap_v[KS, :, rs]
                    spec[qq] = (re, im)
                else:
                    re, im = re - prev[qq][1], im + prev[qq][0]
                gs_v[j, a, 2 * qq] = re
                gs_v[j, a, 2 * qq + 1] = im
            prev = spec

    if 'A' in PH:
        lax.fori_loop(0, NJ, filter_spectrum, None)

    def widen(a, j):
        lanes = slice(j * LANES, (j + 1) * LANES)
        if j == 0:
            for cp in cp_kv[a]:
                cp.wait()
        if a == 0:
            kf_v[j, 0:HIST, :] = jnp.zeros((HIST, LANES), F32)
            kf_v[j, HIST:, :] = k_v[0:C, lanes].astype(F32)
        else:
            kf_v[j] = k_v[a * C - HIST:(a + 1) * C, lanes].astype(F32)
        vf_v[j] = v_v[a * C:(a + 1) * C, lanes].astype(F32)

    def analyse(a, j):
        lanes = slice(j * LANES, (j + 1) * LANES)
        phases = [[] for _ in range(R)]
        for m0 in range(0, M, KM):
            kp = {s: kf_v[j, pl.ds(HIST + R * m0 + s, KM, stride=R), :] for s in range(1 - KS, R)}
            taps = [jnp.concatenate([tap_v[t, :, lanes]] * (KM // 8), axis=0) for t in range(KS)]
            for r in range(R):
                acc = kp[r] * taps[0]
                for t in range(1, KS):
                    acc = acc + kp[r - t] * taps[t]
                phases[r].append(acc * vf_v[j, pl.ds(R * m0 + r, KM, stride=R), :])
        spec = _forward(f_v, [jnp.concatenate(ph, axis=0) for ph in phases])
        for qq in range(R):
            us_v[j, a, 2 * qq], us_v[j, a, 2 * qq + 1] = spec[qq]

    def synthesise(a, j):
        packed = [[] for _ in range(R)]
        for g0 in range(0, M // 8, KG):
            gs = slice(g0, g0 + KG)
            ys = []
            for qq in range(R):
                yr = yi = None
                for b in range(a + 1):
                    ur, ui = us_v[j, a - b, 2 * qq, gs], us_v[j, a - b, 2 * qq + 1, gs]
                    gr, gi = gs_v[j, b, 2 * qq, gs], gs_v[j, b, 2 * qq + 1, gs]
                    tr, ti = gr * ur - gi * ui, gr * ui + gi * ur
                    yr, yi = (tr, ti) if b == 0 else (yr + tr, yi + ti)
                ys.append((yr, yi))
            for r, b in enumerate(_butterfly(ys, inverse=True)):
                packed[r].append(jnp.stack(b, axis=1).reshape(16 * KG, LANES).astype(BF16))
        if a == NA - 1:
            clear(nb - NJ + j)
        for r in range(R):
            y_v[j, pl.ds(a * C + r, M, stride=R), :] = _dot(
                _unpack(fi_v[r]), jnp.concatenate(packed[r], axis=0))

    if 'A' in PH:
        tiles = [(a, j) for a in range(NA) for j in range(NJ)]
        stages = ((widen, 0), (analyse, 1), (synthesise, 2))
        for n in range(len(tiles) + 2):
            for fn, lag in stages:
                if 0 <= n - lag < len(tiles):
                    fn(*tiles[n - lag])

    def modulation(n):
        if n < 5:
            cp_wmod[n].wait()
        return _dot(sc, wmod_v[:, n * D:(n + 1) * D])[0:8]

    cc = c_v[...].astype(F32)
    sc = jnp.broadcast_to(cc * jax.nn.sigmoid(cc), (16, D)).astype(BF16)
    ga, ca, sa, cb, sb = (modulation(n) for n in (2, 1, 0, 4, 3))
    mod_v[0] = ga * (1.0 + ca)
    mod_v[1] = ga * sa
    mod_v[2] = 1.0 + cb
    mod_v[3] = sb

    def scale(x, n):
        return (x.reshape(x.shape[0] // 8, 8, D) * mod_v[n]).reshape(x.shape)

    def shift(x, n):
        return (x.reshape(x.shape[0] // 8, 8, D) + mod_v[n]).reshape(x.shape)


    def halves(i, off=0, n=T):
        return [pl.ds(pl.multiple_of((2 * i + hh) * T + off, n), n) for hh in range(2)]

    def words(i, off=0, n=T):
        return [pl.ds(pl.multiple_of((2 * i + hh) * (T // 2) + off // 2, n // 2), n // 2) for hh in range(2)]

    last = []

    def paced(x, tiles=1):
        if not last:
            return x
        dep = last.pop()
        n = min(dep.shape[0], x.shape[0])
        dep = jnp.concatenate([dep[:n]] * (x.shape[0] // n), axis=0)
        cols = [x[:, c:c + LANES] for c in range(0, x.shape[1], LANES)]
        return jnp.concatenate([jnp.where(flag_v[0] > 0, dep, col) for col in cols[:tiles]] + cols[tiles:], axis=1)

    def delay(x):
        if DL < 0:
            return pltpu.roll(x, 1, 1)
        for _ in range(DL):
            x = jnp.tanh(x)
        return x

    def prepare(i):
        def piece(hh, off):
            rs = halves(i, off, PR)[hh]
            x = paced(q_v[rs, :].astype(F32))
            y = jnp.concatenate([y_v[j, rs, :] for j in range(NJ)], axis=1)
            x1 = x + shift(scale(_ln_rows(x), 0), 1) * y
            x1_v[rs, :] = x1
            h = shift(scale(_ln_rows(x1), 2), 3)
            h_v[words(i, off, PR)[hh], :] = _pack(h)
            last.append(h[:, -LANES:])

        return [functools.partial(piece, hh, off) for hh in range(2) for off in range(0, T, PR)]

    KI, KO = (NJ // 2) * LANES, (FH // (2 * LANES)) * LANES

    def project(i, fh):
        h1, h2 = (_unpack(h_v[hs, :]) for hs in words(i))
        right = _strassen_right(h1[:, :KI], h2[:, :KI], h1[:, KI:2 * KI], h2[:, KI:2 * KI])
        return _strassen(
            lambda n: _dot_nt(_unpack(wis_v[fh, n]), right[n]),
            lambda qh, hh: _dot_nt(_unpack(w_v[fh, qh, :, 2 * KI:]), (h1, h2)[hh][:, 2 * KI:]))

    def activate(i):
        tot = {}
        for (qh, hh), z in project(i, 1):
            a2 = _gelu2(z)
            a2_v[i % 2, hh, qh * HF:(qh + 1) * HF, :] = a2
            tot[hh] = tot.get(hh, 0.0) + jnp.sum(a2.reshape(HF // 8, 8, T), axis=0)
        for hh in range(2):
            mean = jnp.sum(tot[hh], axis=0, keepdims=True) * (1.0 / FH)
            mean_v[i % 2, :, hh * T:(hh + 1) * T] = jnp.broadcast_to(mean, (8, T))

    def normalize(i):
        state = {}

        def centred(rs, n, mean):
            a2 = jnp.concatenate([a2_v[i % 2, hh, rs, :] for hh in range(2)], axis=1)
            return a2.reshape(n // 8, 8, 2 * T) - mean

        def var_piece(r0):
            d = centred(pl.ds(r0, NR), NR, paced(mean_v[i % 2], 2))
            part = jnp.sum(d * d, axis=0)
            state["ss"] = part if r0 == 0 else state["ss"] + part
            last.append(delay(state["ss"][:, :LANES]))
            if r0 + NR == FH:
                var = jnp.sum(state["ss"], axis=0, keepdims=True) * (1.0 / FH)
                state["rstd"] = jnp.broadcast_to(lax.rsqrt(var + 4.0 * EPS), (8, 2 * T))

        def out_piece(r0):
            mean = paced(mean_v[i % 2], 2)
            parts = []
            for odd in range(2):
                za, zb = ((centred(pl.ds(r + odd, NO // 2, stride=2), NO // 2, mean) * state["rstd"]
                           ).reshape(NO // 2, 2 * T) for r in (r0, HF + r0))
                parts.append(jnp.concatenate(
                    _strassen_left(za[:, :T], za[:, T:], zb[:, :T], zb[:, T:]), axis=1))
            words = _join_rows(*parts)
            zs_v[i % 2, r0 // 2:(r0 + NO) // 2, :] = words
            last.append(delay(pltpu.bitcast(words[-8:, :T], F32)))

        return ([functools.partial(var_piece, r0) for r0 in range(0, FH, NR)]
                + [functools.partial(out_piece, r0) for r0 in range(0, HF, NO)])

    def mix(i):
        def block(k0, th, sh, n):
            return jnp.concatenate([wsp_v[i, (2 * k + th) * T:(2 * k + th + 1) * T, sh * T:(sh + 1) * T]
                                    for k in range(k0, k0 + TW)], axis=0)

        for k0 in range(0, nb, TW):
            for n in ORD:
                right = _strassen_right(*(block(k0, th, sh, n) for sh in range(2) for th in range(2)))[n]
                m = _dot_nt(_unpack(zs_v[i % 2, :, n * T:(n + 1) * T]), right)
                for k in range(TW):
                    acc_v[k0 + k, n * HF:(n + 1) * HF] += m[:, k * T:(k + 1) * T]

    def step_b(i):
        if i in SYNC:
            upto = ([n for n in SYNC if n > i] + [nb + 1])[0]
            for n in range(i, upto):
                mix_cols(n - 1).wait()
                if n + 1 < nb:
                    cp_q[n + 1].wait()
            if upto > nb:
                for cp in [cp_wmod[5], cp_win[0]] + cp_rest:
                    cp.wait()
            else:
                fetch_group(upto)
        activate(i)
        mix(i - 1)
        side = prepare(i + 1) if i + 1 < nb else []
        if i == 1 or not XC:
            last.clear()
        _interleave(side + normalize(i))

    def unpaced(pieces):
        for piece in pieces:
            last.clear()
            piece()

    def split_left(dst, top, bottom, width):
        for r0 in range(0, top.shape[0], 8):
            blk = [_split_rows(src[r0:r0 + 8, k:k + width]) for src in (top, bottom) for k in (0, width)]
            even, odd = (_strassen_left(*(b[n] for b in blk)) for n in range(2))
            for n in range(7):
                dst[n, r0:r0 + 8, :] = _join_rows(even[n], odd[n])

    def load_w_in(fh):
        for qh in range(2):
            for dst, src, n in ((0, qh * KO, KO), (KO, 2 * KO + qh * (HF - KO), HF - KO)):
                w_v[fh, qh, dst // 2:(dst + n) // 2] = _pack(win_v[fh * FH + src:fh * FH + src + n, :])
        split_left(wis_v.at[fh], w_v.at[fh, 0], w_v.at[fh, 1], KI)

    cp_q[0].wait()
    if 'C' in PH:
        unpaced(prepare(0))
        cp_win[1].wait()
        load_w_in(1)
        activate(0)
    cp_q[1].wait()
    if 'C' in PH:
        unpaced(prepare(1))
        unpaced(normalize(0))
    if 'B' in PH:
        for i in range(1, nb if 'C' in PH else 4):
            step_b(i)
    if 'C' not in PH:
        out_v[0:16, 0:128] = (x1_v[0:16, 0:128] + y_v[1, 0:16, :] + acc_v[1, 0:16, :]).astype(BF16) + _unpack(h_v[0:8, 0:128] + zs_v[0, 0:8, 0:128])
        pltpu.sync_copy(out_v, out_h)
        pltpu.sync_copy(zs_v.at[0, pl.ds(0, 8), pl.ds(0, 640)], h_v.at[pl.ds(0, 8)])
        return

    out_sem0 = n_sem[0]

    def out_copies(i):
        return [pltpu.make_async_copy(out_v.at[rs], out_h.at[rs], sems.at[out_sem0 + 2 * i + hh])
                for hh, rs in enumerate(halves(i))]

    def gate(i, slot, zs):
        gates = _strassen_sum([acc_v[i, n * HF:(n + 1) * HF] for n in range(7)])
        ps = [None] * 4
        for (qh, hh), z in zs:
            g = gates[2 * qh + hh]
            g = (g.reshape(HF // 8, 8, T) + brow_v[:, halves(i)[hh]]).reshape(HF, T)
            ps[2 * qh + hh] = _gelu2(z) * g
        for n, val in enumerate(_strassen_right(*(p[:KO] for p in ps))):
            p_v[slot, n] = val
        for hh in range(2):
            pr_v[slot, hh] = jnp.concatenate([ps[hh][KO:], ps[2 + hh][KO:]], axis=0).astype(BF16)

    def project_out(slot):
        for (dh, hh), o in _strassen(
                lambda n: _dot(_unpack(wos_v[n]), p_v[slot, n]),
                lambda dh, hh: _dot(_unpack(woutt_v[dh, :, 2 * KO:]), pr_v[slot, hh])):
            o_v[slot, hh, dh * HD:(dh + 1) * HD] = o

    def finish(i, slot):
        for hh, rs in enumerate(halves(i)):
            out_v[rs, :] = (x1_v[rs, :] + scale(o_v[slot, hh].T, 4)).astype(out_v.dtype)
        for cp in out_copies(i):
            cp.start()

    def step_c(i, slot, n_done):
        if CO:
            if n_done >= 2:
                finish(i - 2, slot)
            gate(i, slot, project(i, 0))
            project_out(1 - slot)
        else:
            if n_done >= 2:
                finish(i - 2, slot)
            project_out(1 - slot)
            gate(i, slot, project(i, 0))

    mix(nb - 1)
    load_w_in(0)
    brow_v[...] = jnp.broadcast_to(bsp_v[...].astype(F32).reshape(1, S), (8, S))
    woutt = _pack(wout_v[...].T)
    for dh in range(2):
        woutt_v[dh] = woutt[dh * HD // 2:(dh + 1) * HD // 2]
    split_left(wos_v, woutt_v.at[0], woutt_v.at[1], KO)
    gate(0, 0, project(0, 0))
    mod_v[4] = 0.5 * modulation(5)
    for i in range(1, nb):
        step_c(i, i % 2, i)
    project_out(1)
    finish(nb - 2, 0)
    finish(nb - 1, 1)
    for i in range(nb):
        for cp in out_copies(i):
            cp.wait()


@jax.jit
def pallas_adaLN_cond__ssm_conv_h3__mixer_gmlp__prompt_kernel(
    A_q: jax.Array,
    A_k: jax.Array,
    A_v: jax.Array,
    A_shift_k: jax.Array,
    A_ssm_k: jax.Array,
    A_ssm_D: jax.Array,
    B_x: jax.Array,
    B_w_in: jax.Array,
    B_w_sp: jax.Array,
    B_b_sp: jax.Array,
    B_w_out: jax.Array,
    c: jax.Array,
    w_mod: jax.Array,
):
    del B_x
    B, S, D = A_q.shape
    FH = B_w_out.shape[0]
    assert B == 1 and S % C == 0 and D % LANES == 0 and B_w_in.shape[1] == 2 * FH
    NA, NJ, NB = S // C, D // LANES, S // (2 * T)
    KO = (FH // (2 * LANES)) * LANES
    operands = (
        A_q.reshape(S, D), A_k.reshape(S, D), A_v.reshape(S, D), A_shift_k.T, A_ssm_k, A_ssm_D,
        B_w_in.T, B_w_sp, B_b_sp, B_w_out, c, w_mod,
        _np_pack(_dft_matrix()),
    )
    spectrum = (2 * R, M // 8, 8, LANES)
    scratch = [pltpu.VMEM((NB, S, 2 * T) if o is B_w_sp else o.shape, o.dtype) for o in operands] + [
        pltpu.VMEM((R, M // 2, 2 * M), U32),
        pltpu.VMEM((NJ, NA) + spectrum, F32),
        pltpu.VMEM((NJ, NA) + spectrum, F32),
        pltpu.VMEM((NA, C, LANES), F32),
        pltpu.VMEM((NJ, HIST + C, LANES), F32),
        pltpu.VMEM((NJ, C, LANES), F32),
        pltpu.VMEM((NJ, S, LANES), F32),
        pltpu.VMEM((S, D), F32),
        pltpu.SMEM((1,), jnp.int32),
        pltpu.VMEM((16, D), F32),
        pltpu.VMEM((A_shift_k.shape[1] + 1, 8, D), F32),
        pltpu.VMEM((5, 8, D), F32),
        pltpu.VMEM((S // 2, D), U32),
        pltpu.VMEM((2, 2, FH // 4, D), U32),
        pltpu.VMEM((NB, 7 * FH // 2 + PAD, T), F32),
        pltpu.VMEM((2, 2, FH, T), F32),
        pltpu.VMEM((2, 8, 2 * T), F32),
        pltpu.VMEM((2, FH // 4, 7 * T), U32),
        pltpu.VMEM((2, 7, FH // 4, (NJ // 2) * LANES), U32),
        pltpu.VMEM((7, D // 4, (FH // (2 * LANES)) * LANES), U32),
        pltpu.VMEM((2, 7, KO, T), BF16),
        pltpu.VMEM((2, 2, FH - 2 * KO, T), BF16),
        pltpu.VMEM((2, 2, D, T), F32),
        pltpu.VMEM((2, D // 4, FH), U32),
        pltpu.VMEM((8, S), F32),
        pltpu.VMEM((S, D), A_q.dtype),
        pltpu.SemaphoreType.DMA((64,)),
    ]
    out = pl.pallas_call(
        _kernel,
        out_shape=jax.ShapeDtypeStruct((S, D), A_q.dtype),
        in_specs=[pl.BlockSpec(memory_space=pl.ANY)] * len(operands),
        out_specs=pl.BlockSpec(memory_space=pl.ANY),
        scratch_shapes=scratch,
        compiler_params=pltpu.CompilerParams(vmem_limit_bytes=124 * 2**20, flags=FLAGS),
    )(*operands)
    return out.reshape(B, S, D)
```

```python
import functools

import numpy as np

import jax
import jax.numpy as jnp
from jax import lax
import jax.experimental.pallas as pl
import jax.experimental.pallas.tpu as pltpu

LANES = 128
R = 4
M = 128
C = R * M
HIST = 16
EPS = 1e-5
GELU_C1 = float(np.sqrt(2.0 / np.pi))
GELU_C3 = float(np.sqrt(2.0 / np.pi) * 0.044715)
T = 128
PR = 32
MB = 288
NR = 288
NO = 16
FLAGS = None
PH = 'ABC'
AHEAD = 4
MODAT = 0
TW = 4
SYNC = (1, 2, 4, 6)
ORD = (1, 4, 2, 3, 0, 6, 5)
PAD = 0
XC = 1
CSYNC = (4, 6)
CP = 0
DL = -1
CO = 1
NP = 8
KM = 128
KG = 16

F32 = jnp.float32
BF16 = jnp.bfloat16
U32 = jnp.uint32
NT = (((1,), (1,)), ((), ()))
QUADS = ((0, 0), (0, 1), (1, 0), (1, 1))


def _dft_matrix():
    f0 = np.arange(M)[:, None]
    m = np.arange(M)[None, :]
    fwd = np.zeros((R, 2 * M, M), np.float64)
    for r in range(R):
        n = R * m + r
        ph = -np.pi * ((n * (1 + 4 * f0)) % (4 * C)) / (2 * C)
        re = np.cos(ph).reshape(M // 8, 8, M)
        im = np.sin(ph).reshape(M // 8, 8, M)
        fwd[r] = np.stack([re, im], 1).reshape(2 * M, M)
    return fwd.astype(np.float32)


def _pack(x):
    return pltpu.bitcast(x.astype(BF16), U32)


def _unpack(w):
    return pltpu.bitcast(w, BF16)


def _join_rows(even, odd):
    return pltpu.pack_elementwise([even, odd], packed_dtype=BF16)


def _split_rows(w):
    return [pltpu.unpack_elementwise(w, index=n, packed_dtype=BF16, unpacked_dtype=F32) for n in range(2)]


def _np_pack(x):
    bits = x.astype(BF16).view(np.uint16).astype(np.uint32)
    return bits[..., 0::2, :] | (bits[..., 1::2, :] << 16)


def _dot(a, b):
    return jnp.dot(a, b, preferred_element_type=F32)


def _dot_nt(a, b):
    return lax.dot_general(a, b, NT, preferred_element_type=F32)


def _gelu2(x):
    t = jnp.tanh(x * (x * x * GELU_C3 + GELU_C1))
    return x * t + x


def _ln_rows(x):
    n = x.shape[-1]
    d = x - jnp.sum(x, axis=-1, keepdims=True) * (1.0 / n)
    var = jnp.sum(d * d, axis=-1, keepdims=True) * (1.0 / n)
    return d * lax.rsqrt(var + EPS)


def _interleave(*streams):
    order = sorted(((n + (0.5 if k else 0.0)) / len(st), k, n)
                   for k, st in enumerate(streams) for n in range(len(st)))
    for _, k, n in order:
        streams[k][n]()


def _strassen_left(a11, a12, a21, a22):
    return (a11 + a22, a21 + a22, a11, a22, a11 + a12, a21 - a11, a12 - a22)


def _strassen_right(b11, b12, b21, b22):
    f11, f12, f21, f22 = (b.astype(F32) for b in (b11, b12, b21, b22))
    return [b.astype(BF16) for b in (f11 + f22, b11, f12 - f22, f21 - f11, b22, f11 + f12, f21 + f22)]


def _strassen(product, rest):
    m2, m4 = product(1), product(3)
    yield (1, 0), m2 + m4 + rest(1, 0)
    m5, m3 = product(4), product(2)
    yield (0, 1), m3 + m5 + rest(0, 1)
    m1, m7 = product(0), product(6)
    yield (0, 0), (m4 - m5) + m1 + m7 + rest(0, 0)
    yield (1, 1), (m3 - m2) + m1 + product(5) + rest(1, 1)


def _strassen_sum(products):
    m1, m2, m3, m4, m5, m6, m7 = products
    return (m4 - m5) + m1 + m7, m3 + m5, m2 + m4, (m3 - m2) + m1 + m6


def _butterfly(x, inverse):
    (r0, i0), (r1, i1), (r2, i2), (r3, i3) = x
    ar, ai, br, bi = r0 + r2, i0 + i2, r0 - r2, i0 - i2
    cr, ci, dr, di = r1 + r3, i1 + i3, r1 - r3, i1 - i3
    lo, hi = (br + di, bi - dr), (br - di, bi + dr)
    if inverse:
        lo, hi = hi, lo
    return [(ar + cr, ai + ci), lo, (ar - cr, ai - ci), hi]


def _forward(f_v, phases):
    es = []
    for r in range(R):
        e = _dot(_unpack(f_v[r]), phases[r].astype(BF16)).reshape(M // 8, 2, 8, LANES)
        es.append((e[:, 0], e[:, 1]))
    return _butterfly(es, inverse=False)


def _kernel(q_h, k_h, v_h, sk_h, g_h, sd_h, win_h, wsp_h, bsp_h, wout_h, c_h, wmod_h, f_h,
            out_h,
            q_v, k_v, v_v, sk_v, g_v, sd_v, win_v, wsp_v, bsp_v, wout_v, c_v, wmod_v, f_v, fi_v,
            gs_v, us_v, gt_v, kf_v, vf_v, y_v, x1_v, flag_v, row_v, tap_v, mod_v, h_v, w_v, acc_v, a2_v, mean_v, zs_v,
            wis_v, wos_v, p_v, pr_v, o_v, woutt_v, brow_v, out_v, sems):
    S, D = q_v.shape
    FH = wout_v.shape[0]
    NA, NJ = S // C, D // LANES
    KS = sk_v.shape[0]
    HS, HF, HD = S // 2, FH // 2, D // 2
    nb = S // (2 * T)

    n_sem = [nb]

    def fetch(src, dst):
        cp = pltpu.make_async_copy(src, dst, sems.at[n_sem[0]])
        n_sem[0] += 1
        cp.start()
        return cp

    def rows(ref, i, n):
        return ref.at[pl.ds(i * n, n)]

    def cols(ref, i, n):
        return ref.at[:, pl.ds(i * n, n)]

    def mix_cols(i):
        cs = pl.ds(pl.multiple_of(i * 2 * T, 2 * T), 2 * T)
        return pltpu.make_async_copy(wsp_h.at[:, cs], wsp_v.at[i], sems.at[i])

    cp_g = [fetch(cols(g_h, 0, C), cols(g_v, 0, C))]
    cp_small = [fetch(f_h, f_v), fetch(sd_h, sd_v), fetch(sk_h, sk_v), fetch(c_h, c_v)]
    cp_kv = []
    for n in range(1, NA + AHEAD):
        if n < NA:
            cp_g.append(fetch(cols(g_h, n, C), cols(g_v, n, C)))
        if n >= AHEAD:
            cp_kv.append([fetch(rows(src, n - AHEAD, C), rows(dst, n - AHEAD, C))
                          for src, dst in ((k_h, k_v), (v_h, v_v))])

    def q_block(i):
        return fetch(rows(q_h, i, 2 * T), rows(q_v, i, 2 * T))

    cp_q = [q_block(0)]
    cp_wmod = {0: fetch(cols(wmod_h, 0, 5 * D), cols(wmod_v, 0, 5 * D))}
    cp_win = {1: fetch(rows(win_h, 1, FH), rows(win_v, 1, FH))}
    cp_q += [q_block(1)]
    cp_rest = []

    def fetch_group(i):
        later = [n for n in SYNC if n > i]
        for n in range(i, (later + [nb + 1])[0]):
            if n + 1 < nb:
                cp_q.append(q_block(n + 1))
            mix_cols(n - 1).start()
        if not later:
            cp_wmod[5] = fetch(cols(wmod_h, 5, D), cols(wmod_v, 5, D))
            cp_win[0] = fetch(rows(win_h, 0, FH), rows(win_v, 0, FH))
            cp_rest.extend([fetch(bsp_h, bsp_v), fetch(wout_h, wout_v)])

    fetch_group(SYNC[0])
    flag_v[0] = 0

    for cp in cp_small:
        cp.wait()
    sd_row = sd_v[...].astype(F32).reshape(1, D)
    sk = sk_v[...].astype(F32)
    tap_v[KS] = jnp.broadcast_to(sd_row, (8, D))
    for t in range(KS):
        tap_v[t] = jnp.broadcast_to(sk[t:t + 1] * (1.0 / C), (8, D))

    for r in range(R):
        fi_v[r] = _pack(_unpack(f_v[r]).T)

    raw = {}

    def transpose(a, j):
        gt_v[j] = g_v[j * LANES:(j + 1) * LANES, a * C:(a + 1) * C].T.astype(F32)

    def filter_spectrum(a, j):
        spec = _forward(f_v, [gt_v[j, pl.ds(r, M, stride=R), :] for r in range(R)])
        for qq in range(R):
            re, im = spec[qq]
            if a == 0:
                re = re + tap_v[KS, :, j * LANES:(j + 1) * LANES]
                spec[qq] = (re, im)
            else:
                re, im = re - raw[j][qq][1], im + raw[j][qq][0]
            gs_v[j, a, 2 * qq] = re
            gs_v[j, a, 2 * qq + 1] = im
        raw[j] = spec

    def widen(a, j):
        lanes = slice(j * LANES, (j + 1) * LANES)
        if a == 0:
            kf_v[j, 0:HIST, :] = jnp.zeros((HIST, LANES), F32)
            kf_v[j, HIST:, :] = k_v[0:C, lanes].astype(F32)
        else:
            kf_v[j] = k_v[a * C - HIST:(a + 1) * C, lanes].astype(F32)
        vf_v[j] = v_v[a * C:(a + 1) * C, lanes].astype(F32)

    def analyse(a, j):
        lanes = slice(j * LANES, (j + 1) * LANES)
        phases = [[] for _ in range(R)]
        for m0 in range(0, M, KM):
            kp = {s: kf_v[j, pl.ds(HIST + R * m0 + s, KM, stride=R), :] for s in range(1 - KS, R)}
            taps = [jnp.concatenate([tap_v[t, :, lanes]] * (KM // 8), axis=0) for t in range(KS)]
            for r in range(R):
                acc = kp[r] * taps[0]
                for t in range(1, KS):
                    acc = acc + kp[r - t] * taps[t]
                phases[r].append(acc * vf_v[j, pl.ds(R * m0 + r, KM, stride=R), :])
        spec = _forward(f_v, [jnp.concatenate(ph, axis=0) for ph in phases])
        for qq in range(R):
            us_v[j, a, 2 * qq], us_v[j, a, 2 * qq + 1] = spec[qq]

    def synthesise(a, j):
        packed = [[] for _ in range(R)]
        for g0 in range(0, M // 8, KG):
            gs = slice(g0, g0 + KG)
            ys = []
            for qq in range(R):
                yr = yi = None
                for b in range(a + 1):
                    ur, ui = us_v[j, a - b, 2 * qq, gs], us_v[j, a - b, 2 * qq + 1, gs]
                    gr, gi = gs_v[j, b, 2 * qq, gs], gs_v[j, b, 2 * qq + 1, gs]
                    tr, ti = gr * ur - gi * ui, gr * ui + gi * ur
                    yr, yi = (tr, ti) if b == 0 else (yr + tr, yi + ti)
                ys.append((yr, yi))
            for r, b in enumerate(_butterfly(ys, inverse=True)):
                packed[r].append(jnp.stack(b, axis=1).reshape(16 * KG, LANES).astype(BF16))
        for r in range(R):
            y_v[j, pl.ds(a * C + r, M, stride=R), :] = _dot(
                _unpack(fi_v[r]), jnp.concatenate(packed[r], axis=0))

    def modulation(n):
        cc = c_v[...].astype(F32)
        sc = jnp.broadcast_to(cc * jax.nn.sigmoid(cc), (16, D)).astype(BF16)
        return _dot(sc, wmod_v[:, n * D:(n + 1) * D])[0:8]

    def modulate():
        sa, ca, ga, sb, cb = (modulation(n) for n in range(5))
        mod_v[0] = ga * (1.0 + ca)
        mod_v[1] = ga * sa
        mod_v[2] = 1.0 + cb
        mod_v[3] = sb

    def scale(x, n):
        return (x.reshape(x.shape[0] // 8, 8, D) * mod_v[n]).reshape(x.shape)

    def shift(x, n):
        return (x.reshape(x.shape[0] // 8, 8, D) + mod_v[n]).reshape(x.shape)


    def halves(i, off=0, n=T):
        return [pl.ds(pl.multiple_of((2 * i + hh) * T + off, n), n) for hh in range(2)]

    def words(i, off=0, n=T):
        return [pl.ds(pl.multiple_of((2 * i + hh) * (T // 2) + off // 2, n // 2), n // 2) for hh in range(2)]

    last = []

    def paced(x, tiles=1):
        if not last:
            return x
        dep = last.pop()
        n = min(dep.shape[0], x.shape[0])
        dep = jnp.concatenate([dep[:n]] * (x.shape[0] // n), axis=0)
        cols = [x[:, c:c + LANES] for c in range(0, x.shape[1], LANES)]
        return jnp.concatenate([jnp.where(flag_v[0] > 0, dep, col) for col in cols[:tiles]] + cols[tiles:], axis=1)

    def delay(x):
        if DL < 0:
            return pltpu.roll(x, 1, 1)
        for _ in range(DL):
            x = jnp.tanh(x)
        return x

    def prepare(i):
        def piece(hh, off):
            rs = halves(i, off, PR)[hh]
            x = paced(q_v[rs, :].astype(F32))
            y = jnp.concatenate([y_v[j, rs, :] for j in range(NJ)], axis=1)
            x1 = x + shift(scale(_ln_rows(x), 0), 1) * y
            x1_v[rs, :] = x1
            h = shift(scale(_ln_rows(x1), 2), 3)
            h_v[words(i, off, PR)[hh], :] = _pack(h)
            last.append(h[:, -LANES:])

        return [functools.partial(piece, hh, off) for hh in range(2) for off in range(0, T, PR)]

    KI, KO = (NJ // 2) * LANES, (FH // (2 * LANES)) * LANES

    def project(i, fh):
        h1, h2 = (_unpack(h_v[hs, :]) for hs in words(i))
        right = _strassen_right(h1[:, :KI], h2[:, :KI], h1[:, KI:2 * KI], h2[:, KI:2 * KI])
        return _strassen(
            lambda n: _dot_nt(_unpack(wis_v[fh, n]), right[n]),
            lambda qh, hh: _dot_nt(_unpack(w_v[fh, qh, :, 2 * KI:]), (h1, h2)[hh][:, 2 * KI:]))

    def activate(i):
        tot = {}
        for (qh, hh), z in project(i, 1):
            a2 = _gelu2(z)
            a2_v[i % 2, hh, qh * HF:(qh + 1) * HF, :] = a2
            tot[hh] = tot.get(hh, 0.0) + jnp.sum(a2.reshape(HF // 8, 8, T), axis=0)
        for hh in range(2):
            mean = jnp.sum(tot[hh], axis=0, keepdims=True) * (1.0 / FH)
            mean_v[i % 2, :, hh * T:(hh + 1) * T] = jnp.broadcast_to(mean, (8, T))

    def normalize(i):
        state = {}

        def centred(rs, n, mean):
            a2 = jnp.concatenate([a2_v[i % 2, hh, rs, :] for hh in range(2)], axis=1)
            return a2.reshape(n // 8, 8, 2 * T) - mean

        def var_piece(r0):
            d = centred(pl.ds(r0, NR), NR, paced(mean_v[i % 2], 2))
            part = jnp.sum(d * d, axis=0)
            state["ss"] = part if r0 == 0 else state["ss"] + part
            last.append(delay(state["ss"][:, :LANES]))
            if r0 + NR == FH:
                var = jnp.sum(state["ss"], axis=0, keepdims=True) * (1.0 / FH)
                state["rstd"] = jnp.broadcast_to(lax.rsqrt(var + 4.0 * EPS), (8, 2 * T))

        def out_piece(r0):
            mean = paced(mean_v[i % 2], 2)
            parts = []
            for odd in range(2):
                za, zb = ((centred(pl.ds(r + odd, NO // 2, stride=2), NO // 2, mean) * state["rstd"]
                           ).reshape(NO // 2, 2 * T) for r in (r0, HF + r0))
                parts.append(jnp.concatenate(
                    _strassen_left(za[:, :T], za[:, T:], zb[:, :T], zb[:, T:]), axis=1))
            words = _join_rows(*parts)
            zs_v[i % 2, r0 // 2:(r0 + NO) // 2, :] = words
            last.append(delay(pltpu.bitcast(words[-8:, :T], F32)))

        return ([functools.partial(var_piece, r0) for r0 in range(0, FH, NR)]
                + [functools.partial(out_piece, r0) for r0 in range(0, HF, NO)])

    def mix(i):
        def block(k0, th, sh, n):
            return jnp.concatenate([wsp_v[i, (2 * k + th) * T:(2 * k + th + 1) * T, sh * T:(sh + 1) * T]
                                    for k in range(k0, k0 + TW)], axis=0)

        for k0 in range(0, nb, TW):
            for n in ORD:
                right = _strassen_right(*(block(k0, th, sh, n) for sh in range(2) for th in range(2)))[n]
                m = _dot_nt(_unpack(zs_v[i % 2, :, n * T:(n + 1) * T]), right)
                for k in range(TW):
                    at = (k0 + k, slice(n * HF, (n + 1) * HF))
                    part = m[:, k * T:(k + 1) * T]
                    acc_v[at] = acc_v[at] + part if i else part

    def step_b(i):
        if i in SYNC:
            upto = ([n for n in SYNC if n > i] + [nb + 1])[0]
            if upto <= nb:
                fetch_group(upto)
            for n in range(i, upto):
                mix_cols(n - 1).wait()
                if n + 1 < nb:
                    cp_q[n + 1].wait()
            if upto > nb:
                for cp in [cp_wmod[5], cp_win[0]] + cp_rest:
                    cp.wait()
        if i == 1:
            last.clear()
            _interleave(normalize(0))
        activate(i)
        mix(i - 1)
        side = prepare(i + 1) if i + 1 < nb else []
        if i == 1 or not XC:
            last.clear()
        _interleave(side + normalize(i))

    def unpaced(pieces):
        for piece in pieces:
            last.clear()
            piece()

    def split_left(dst, top, bottom, width):
        for r0 in range(0, top.shape[0], 8):
            blk = [_split_rows(src[r0:r0 + 8, k:k + width]) for src in (top, bottom) for k in (0, width)]
            even, odd = (_strassen_left(*(b[n] for b in blk)) for n in range(2))
            for n in range(7):
                dst[n, r0:r0 + 8, :] = _join_rows(even[n], odd[n])

    def load_w_in(fh):
        for qh in range(2):
            for dst, src, n in ((0, qh * KO, KO), (KO, 2 * KO + qh * (HF - KO), HF - KO)):
                w_v[fh, qh, dst // 2:(dst + n) // 2] = _pack(win_v[fh * FH + src:fh * FH + src + n, :])
        split_left(wis_v.at[fh], w_v.at[fh, 0], w_v.at[fh, 1], KI)

    tiles = [(a, j) for a in range(NA) for j in range(NJ)]
    lead = AHEAD * NJ
    stages = ((transpose, 0), (filter_spectrum, 1), (widen, lead), (analyse, lead + 1), (synthesise, lead + 2))
    for n in range(len(tiles) + lead + 2):
        if n % NJ == 0:
            if n < len(tiles):
                cp_g[n // NJ].wait()
            if 0 <= n - lead < len(tiles):
                for cp in cp_kv[(n - lead) // NJ]:
                    cp.wait()
        if n == len(tiles) + lead - MODAT:
            cp_q[0].wait()
            cp_wmod[0].wait()
            modulate()
            unpaced(prepare(0))
        for fn, lag in stages:
            if 0 <= n - lag < len(tiles) and 'A' in PH:
                fn(*tiles[n - lag])

    cp_win[1].wait()
    cp_q[1].wait()
    if 'C' in PH:
        load_w_in(1)
        activate(0)
        unpaced(prepare(1))
    if 'S' in PH:
        mix_cols(0).wait()
        cp_q[2].wait()
        _interleave(normalize(0))
        activate(1)
        pltpu.sync_copy(out_v.at[pl.ds(0, 8)], out_h.at[pl.ds(0, 8)])
        pltpu.sync_copy(zs_v.at[0, pl.ds(0, 8), pl.ds(0, 640)], h_v.at[pl.ds(0, 8)])
        return
    if 'B' in PH:
        for i in range(1, nb if 'C' in PH else 4):
            step_b(i)
    if 'C' not in PH:
        out_v[0:16, 0:128] = (x1_v[0:16, 0:128] + y_v[1, 0:16, :] + acc_v[1, 0:16, :]).astype(BF16) + _unpack(h_v[0:8, 0:128] + zs_v[0, 0:8, 0:128])
        pltpu.sync_copy(out_v, out_h)
        pltpu.sync_copy(zs_v.at[0, pl.ds(0, 8), pl.ds(0, 640)], h_v.at[pl.ds(0, 8)])
        return

    out_sem0 = n_sem[0]

    def out_copies(i):
        return [pltpu.make_async_copy(out_v.at[rs], out_h.at[rs], sems.at[out_sem0 + 2 * i + hh])
                for hh, rs in enumerate(halves(i))]

    def gate(i, slot, zs):
        gates = _strassen_sum([acc_v[i, n * HF:(n + 1) * HF] for n in range(7)])
        ps = [None] * 4
        for (qh, hh), z in zs:
            g = gates[2 * qh + hh]
            g = (g.reshape(HF // 8, 8, T) + brow_v[:, halves(i)[hh]]).reshape(HF, T)
            ps[2 * qh + hh] = _gelu2(z) * g
        for n, val in enumerate(_strassen_right(*(p[:KO] for p in ps))):
            p_v[slot, n] = val
        for hh in range(2):
            pr_v[slot, hh] = jnp.concatenate([ps[hh][KO:], ps[2 + hh][KO:]], axis=0).astype(BF16)

    def project_out(slot):
        for (dh, hh), o in _strassen(
                lambda n: _dot(_unpack(wos_v[n]), p_v[slot, n]),
                lambda dh, hh: _dot(_unpack(woutt_v[dh, :, 2 * KO:]), pr_v[slot, hh])):
            o_v[slot, hh, dh * HD:(dh + 1) * HD] = o

    def finish(i, slot):
        for hh, rs in enumerate(halves(i)):
            out_v[rs, :] = (x1_v[rs, :] + scale(o_v[slot, hh].T, 4)).astype(out_v.dtype)
        for cp in out_copies(i):
            cp.start()

    def step_c(i, slot, n_done):
        if CO:
            if n_done >= 2:
                finish(i - 2, slot)
            gate(i, slot, project(i, 0))
            project_out(1 - slot)
        else:
            if n_done >= 2:
                finish(i - 2, slot)
            project_out(1 - slot)
            gate(i, slot, project(i, 0))

    mix(nb - 1)
    load_w_in(0)
    brow_v[...] = jnp.broadcast_to(bsp_v[...].astype(F32).reshape(1, S), (8, S))
    woutt = _pack(wout_v[...].T)
    for dh in range(2):
        woutt_v[dh] = woutt[dh * HD // 2:(dh + 1) * HD // 2]
    split_left(wos_v, woutt_v.at[0], woutt_v.at[1], KO)
    gate(0, 0, project(0, 0))
    mod_v[4] = 0.5 * modulation(5)
    done = 0
    for i in range(1, nb):
        if i in CSYNC:
            for cp in out_copies(done):
                cp.wait()
            done += 1
        step_c(i, i % 2, i)
    project_out(1)
    finish(nb - 2, 0)
    finish(nb - 1, 1)
    for i in range(done, nb):
        for cp in out_copies(i):
            cp.wait()


@jax.jit
def pallas_adaLN_cond__ssm_conv_h3__mixer_gmlp__prompt_kernel(
    A_q: jax.Array,
    A_k: jax.Array,
    A_v: jax.Array,
    A_shift_k: jax.Array,
    A_ssm_k: jax.Array,
    A_ssm_D: jax.Array,
    B_x: jax.Array,
    B_w_in: jax.Array,
    B_w_sp: jax.Array,
    B_b_sp: jax.Array,
    B_w_out: jax.Array,
    c: jax.Array,
    w_mod: jax.Array,
):
    del B_x
    B, S, D = A_q.shape
    FH = B_w_out.shape[0]
    assert B == 1 and S % C == 0 and D % LANES == 0 and B_w_in.shape[1] == 2 * FH
    NA, NJ, NB = S // C, D // LANES, S // (2 * T)
    KO = (FH // (2 * LANES)) * LANES
    operands = (
        A_q.reshape(S, D), A_k.reshape(S, D), A_v.reshape(S, D), A_shift_k.T, A_ssm_k, A_ssm_D,
        B_w_in.T, B_w_sp, B_b_sp, B_w_out, c, w_mod,
        _np_pack(_dft_matrix()),
    )
    spectrum = (2 * R, M // 8, 8, LANES)
    scratch = [pltpu.VMEM((NB, S, 2 * T) if o is B_w_sp else o.shape, o.dtype) for o in operands] + [
        pltpu.VMEM((R, M // 2, 2 * M), U32),
        pltpu.VMEM((NJ, NA) + spectrum, F32),
        pltpu.VMEM((NJ, NA) + spectrum, F32),
        pltpu.VMEM((NJ, C, LANES), F32),
        pltpu.VMEM((NJ, HIST + C, LANES), F32),
        pltpu.VMEM((NJ, C, LANES), F32),
        pltpu.VMEM((NJ, S, LANES), F32),
        pltpu.VMEM((S, D), F32),
        pltpu.SMEM((1,), jnp.int32),
        pltpu.VMEM((16, D), F32),
        pltpu.VMEM((A_shift_k.shape[1] + 1, 8, D), F32),
        pltpu.VMEM((5, 8, D), F32),
        pltpu.VMEM((S // 2, D), U32),
        pltpu.VMEM((2, 2, FH // 4, D), U32),
        pltpu.VMEM((NB, 7 * FH // 2 + PAD, T), F32),
        pltpu.VMEM((2, 2, FH, T), F32),
        pltpu.VMEM((2, 8, 2 * T), F32),
        pltpu.VMEM((2, FH // 4, 7 * T), U32),
        pltpu.VMEM((2, 7, FH // 4, (NJ // 2) * LANES), U32),
        pltpu.VMEM((7, D // 4, (FH // (2 * LANES)) * LANES), U32),
        pltpu.VMEM((2, 7, KO, T), BF16),
        pltpu.VMEM((2, 2, FH - 2 * KO, T), BF16),
        pltpu.VMEM((2, 2, D, T), F32),
        pltpu.VMEM((2, D // 4, FH), U32),
        pltpu.VMEM((8, S), F32),
        pltpu.VMEM((S, D), A_q.dtype),
        pltpu.SemaphoreType.DMA((64,)),
    ]
    out = pl.pallas_call(
        _kernel,
        out_shape=jax.ShapeDtypeStruct((S, D), A_q.dtype),
        in_specs=[pl.BlockSpec(memory_space=pl.ANY)] * len(operands),
        out_specs=pl.BlockSpec(memory_space=pl.ANY),
        scratch_shapes=scratch,
        compiler_params=pltpu.CompilerParams(vmem_limit_bytes=124 * 2**20, flags=FLAGS),
    )(*operands)
    return out.reshape(B, S, D)
```

```python
import functools

import numpy as np

import jax
import jax.numpy as jnp
from jax import lax
import jax.experimental.pallas as pl
import jax.experimental.pallas.tpu as pltpu

LANES = 128
R = 4
M = 128
C = R * M
HIST = 16
EPS = 1e-5
GELU_C1 = float(np.sqrt(2.0 / np.pi))
GELU_C3 = float(np.sqrt(2.0 / np.pi) * 0.044715)
T = 128
PR = 32
MB = 288
NR = 288
NO = 16
FLAGS = None
PH = 'ABC'
AHEAD = 4
MODAT = 0
TW = 4
SYNC = (1, 2, 4, 6)
ORD = (1, 4, 2, 3, 0, 6, 5)
PAD = 0
XC = 1
B8 = 1
CP = 0
DL = -1
CO = 1
NP = 8
KM = 128
KG = 16

F32 = jnp.float32
BF16 = jnp.bfloat16
U32 = jnp.uint32
NT = (((1,), (1,)), ((), ()))
QUADS = ((0, 0), (0, 1), (1, 0), (1, 1))


def _dft_matrix():
    f0 = np.arange(M)[:, None]
    m = np.arange(M)[None, :]
    fwd = np.zeros((R, 2 * M, M), np.float64)
    for r in range(R):
        n = R * m + r
        ph = -np.pi * ((n * (1 + 4 * f0)) % (4 * C)) / (2 * C)
        re = np.cos(ph).reshape(M // 8, 8, M)
        im = np.sin(ph).reshape(M // 8, 8, M)
        fwd[r] = np.stack([re, im], 1).reshape(2 * M, M)
    return fwd.astype(np.float32)


def _pack(x):
    return pltpu.bitcast(x.astype(BF16), U32)


def _unpack(w):
    return pltpu.bitcast(w, BF16)


def _join_rows(even, odd):
    return pltpu.pack_elementwise([even, odd], packed_dtype=BF16)


def _split_rows(w):
    return [pltpu.unpack_elementwise(w, index=n, packed_dtype=BF16, unpacked_dtype=F32) for n in range(2)]


def _np_pack(x):
    bits = x.astype(BF16).view(np.uint16).astype(np.uint32)
    return bits[..., 0::2, :] | (bits[..., 1::2, :] << 16)


def _dot(a, b):
    return jnp.dot(a, b, preferred_element_type=F32)


def _dot_nt(a, b):
    return lax.dot_general(a, b, NT, preferred_element_type=F32)


def _gelu2(x):
    t = jnp.tanh(x * (x * x * GELU_C3 + GELU_C1))
    return x * t + x


def _ln_rows(x):
    n = x.shape[-1]
    d = x - jnp.sum(x, axis=-1, keepdims=True) * (1.0 / n)
    var = jnp.sum(d * d, axis=-1, keepdims=True) * (1.0 / n)
    return d * lax.rsqrt(var + EPS)


def _interleave(*streams):
    order = sorted(((n + (0.5 if k else 0.0)) / len(st), k, n)
                   for k, st in enumerate(streams) for n in range(len(st)))
    for _, k, n in order:
        streams[k][n]()


def _strassen_left(a11, a12, a21, a22):
    return (a11 + a22, a21 + a22, a11, a22, a11 + a12, a21 - a11, a12 - a22)


def _strassen_right(b11, b12, b21, b22):
    f11, f12, f21, f22 = (b.astype(F32) for b in (b11, b12, b21, b22))
    return [b.astype(BF16) for b in (f11 + f22, b11, f12 - f22, f21 - f11, b22, f11 + f12, f21 + f22)]


def _strassen(product, rest):
    m2, m4 = product(1), product(3)
    yield (1, 0), m2 + m4 + rest(1, 0)
    m5, m3 = product(4), product(2)
    yield (0, 1), m3 + m5 + rest(0, 1)
    m1, m7 = product(0), product(6)
    yield (0, 0), (m4 - m5) + m1 + m7 + rest(0, 0)
    yield (1, 1), (m3 - m2) + m1 + product(5) + rest(1, 1)


def _strassen_sum(products):
    m1, m2, m3, m4, m5, m6, m7 = products
    return (m4 - m5) + m1 + m7, m3 + m5, m2 + m4, (m3 - m2) + m1 + m6


def _butterfly(x, inverse):
    (r0, i0), (r1, i1), (r2, i2), (r3, i3) = x
    ar, ai, br, bi = r0 + r2, i0 + i2, r0 - r2, i0 - i2
    cr, ci, dr, di = r1 + r3, i1 + i3, r1 - r3, i1 - i3
    lo, hi = (br + di, bi - dr), (br - di, bi + dr)
    if inverse:
        lo, hi = hi, lo
    return [(ar + cr, ai + ci), lo, (ar - cr, ai - ci), hi]


def _forward(f_v, phases):
    es = []
    for r in range(R):
        e = _dot(_unpack(f_v[r]), phases[r].astype(BF16)).reshape(M // 8, 2, 8, LANES)
        es.append((e[:, 0], e[:, 1]))
    return _butterfly(es, inverse=False)


def _kernel(q_h, k_h, v_h, sk_h, g_h, sd_h, win_h, wsp_h, bsp_h, wout_h, c_h, wmod_h, f_h,
            out_h,
            q_v, k_v, v_v, sk_v, g_v, sd_v, win_v, wsp_v, bsp_v, wout_v, c_v, wmod_v, f_v, fi_v,
            gs_v, us_v, gt_v, kf_v, vf_v, y_v, x1_v, flag_v, row_v, tap_v, mod_v, h_v, w_v, acc_v, a2_v, mean_v, zs_v,
            wis_v, wos_v, p_v, pr_v, o_v, woutt_v, brow_v, out_v, sems):
    S, D = q_v.shape
    FH = wout_v.shape[0]
    NA, NJ = S // C, D // LANES
    KS = sk_v.shape[0]
    HS, HF, HD = S // 2, FH // 2, D // 2
    nb = S // (2 * T)

    n_sem = [nb]

    def fetch(src, dst):
        cp = pltpu.make_async_copy(src, dst, sems.at[n_sem[0]])
        n_sem[0] += 1
        cp.start()
        return cp

    def rows(ref, i, n):
        return ref.at[pl.ds(i * n, n)]

    def cols(ref, i, n):
        return ref.at[:, pl.ds(i * n, n)]

    def mix_cols(i):
        cs = pl.ds(pl.multiple_of(i * 2 * T, 2 * T), 2 * T)
        return pltpu.make_async_copy(wsp_h.at[:, cs], wsp_v.at[i], sems.at[i])

    cp_g = [fetch(cols(g_h, 0, C), cols(g_v, 0, C))]
    cp_small = [fetch(f_h, f_v), fetch(sd_h, sd_v), fetch(sk_h, sk_v), fetch(c_h, c_v)]
    cp_kv = []
    for n in range(1, NA + AHEAD):
        if n < NA:
            cp_g.append(fetch(cols(g_h, n, C), cols(g_v, n, C)))
        if n >= AHEAD:
            cp_kv.append([fetch(rows(src, n - AHEAD, C), rows(dst, n - AHEAD, C))
                          for src, dst in ((k_h, k_v), (v_h, v_v))])

    def q_block(i):
        return fetch(rows(q_h, i, 2 * T), rows(q_v, i, 2 * T))

    cp_q = [q_block(0)]
    cp_wmod = {0: fetch(cols(wmod_h, 0, 5 * D), cols(wmod_v, 0, 5 * D))}
    cp_win = {1: fetch(rows(win_h, 1, FH), rows(win_v, 1, FH))}
    cp_q += [q_block(1)]
    cp_rest = []

    def fetch_group(i):
        later = [n for n in SYNC if n > i]
        for n in range(i, (later + [nb + 1])[0]):
            if n + 1 < nb:
                cp_q.append(q_block(n + 1))
            mix_cols(n - 1).start()
        if not later:
            cp_wmod[5] = fetch(cols(wmod_h, 5, D), cols(wmod_v, 5, D))
            cp_win[0] = fetch(rows(win_h, 0, FH), rows(win_v, 0, FH))
            cp_rest.extend([fetch(bsp_h, bsp_v), fetch(wout_h, wout_v)])

    fetch_group(SYNC[0])
    flag_v[0] = 0

    @pl.loop(0, 2)
    def _(n):
        acc_v[n, 0:8] = jnp.zeros((8, T), F32)

    for cp in cp_small:
        cp.wait()
    sd_row = sd_v[...].astype(F32).reshape(1, D)
    sk = sk_v[...].astype(F32)
    tap_v[KS] = jnp.broadcast_to(sd_row, (8, D))
    for t in range(KS):
        tap_v[t] = jnp.broadcast_to(sk[t:t + 1] * (1.0 / C), (8, D))

    for r in range(R):
        fi_v[r] = _pack(_unpack(f_v[r]).T)

    raw = {}

    def transpose(a, j):
        gt_v[j] = g_v[j * LANES:(j + 1) * LANES, a * C:(a + 1) * C].T.astype(F32)

    def filter_spectrum(a, j):
        spec = _forward(f_v, [gt_v[j, pl.ds(r, M, stride=R), :] for r in range(R)])
        for qq in range(R):
            re, im = spec[qq]
            if a == 0:
                re = re + tap_v[KS, :, j * LANES:(j + 1) * LANES]
                spec[qq] = (re, im)
            else:
                re, im = re - raw[j][qq][1], im + raw[j][qq][0]
            gs_v[j, a, 2 * qq] = re
            gs_v[j, a, 2 * qq + 1] = im
        raw[j] = spec

    def widen(a, j):
        lanes = slice(j * LANES, (j + 1) * LANES)
        if a == 0:
            kf_v[j, 0:HIST, :] = jnp.zeros((HIST, LANES), F32)
            kf_v[j, HIST:, :] = k_v[0:C, lanes].astype(F32)
        else:
            kf_v[j] = k_v[a * C - HIST:(a + 1) * C, lanes].astype(F32)
        vf_v[j] = v_v[a * C:(a + 1) * C, lanes].astype(F32)

    def analyse(a, j):
        lanes = slice(j * LANES, (j + 1) * LANES)
        phases = [[] for _ in range(R)]
        for m0 in range(0, M, KM):
            kp = {s: kf_v[j, pl.ds(HIST + R * m0 + s, KM, stride=R), :] for s in range(1 - KS, R)}
            taps = [jnp.concatenate([tap_v[t, :, lanes]] * (KM // 8), axis=0) for t in range(KS)]
            for r in range(R):
                acc = kp[r] * taps[0]
                for t in range(1, KS):
                    acc = acc + kp[r - t] * taps[t]
                phases[r].append(acc * vf_v[j, pl.ds(R * m0 + r, KM, stride=R), :])
        spec = _forward(f_v, [jnp.concatenate(ph, axis=0) for ph in phases])
        for qq in range(R):
            us_v[j, a, 2 * qq], us_v[j, a, 2 * qq + 1] = spec[qq]

    def synthesise(a, j):
        packed = [[] for _ in range(R)]
        for g0 in range(0, M // 8, KG):
            gs = slice(g0, g0 + KG)
            ys = []
            for qq in range(R):
                yr = yi = None
                for b in range(a + 1):
                    ur, ui = us_v[j, a - b, 2 * qq, gs], us_v[j, a - b, 2 * qq + 1, gs]
                    gr, gi = gs_v[j, b, 2 * qq, gs], gs_v[j, b, 2 * qq + 1, gs]
                    tr, ti = gr * ur - gi * ui, gr * ui + gi * ur
                    yr, yi = (tr, ti) if b == 0 else (yr + tr, yi + ti)
                ys.append((yr, yi))
            for r, b in enumerate(_butterfly(ys, inverse=True)):
                packed[r].append(jnp.stack(b, axis=1).reshape(16 * KG, LANES).astype(BF16))
        for r in range(R):
            y_v[j, pl.ds(a * C + r, M, stride=R), :] = _dot(
                _unpack(fi_v[r]), jnp.concatenate(packed[r], axis=0))

    def modulation(n):
        cc = c_v[...].astype(F32)
        sc = jnp.broadcast_to(cc * jax.nn.sigmoid(cc), (16, D)).astype(BF16)
        return _dot(sc, wmod_v[:, n * D:(n + 1) * D])[0:8]

    def modulate():
        sa, ca, ga, sb, cb = (modulation(n) for n in range(5))
        mod_v[0] = ga * (1.0 + ca)
        mod_v[1] = ga * sa
        mod_v[2] = 1.0 + cb
        mod_v[3] = sb

    def scale(x, n):
        return (x.reshape(x.shape[0] // 8, 8, D) * mod_v[n]).reshape(x.shape)

    def shift(x, n):
        return (x.reshape(x.shape[0] // 8, 8, D) + mod_v[n]).reshape(x.shape)


    def halves(i, off=0, n=T):
        return [pl.ds(pl.multiple_of((2 * i + hh) * T + off, n), n) for hh in range(2)]

    def words(i, off=0, n=T):
        return [pl.ds(pl.multiple_of((2 * i + hh) * (T // 2) + off // 2, n // 2), n // 2) for hh in range(2)]

    last = []

    def paced(x, tiles=1):
        if not last:
            return x
        dep = last.pop()
        n = min(dep.shape[0], x.shape[0])
        dep = jnp.concatenate([dep[:n]] * (x.shape[0] // n), axis=0)
        cols = [x[:, c:c + LANES] for c in range(0, x.shape[1], LANES)]
        return jnp.concatenate([jnp.where(flag_v[0] > 0, dep, col) for col in cols[:tiles]] + cols[tiles:], axis=1)

    def delay(x):
        if DL < 0:
            return pltpu.roll(x, 1, 1)
        for _ in range(DL):
            x = jnp.tanh(x)
        return x

    def prepare(i):
        def piece(hh, off):
            rs = halves(i, off, PR)[hh]
            x = paced(q_v[rs, :].astype(F32))
            y = jnp.concatenate([y_v[j, rs, :] for j in range(NJ)], axis=1)
            x1 = x + shift(scale(_ln_rows(x), 0), 1) * y
            x1_v[rs, :] = x1
            h = shift(scale(_ln_rows(x1), 2), 3)
            h_v[words(i, off, PR)[hh], :] = _pack(h)
            last.append(h[:, -LANES:])

        return [functools.partial(piece, hh, off) for hh in range(2) for off in range(0, T, PR)]

    KI, KO = (NJ // 2) * LANES, (FH // (2 * LANES)) * LANES

    def project(i, fh):
        h1, h2 = (_unpack(h_v[hs, :]) for hs in words(i))
        right = _strassen_right(h1[:, :KI], h2[:, :KI], h1[:, KI:2 * KI], h2[:, KI:2 * KI])
        return _strassen(
            lambda n: _dot_nt(_unpack(wis_v[fh, n]), right[n]),
            lambda qh, hh: _dot_nt(_unpack(w_v[fh, qh, :, 2 * KI:]), (h1, h2)[hh][:, 2 * KI:]))

    def activate(i):
        tot = {}
        for (qh, hh), z in project(i, 1):
            a2 = _gelu2(z)
            a2_v[i % 2, hh, qh * HF:(qh + 1) * HF, :] = a2
            tot[hh] = tot.get(hh, 0.0) + jnp.sum(a2.reshape(HF // 8, 8, T), axis=0)
        for hh in range(2):
            mean = jnp.sum(tot[hh], axis=0, keepdims=True) * (1.0 / FH)
            mean_v[i % 2, :, hh * T:(hh + 1) * T] = jnp.broadcast_to(mean, (8, T))

    def normalize(i):
        state = {}

        def centred(rs, n, mean):
            a2 = jnp.concatenate([a2_v[i % 2, hh, rs, :] for hh in range(2)], axis=1)
            return a2.reshape(n // 8, 8, 2 * T) - mean

        def var_piece(r0):
            d = centred(pl.ds(r0, NR), NR, paced(mean_v[i % 2], 2))
            part = jnp.sum(d * d, axis=0)
            state["ss"] = part if r0 == 0 else state["ss"] + part
            last.append(delay(state["ss"][:, :LANES]))
            if r0 + NR == FH:
                var = jnp.sum(state["ss"], axis=0, keepdims=True) * (1.0 / FH)
                state["rstd"] = jnp.broadcast_to(lax.rsqrt(var + 4.0 * EPS), (8, 2 * T))

        def out_piece(r0):
            mean = paced(mean_v[i % 2], 2)
            parts = []
            for odd in range(2):
                za, zb = ((centred(pl.ds(r + odd, NO // 2, stride=2), NO // 2, mean) * state["rstd"]
                           ).reshape(NO // 2, 2 * T) for r in (r0, HF + r0))
                parts.append(jnp.concatenate(
                    _strassen_left(za[:, :T], za[:, T:], zb[:, :T], zb[:, T:]), axis=1))
            words = _join_rows(*parts)
            zs_v[i % 2, r0 // 2:(r0 + NO) // 2, :] = words
            last.append(delay(pltpu.bitcast(words[-8:, :T], F32)))

        return ([functools.partial(var_piece, r0) for r0 in range(0, FH, NR)]
                + [functools.partial(out_piece, r0) for r0 in range(0, HF, NO)])

    def mix(i):
        def block(k0, th, sh, n):
            return jnp.concatenate([wsp_v[i, (2 * k + th) * T:(2 * k + th + 1) * T, sh * T:(sh + 1) * T]
                                    for k in range(k0, k0 + TW)], axis=0)

        for k0 in range(0, nb, TW):
            for n in ORD:
                right = _strassen_right(*(block(k0, th, sh, n) for sh in range(2) for th in range(2)))[n]
                m = _dot_nt(_unpack(zs_v[i % 2, :, n * T:(n + 1) * T]), right)
                for k in range(TW):
                    at = (k0 + k, slice(n * HF, (n + 1) * HF))
                    part = m[:, k * T:(k + 1) * T]
                    acc_v[at] = acc_v[at] + part if i else part

    def step_b(i):
        if i in SYNC:
            upto = ([n for n in SYNC if n > i] + [nb + 1])[0]
            if upto <= nb:
                fetch_group(upto)
            for n in range(i, upto):
                mix_cols(n - 1).wait()
                if n + 1 < nb:
                    cp_q[n + 1].wait()
            if upto > nb:
                for cp in [cp_wmod[5], cp_win[0]] + cp_rest:
                    cp.wait()
        if i == 1:
            unpaced(normalize(0))
            last.clear()
        activate(i)
        mix(i - 1)
        side = prepare(i + 1) if i + 1 < nb else []
        if i == 1 or not XC:
            last.clear()
        _interleave(side + normalize(i))

    def unpaced(pieces):
        for piece in pieces:
            last.clear()
            piece()

    def split_left(dst, top, bottom, width):
        for r0 in range(0, top.shape[0], 8):
            blk = [_split_rows(src[r0:r0 + 8, k:k + width]) for src in (top, bottom) for k in (0, width)]
            even, odd = (_strassen_left(*(b[n] for b in blk)) for n in range(2))
            for n in range(7):
                dst[n, r0:r0 + 8, :] = _join_rows(even[n], odd[n])

    def load_w_in(fh):
        for qh in range(2):
            for dst, src, n in ((0, qh * KO, KO), (KO, 2 * KO + qh * (HF - KO), HF - KO)):
                w_v[fh, qh, dst // 2:(dst + n) // 2] = _pack(win_v[fh * FH + src:fh * FH + src + n, :])
        split_left(wis_v.at[fh], w_v.at[fh, 0], w_v.at[fh, 1], KI)

    tiles = [(a, j) for a in range(NA) for j in range(NJ)]
    lead = AHEAD * NJ
    stages = ((transpose, 0), (filter_spectrum, 1), (widen, lead), (analyse, lead + 1), (synthesise, lead + 2))
    for n in range(len(tiles) + lead + 2):
        if n % NJ == 0:
            if n < len(tiles):
                cp_g[n // NJ].wait()
            if 0 <= n - lead < len(tiles):
                for cp in cp_kv[(n - lead) // NJ]:
                    cp.wait()
        if n == len(tiles) + lead - MODAT:
            cp_q[0].wait()
            cp_wmod[0].wait()
            modulate()
            unpaced(prepare(0))
        for fn, lag in stages:
            if 0 <= n - lag < len(tiles) and 'A' in PH:
                fn(*tiles[n - lag])

    cp_win[1].wait()
    cp_q[1].wait()
    if 'C' in PH:
        load_w_in(1)
        activate(0)
        unpaced(prepare(1))
    if 'S' in PH:
        mix_cols(0).wait()
        cp_q[2].wait()
        _interleave(normalize(0))
        activate(1)
        pltpu.sync_copy(out_v.at[pl.ds(0, 8)], out_h.at[pl.ds(0, 8)])
        pltpu.sync_copy(zs_v.at[0, pl.ds(0, 8), pl.ds(0, 640)], h_v.at[pl.ds(0, 8)])
        return
    if 'B' in PH:
        for i in range(1, nb if 'C' in PH else 4):
            step_b(i)
    if 'C' not in PH:
        out_v[0:16, 0:128] = (x1_v[0:16, 0:128] + y_v[1, 0:16, :] + acc_v[1, 0:16, :]).astype(BF16) + _unpack(h_v[0:8, 0:128] + zs_v[0, 0:8, 0:128])
        pltpu.sync_copy(out_v, out_h)
        pltpu.sync_copy(zs_v.at[0, pl.ds(0, 8), pl.ds(0, 640)], h_v.at[pl.ds(0, 8)])
        return

    out_sem0 = n_sem[0]

    def out_copies(i):
        return [pltpu.make_async_copy(out_v.at[rs], out_h.at[rs], sems.at[out_sem0 + 2 * i + hh])
                for hh, rs in enumerate(halves(i))]

    def gate(i, slot, zs):
        gates = _strassen_sum([acc_v[i, n * HF:(n + 1) * HF] for n in range(7)])
        ps = [None] * 4
        for (qh, hh), z in zs:
            g = gates[2 * qh + hh]
            g = (g.reshape(HF // 8, 8, T) + brow_v[:, halves(i)[hh]]).reshape(HF, T)
            ps[2 * qh + hh] = _gelu2(z) * g
        for n, val in enumerate(_strassen_right(*(p[:KO] for p in ps))):
            p_v[slot, n] = val
        for hh in range(2):
            pr_v[slot, hh] = jnp.concatenate([ps[hh][KO:], ps[2 + hh][KO:]], axis=0).astype(BF16)

    def project_out(slot):
        for (dh, hh), o in _strassen(
                lambda n: _dot(_unpack(wos_v[n]), p_v[slot, n]),
                lambda dh, hh: _dot(_unpack(woutt_v[dh, :, 2 * KO:]), pr_v[slot, hh])):
            o_v[slot, hh, dh * HD:(dh + 1) * HD] = o

    def finish(i, slot):
        for hh, rs in enumerate(halves(i)):
            out_v[rs, :] = (x1_v[rs, :] + scale(o_v[slot, hh].T, 4)).astype(out_v.dtype)
        for cp in out_copies(i):
            cp.start()

    def step_c(i, slot, n_done):
        if n_done >= 2:
            finish(i - 2, slot)
        gate(i, slot, project(i, 0))
        project_out(1 - slot)

    def small_operands():
        brow_v[...] = jnp.broadcast_to(bsp_v[...].astype(F32).reshape(1, S), (8, S))
        mod_v[4] = 0.5 * modulation(5)

    def load_w_out():
        woutt = _pack(wout_v[...].T)
        for dh in range(2):
            woutt_v[dh] = woutt[dh * HD // 2:(dh + 1) * HD // 2]
        split_left(wos_v, woutt_v.at[0], woutt_v.at[1], KO)

    load_w_in(0)
    small_operands()
    if B8 == 0:
        mix(nb - 1)
        gate(0, 0, project(0, 0))
    elif B8 == 1:
        z_first = list(project(0, 0))
        mix(nb - 1)
        gate(0, 0, z_first)
    load_w_out()
    for i in range(1, nb):
        step_c(i, i % 2, i)
    project_out(1)
    finish(nb - 2, 0)
    finish(nb - 1, 1)
    for i in range(nb):
        for cp in out_copies(i):
            cp.wait()


@jax.jit
def pallas_adaLN_cond__ssm_conv_h3__mixer_gmlp__prompt_kernel(
    A_q: jax.Array,
    A_k: jax.Array,
    A_v: jax.Array,
    A_shift_k: jax.Array,
    A_ssm_k: jax.Array,
    A_ssm_D: jax.Array,
    B_x: jax.Array,
    B_w_in: jax.Array,
    B_w_sp: jax.Array,
    B_b_sp: jax.Array,
    B_w_out: jax.Array,
    c: jax.Array,
    w_mod: jax.Array,
):
    del B_x
    B, S, D = A_q.shape
    FH = B_w_out.shape[0]
    assert B == 1 and S % C == 0 and D % LANES == 0 and B_w_in.shape[1] == 2 * FH
    NA, NJ, NB = S // C, D // LANES, S // (2 * T)
    KO = (FH // (2 * LANES)) * LANES
    operands = (
        A_q.reshape(S, D), A_k.reshape(S, D), A_v.reshape(S, D), A_shift_k.T, A_ssm_k, A_ssm_D,
        B_w_in.T, B_w_sp, B_b_sp, B_w_out, c, w_mod,
        _np_pack(_dft_matrix()),
    )
    spectrum = (2 * R, M // 8, 8, LANES)
    scratch = [pltpu.VMEM((NB, S, 2 * T) if o is B_w_sp else o.shape, o.dtype) for o in operands] + [
        pltpu.VMEM((R, M // 2, 2 * M), U32),
        pltpu.VMEM((NJ, NA) + spectrum, F32),
        pltpu.VMEM((NJ, NA) + spectrum, F32),
        pltpu.VMEM((NJ, C, LANES), F32),
        pltpu.VMEM((NJ, HIST + C, LANES), F32),
        pltpu.VMEM((NJ, C, LANES), F32),
        pltpu.VMEM((NJ, S, LANES), F32),
        pltpu.VMEM((S, D), F32),
        pltpu.SMEM((1,), jnp.int32),
        pltpu.VMEM((16, D), F32),
        pltpu.VMEM((A_shift_k.shape[1] + 1, 8, D), F32),
        pltpu.VMEM((5, 8, D), F32),
        pltpu.VMEM((S // 2, D), U32),
        pltpu.VMEM((2, 2, FH // 4, D), U32),
        pltpu.VMEM((NB, 7 * FH // 2 + PAD, T), F32),
        pltpu.VMEM((2, 2, FH, T), F32),
        pltpu.VMEM((2, 8, 2 * T), F32),
        pltpu.VMEM((2, FH // 4, 7 * T), U32),
        pltpu.VMEM((2, 7, FH // 4, (NJ // 2) * LANES), U32),
        pltpu.VMEM((7, D // 4, (FH // (2 * LANES)) * LANES), U32),
        pltpu.VMEM((2, 7, KO, T), BF16),
        pltpu.VMEM((2, 2, FH - 2 * KO, T), BF16),
        pltpu.VMEM((2, 2, D, T), F32),
        pltpu.VMEM((2, D // 4, FH), U32),
        pltpu.VMEM((8, S), F32),
        pltpu.VMEM((S, D), A_q.dtype),
        pltpu.SemaphoreType.DMA((64,)),
    ]
    out = pl.pallas_call(
        _kernel,
        out_shape=jax.ShapeDtypeStruct((S, D), A_q.dtype),
        in_specs=[pl.BlockSpec(memory_space=pl.ANY)] * len(operands),
        out_specs=pl.BlockSpec(memory_space=pl.ANY),
        scratch_shapes=scratch,
        compiler_params=pltpu.CompilerParams(vmem_limit_bytes=124 * 2**20, flags=FLAGS),
    )(*operands)
    return out.reshape(B, S, D)
```

```python
import functools

import numpy as np

import jax
import jax.numpy as jnp
from jax import lax
import jax.experimental.pallas as pl
import jax.experimental.pallas.tpu as pltpu

LANES = 128
R = 4
M = 128
C = R * M
HIST = 16
EPS = 1e-5
GELU_C1 = float(np.sqrt(2.0 / np.pi))
GELU_C3 = float(np.sqrt(2.0 / np.pi) * 0.044715)
T = 128
PR = 32
MB = 288
NR = 288
NO = 16
FLAGS = None
PH = 'ABC'
AHEAD = 3
WAT = 4
MODAT = 1
J0 = 2
KVW = {0: (0,), 5: (1,), 10: (2,), 15: (3,)}
TW = 4
SYNC = (1, 2, 4, 6)
ORD = (1, 4, 2, 3, 0, 6, 5)
PAD = 0
XC = 1
B8 = 1
CP = 0
DL = -1
CO = 1
NP = 8
KM = 128
KG = 16

F32 = jnp.float32
BF16 = jnp.bfloat16
U32 = jnp.uint32
NT = (((1,), (1,)), ((), ()))
QUADS = ((0, 0), (0, 1), (1, 0), (1, 1))


def _dft_matrix():
    f0 = np.arange(M)[:, None]
    m = np.arange(M)[None, :]
    fwd = np.zeros((R, 2 * M, M), np.float64)
    for r in range(R):
        n = R * m + r
        ph = -np.pi * ((n * (1 + 4 * f0)) % (4 * C)) / (2 * C)
        re = np.cos(ph).reshape(M // 8, 8, M)
        im = np.sin(ph).reshape(M // 8, 8, M)
        fwd[r] = np.stack([re, im], 1).reshape(2 * M, M)
    return fwd.astype(np.float32)


def _pack(x):
    return pltpu.bitcast(x.astype(BF16), U32)


def _unpack(w):
    return pltpu.bitcast(w, BF16)


def _join_rows(even, odd):
    return pltpu.pack_elementwise([even, odd], packed_dtype=BF16)


def _split_rows(w):
    return [pltpu.unpack_elementwise(w, index=n, packed_dtype=BF16, unpacked_dtype=F32) for n in range(2)]


def _np_pack(x):
    bits = x.astype(BF16).view(np.uint16).astype(np.uint32)
    return bits[..., 0::2, :] | (bits[..., 1::2, :] << 16)


def _dot(a, b):
    return jnp.dot(a, b, preferred_element_type=F32)


def _dot_nt(a, b):
    return lax.dot_general(a, b, NT, preferred_element_type=F32)


def _gelu2(x):
    t = jnp.tanh(x * (x * x * GELU_C3 + GELU_C1))
    return x * t + x


def _ln_rows(x):
    n = x.shape[-1]
    d = x - jnp.sum(x, axis=-1, keepdims=True) * (1.0 / n)
    var = jnp.sum(d * d, axis=-1, keepdims=True) * (1.0 / n)
    return d * lax.rsqrt(var + EPS)


def _interleave(*streams):
    order = sorted(((n + (0.5 if k else 0.0)) / len(st), k, n)
                   for k, st in enumerate(streams) for n in range(len(st)))
    for _, k, n in order:
        streams[k][n]()


def _strassen_left(a11, a12, a21, a22):
    return (a11 + a22, a21 + a22, a11, a22, a11 + a12, a21 - a11, a12 - a22)


def _strassen_right(b11, b12, b21, b22):
    f11, f12, f21, f22 = (b.astype(F32) for b in (b11, b12, b21, b22))
    return [b.astype(BF16) for b in (f11 + f22, b11, f12 - f22, f21 - f11, b22, f11 + f12, f21 + f22)]


def _strassen(product, rest):
    m2, m4 = product(1), product(3)
    yield (1, 0), m2 + m4 + rest(1, 0)
    m5, m3 = product(4), product(2)
    yield (0, 1), m3 + m5 + rest(0, 1)
    m1, m7 = product(0), product(6)
    yield (0, 0), (m4 - m5) + m1 + m7 + rest(0, 0)
    yield (1, 1), (m3 - m2) + m1 + product(5) + rest(1, 1)


def _strassen_sum(products):
    m1, m2, m3, m4, m5, m6, m7 = products
    return (m4 - m5) + m1 + m7, m3 + m5, m2 + m4, (m3 - m2) + m1 + m6


def _butterfly(x, inverse):
    (r0, i0), (r1, i1), (r2, i2), (r3, i3) = x
    ar, ai, br, bi = r0 + r2, i0 + i2, r0 - r2, i0 - i2
    cr, ci, dr, di = r1 + r3, i1 + i3, r1 - r3, i1 - i3
    lo, hi = (br + di, bi - dr), (br - di, bi + dr)
    if inverse:
        lo, hi = hi, lo
    return [(ar + cr, ai + ci), lo, (ar - cr, ai - ci), hi]


def _forward(f_v, phases):
    es = []
    for r in range(R):
        e = _dot(_unpack(f_v[r]), phases[r].astype(BF16)).reshape(M // 8, 2, 8, LANES)
        es.append((e[:, 0], e[:, 1]))
    return _butterfly(es, inverse=False)


def _kernel(q_h, k_h, v_h, sk_h, g_h, sd_h, win_h, wsp_h, bsp_h, wout_h, c_h, wmod_h, f_h,
            out_h,
            q_v, k_v, v_v, sk_v, g_v, sd_v, win_v, wsp_v, bsp_v, wout_v, c_v, wmod_v, f_v, fi_v,
            gs_v, us_v, gt_v, kf_v, vf_v, y_v, x1_v, flag_v, row_v, tap_v, mod_v, h_v, w_v, acc_v, a2_v, mean_v, zs_v,
            wis_v, wos_v, p_v, pr_v, o_v, woutt_v, brow_v, out_v, sems):
    S, D = q_v.shape
    FH = wout_v.shape[0]
    NA, NJ = S // C, D // LANES
    KS = sk_v.shape[0]
    HS, HF, HD = S // 2, FH // 2, D // 2
    nb = S // (2 * T)

    n_sem = [nb]

    def fetch(src, dst):
        cp = pltpu.make_async_copy(src, dst, sems.at[n_sem[0]])
        n_sem[0] += 1
        cp.start()
        return cp

    def rows(ref, i, n):
        return ref.at[pl.ds(i * n, n)]

    def cols(ref, i, n):
        return ref.at[:, pl.ds(i * n, n)]

    def mix_cols(i):
        cs = pl.ds(pl.multiple_of(i * 2 * T, 2 * T), 2 * T)
        return pltpu.make_async_copy(wsp_h.at[:, cs], wsp_v.at[i], sems.at[i])

    cp_g = [fetch(cols(g_h, 0, C), cols(g_v, 0, C))]
    cp_small = [fetch(f_h, f_v), fetch(sd_h, sd_v), fetch(sk_h, sk_v), fetch(c_h, c_v)]
    cp_kv = {}
    for n in range(1, NA + AHEAD):
        if n < NA:
            cp_g.append(fetch(cols(g_h, n, C), cols(g_v, n, C)))
        if n >= AHEAD:
            a = n - AHEAD
            for j0, j1 in ((0, J0), (J0, NJ)) if a == 0 else ((0, NJ),):
                at = (pl.ds(a * C, C), pl.ds(j0 * LANES, (j1 - j0) * LANES))
                cp_kv[a * NJ + j0] = [fetch(src.at[at], dst.at[at]) for src, dst in ((k_h, k_v), (v_h, v_v))]

    def q_block(i):
        return fetch(rows(q_h, i, 2 * T), rows(q_v, i, 2 * T))

    cp_q = [q_block(0)]
    cp_wmod = {0: fetch(cols(wmod_h, 0, 5 * D), cols(wmod_v, 0, 5 * D))}
    cp_win = {1: fetch(rows(win_h, 1, FH), rows(win_v, 1, FH))}
    cp_q += [q_block(1)]
    cp_rest = []

    def fetch_group(i):
        later = [n for n in SYNC if n > i]
        for n in range(i, (later + [nb + 1])[0]):
            if n + 1 < nb:
                cp_q.append(q_block(n + 1))
            mix_cols(n - 1).start()
        if not later:
            cp_wmod[5] = fetch(cols(wmod_h, 5, D), cols(wmod_v, 5, D))
            cp_win[0] = fetch(rows(win_h, 0, FH), rows(win_v, 0, FH))
            cp_rest.extend([fetch(bsp_h, bsp_v), fetch(wout_h, wout_v)])

    fetch_group(SYNC[0])
    flag_v[0] = 0

    @pl.loop(0, 2)
    def _(n):
        acc_v[n, 0:8] = jnp.zeros((8, T), F32)

    for cp in cp_small:
        cp.wait()
    sd_row = sd_v[...].astype(F32).reshape(1, D)
    sk = sk_v[...].astype(F32)
    tap_v[KS] = jnp.broadcast_to(sd_row, (8, D))
    for t in range(KS):
        tap_v[t] = jnp.broadcast_to(sk[t:t + 1] * (1.0 / C), (8, D))

    for r in range(R):
        fi_v[r] = _pack(_unpack(f_v[r]).T)

    raw = {}

    def transpose(a, j):
        gt_v[j] = g_v[j * LANES:(j + 1) * LANES, a * C:(a + 1) * C].T.astype(F32)

    def filter_spectrum(a, j):
        spec = _forward(f_v, [gt_v[j, pl.ds(r, M, stride=R), :] for r in range(R)])
        for qq in range(R):
            re, im = spec[qq]
            if a == 0:
                re = re + tap_v[KS, :, j * LANES:(j + 1) * LANES]
                spec[qq] = (re, im)
            else:
                re, im = re - raw[j][qq][1], im + raw[j][qq][0]
            gs_v[j, a, 2 * qq] = re
            gs_v[j, a, 2 * qq + 1] = im
        raw[j] = spec

    def widen(a, j):
        lanes = slice(j * LANES, (j + 1) * LANES)
        if a == 0:
            kf_v[j, 0:HIST, :] = jnp.zeros((HIST, LANES), F32)
            kf_v[j, HIST:, :] = k_v[0:C, lanes].astype(F32)
        else:
            kf_v[j] = k_v[a * C - HIST:(a + 1) * C, lanes].astype(F32)
        vf_v[j] = v_v[a * C:(a + 1) * C, lanes].astype(F32)

    def analyse(a, j):
        lanes = slice(j * LANES, (j + 1) * LANES)
        phases = [[] for _ in range(R)]
        for m0 in range(0, M, KM):
            kp = {s: kf_v[j, pl.ds(HIST + R * m0 + s, KM, stride=R), :] for s in range(1 - KS, R)}
            taps = [jnp.concatenate([tap_v[t, :, lanes]] * (KM // 8), axis=0) for t in range(KS)]
            for r in range(R):
                acc = kp[r] * taps[0]
                for t in range(1, KS):
                    acc = acc + kp[r - t] * taps[t]
                phases[r].append(acc * vf_v[j, pl.ds(R * m0 + r, KM, stride=R), :])
        spec = _forward(f_v, [jnp.concatenate(ph, axis=0) for ph in phases])
        for qq in range(R):
            us_v[j, a, 2 * qq], us_v[j, a, 2 * qq + 1] = spec[qq]

    def synthesise(a, j):
        packed = [[] for _ in range(R)]
        for g0 in range(0, M // 8, KG):
            gs = slice(g0, g0 + KG)
            ys = []
            for qq in range(R):
                yr = yi = None
                for b in range(a + 1):
                    ur, ui = us_v[j, a - b, 2 * qq, gs], us_v[j, a - b, 2 * qq + 1, gs]
                    gr, gi = gs_v[j, b, 2 * qq, gs], gs_v[j, b, 2 * qq + 1, gs]
                    tr, ti = gr * ur - gi * ui, gr * ui + gi * ur
                    yr, yi = (tr, ti) if b == 0 else (yr + tr, yi + ti)
                ys.append((yr, yi))
            for r, b in enumerate(_butterfly(ys, inverse=True)):
                packed[r].append(jnp.stack(b, axis=1).reshape(16 * KG, LANES).astype(BF16))
        for r in range(R):
            y_v[j, pl.ds(a * C + r, M, stride=R), :] = _dot(
                _unpack(fi_v[r]), jnp.concatenate(packed[r], axis=0))

    def modulation(n):
        cc = c_v[...].astype(F32)
        sc = jnp.broadcast_to(cc * jax.nn.sigmoid(cc), (16, D)).astype(BF16)
        return _dot(sc, wmod_v[:, n * D:(n + 1) * D])[0:8]

    def modulate():
        sa, ca, ga, sb, cb = (modulation(n) for n in range(5))
        mod_v[0] = ga * (1.0 + ca)
        mod_v[1] = ga * sa
        mod_v[2] = 1.0 + cb
        mod_v[3] = sb

    def scale(x, n):
        return (x.reshape(x.shape[0] // 8, 8, D) * mod_v[n]).reshape(x.shape)

    def shift(x, n):
        return (x.reshape(x.shape[0] // 8, 8, D) + mod_v[n]).reshape(x.shape)


    def halves(i, off=0, n=T):
        return [pl.ds(pl.multiple_of((2 * i + hh) * T + off, n), n) for hh in range(2)]

    def words(i, off=0, n=T):
        return [pl.ds(pl.multiple_of((2 * i + hh) * (T // 2) + off // 2, n // 2), n // 2) for hh in range(2)]

    last = []

    def paced(x, tiles=1):
        if not last:
            return x
        dep = last.pop()
        n = min(dep.shape[0], x.shape[0])
        dep = jnp.concatenate([dep[:n]] * (x.shape[0] // n), axis=0)
        cols = [x[:, c:c + LANES] for c in range(0, x.shape[1], LANES)]
        return jnp.concatenate([jnp.where(flag_v[0] > 0, dep, col) for col in cols[:tiles]] + cols[tiles:], axis=1)

    def delay(x):
        if DL < 0:
            return pltpu.roll(x, 1, 1)
        for _ in range(DL):
            x = jnp.tanh(x)
        return x

    def prepare(i):
        def piece(hh, off):
            rs = halves(i, off, PR)[hh]
            x = paced(q_v[rs, :].astype(F32))
            y = jnp.concatenate([y_v[j, rs, :] for j in range(NJ)], axis=1)
            x1 = x + shift(scale(_ln_rows(x), 0), 1) * y
            x1_v[rs, :] = x1
            h = shift(scale(_ln_rows(x1), 2), 3)
            h_v[words(i, off, PR)[hh], :] = _pack(h)
            last.append(h[:, -LANES:])

        return [functools.partial(piece, hh, off) for hh in range(2) for off in range(0, T, PR)]

    KI, KO = (NJ // 2) * LANES, (FH // (2 * LANES)) * LANES

    def project(i, fh):
        h1, h2 = (_unpack(h_v[hs, :]) for hs in words(i))
        right = _strassen_right(h1[:, :KI], h2[:, :KI], h1[:, KI:2 * KI], h2[:, KI:2 * KI])
        return _strassen(
            lambda n: _dot_nt(_unpack(wis_v[fh, n]), right[n]),
            lambda qh, hh: _dot_nt(_unpack(w_v[fh, qh, :, 2 * KI:]), (h1, h2)[hh][:, 2 * KI:]))

    def activate(i):
        tot = {}
        for (qh, hh), z in project(i, 1):
            a2 = _gelu2(z)
            a2_v[i % 2, hh, qh * HF:(qh + 1) * HF, :] = a2
            tot[hh] = tot.get(hh, 0.0) + jnp.sum(a2.reshape(HF // 8, 8, T), axis=0)
        for hh in range(2):
            mean = jnp.sum(tot[hh], axis=0, keepdims=True) * (1.0 / FH)
            mean_v[i % 2, :, hh * T:(hh + 1) * T] = jnp.broadcast_to(mean, (8, T))

    def normalize(i):
        state = {}

        def centred(rs, n, mean):
            a2 = jnp.concatenate([a2_v[i % 2, hh, rs, :] for hh in range(2)], axis=1)
            return a2.reshape(n // 8, 8, 2 * T) - mean

        def var_piece(r0):
            d = centred(pl.ds(r0, NR), NR, paced(mean_v[i % 2], 2))
            part = jnp.sum(d * d, axis=0)
            state["ss"] = part if r0 == 0 else state["ss"] + part
            last.append(delay(state["ss"][:, :LANES]))
            if r0 + NR == FH:
                var = jnp.sum(state["ss"], axis=0, keepdims=True) * (1.0 / FH)
                state["rstd"] = jnp.broadcast_to(lax.rsqrt(var + 4.0 * EPS), (8, 2 * T))

        def out_piece(r0):
            mean = paced(mean_v[i % 2], 2)
            parts = []
            for odd in range(2):
                za, zb = ((centred(pl.ds(r + odd, NO // 2, stride=2), NO // 2, mean) * state["rstd"]
                           ).reshape(NO // 2, 2 * T) for r in (r0, HF + r0))
                parts.append(jnp.concatenate(
                    _strassen_left(za[:, :T], za[:, T:], zb[:, :T], zb[:, T:]), axis=1))
            words = _join_rows(*parts)
            zs_v[i % 2, r0 // 2:(r0 + NO) // 2, :] = words
            last.append(delay(pltpu.bitcast(words[-8:, :T], F32)))

        return ([functools.partial(var_piece, r0) for r0 in range(0, FH, NR)]
                + [functools.partial(out_piece, r0) for r0 in range(0, HF, NO)])

    def mix(i):
        def block(k0, th, sh, n):
            return jnp.concatenate([wsp_v[i, (2 * k + th) * T:(2 * k + th + 1) * T, sh * T:(sh + 1) * T]
                                    for k in range(k0, k0 + TW)], axis=0)

        for k0 in range(0, nb, TW):
            for n in ORD:
                right = _strassen_right(*(block(k0, th, sh, n) for sh in range(2) for th in range(2)))[n]
                m = _dot_nt(_unpack(zs_v[i % 2, :, n * T:(n + 1) * T]), right)
                for k in range(TW):
                    at = (k0 + k, slice(n * HF, (n + 1) * HF))
                    part = m[:, k * T:(k + 1) * T]
                    acc_v[at] = acc_v[at] + part if i else part

    def step_b(i):
        if i in SYNC:
            upto = ([n for n in SYNC if n > i] + [nb + 1])[0]
            if upto <= nb:
                fetch_group(upto)
            for n in range(i, upto):
                mix_cols(n - 1).wait()
                if n + 1 < nb:
                    cp_q[n + 1].wait()
            if upto > nb:
                for cp in [cp_wmod[5], cp_win[0]] + cp_rest:
                    cp.wait()
        if i == 1:
            unpaced(normalize(0))
            last.clear()
        activate(i)
        mix(i - 1)
        side = prepare(i + 1) if i + 1 < nb else []
        if i == 1 or not XC:
            last.clear()
        _interleave(side + normalize(i))

    def unpaced(pieces):
        for piece in pieces:
            last.clear()
            piece()

    def split_left(dst, top, bottom, width):
        for r0 in range(0, top.shape[0], 8):
            blk = [_split_rows(src[r0:r0 + 8, k:k + width]) for src in (top, bottom) for k in (0, width)]
            even, odd = (_strassen_left(*(b[n] for b in blk)) for n in range(2))
            for n in range(7):
                dst[n, r0:r0 + 8, :] = _join_rows(even[n], odd[n])

    def load_w_in(fh):
        for qh in range(2):
            for dst, src, n in ((0, qh * KO, KO), (KO, 2 * KO + qh * (HF - KO), HF - KO)):
                w_v[fh, qh, dst // 2:(dst + n) // 2] = _pack(win_v[fh * FH + src:fh * FH + src + n, :])
        split_left(wis_v.at[fh], w_v.at[fh, 0], w_v.at[fh, 1], KI)

    tiles = [(a, j) for a in range(NA) for j in range(NJ)]
    lead = AHEAD * NJ
    stages = ((transpose, 0), (filter_spectrum, 1), (widen, lead), (analyse, lead + 1), (synthesise, lead + 2))
    def await_inputs(n):
        todo = []
        if n % NJ == 0 and n < len(tiles):
            todo += [cp_g[n // NJ]]
        todo += cp_kv.get(n - lead, [])
        if n == len(tiles) + lead + MODAT:
            todo += [cp_q[0], cp_wmod[0]]
        if todo:
            for cp in todo:
                cp.wait()

    await_inputs(0)
    for n in range(len(tiles) + lead + 2):
        if n == len(tiles) + lead + MODAT:
            modulate()
            unpaced(prepare(0))
        for k, (fn, lag) in enumerate(stages):
            if k == WAT:
                await_inputs(n + 1)
            if 0 <= n - lag < len(tiles):
                fn(*tiles[n - lag])
        if WAT == len(stages):
            await_inputs(n + 1)

    cp_win[1].wait()
    cp_q[1].wait()
    load_w_in(1)
    activate(0)
    unpaced(prepare(1))
    if 'S' in PH:
        mix_cols(0).wait()
        cp_q[2].wait()
        _interleave(normalize(0))
        activate(1)
        pltpu.sync_copy(out_v.at[pl.ds(0, 8)], out_h.at[pl.ds(0, 8)])
        pltpu.sync_copy(zs_v.at[0, pl.ds(0, 8), pl.ds(0, 640)], h_v.at[pl.ds(0, 8)])
        return
    if 'B' in PH:
        for i in range(1, nb if 'F' not in PH else 4):
            step_b(i)
    if 'F' in PH:
        out_v[0:16, 0:128] = (x1_v[0:16, 0:128] + y_v[1, 0:16, :] + acc_v[1, 0:16, :]).astype(BF16) + _unpack(h_v[0:8, 0:128] + zs_v[0, 0:8, 0:128])
        pltpu.sync_copy(out_v, out_h)
        pltpu.sync_copy(zs_v.at[0, pl.ds(0, 8), pl.ds(0, 640)], h_v.at[pl.ds(0, 8)])
        return

    out_sem0 = n_sem[0]

    def out_copy(i, hh):
        rs = halves(i)[hh]
        return pltpu.make_async_copy(out_v.at[rs], out_h.at[rs], sems.at[out_sem0 + 2 * i + hh])

    def gate(i, slot, zs):
        gates = _strassen_sum([acc_v[i, n * HF:(n + 1) * HF] for n in range(7)])
        ps = [None] * 4
        for (qh, hh), z in zs:
            g = gates[2 * qh + hh]
            g = (g.reshape(HF // 8, 8, T) + brow_v[:, halves(i)[hh]]).reshape(HF, T)
            ps[2 * qh + hh] = _gelu2(z) * g
        for n, val in enumerate(_strassen_right(*(p[:KO] for p in ps))):
            p_v[slot, n] = val
        for hh in range(2):
            pr_v[slot, hh] = jnp.concatenate([ps[hh][KO:], ps[2 + hh][KO:]], axis=0).astype(BF16)

    def project_out(slot):
        for (dh, hh), o in _strassen(
                lambda n: _dot(_unpack(wos_v[n]), p_v[slot, n]),
                lambda dh, hh: _dot(_unpack(woutt_v[dh, :, 2 * KO:]), pr_v[slot, hh])):
            o_v[slot, hh, dh * HD:(dh + 1) * HD] = o

    def finish(i, slot):
        for hh, rs in enumerate(halves(i)):
            out_v[rs, :] = (x1_v[rs, :] + scale(o_v[slot, hh].T, 4)).astype(out_v.dtype)
            out_copy(i, hh).start()

    def step_c(i, slot, n_done):
        if n_done >= 2:
            finish(i - 2, slot)
        gate(i, slot, project(i, 0))
        project_out(1 - slot)

    def small_operands():
        brow_v[...] = jnp.broadcast_to(bsp_v[...].astype(F32).reshape(1, S), (8, S))
        mod_v[4] = 0.5 * modulation(5)

    def load_w_out():
        woutt = _pack(wout_v[...].T)
        for dh in range(2):
            woutt_v[dh] = woutt[dh * HD // 2:(dh + 1) * HD // 2]
        split_left(wos_v, woutt_v.at[0], woutt_v.at[1], KO)

    load_w_in(0)
    small_operands()
    if B8 == 0:
        mix(nb - 1)
        gate(0, 0, project(0, 0))
    elif B8 == 1:
        z_first = list(project(0, 0))
        mix(nb - 1)
        gate(0, 0, z_first)
    load_w_out()
    for i in range(1, nb):
        step_c(i, i % 2, i)
    project_out(1)
    finish(nb - 2, 0)
    finish(nb - 1, 1)
    for i in range(nb):
        for hh in range(2):
            out_copy(i, hh).wait()


@jax.jit
def pallas_adaLN_cond__ssm_conv_h3__mixer_gmlp__prompt_kernel(
    A_q: jax.Array,
    A_k: jax.Array,
    A_v: jax.Array,
    A_shift_k: jax.Array,
    A_ssm_k: jax.Array,
    A_ssm_D: jax.Array,
    B_x: jax.Array,
    B_w_in: jax.Array,
    B_w_sp: jax.Array,
    B_b_sp: jax.Array,
    B_w_out: jax.Array,
    c: jax.Array,
    w_mod: jax.Array,
):
    del B_x
    B, S, D = A_q.shape
    FH = B_w_out.shape[0]
    assert B == 1 and S % C == 0 and D % LANES == 0 and B_w_in.shape[1] == 2 * FH
    NA, NJ, NB = S // C, D // LANES, S // (2 * T)
    KO = (FH // (2 * LANES)) * LANES
    operands = (
        A_q.reshape(S, D), A_k.reshape(S, D), A_v.reshape(S, D), A_shift_k.T, A_ssm_k, A_ssm_D,
        B_w_in.T, B_w_sp, B_b_sp, B_w_out, c, w_mod,
        _np_pack(_dft_matrix()),
    )
    spectrum = (2 * R, M // 8, 8, LANES)
    scratch = [pltpu.VMEM((NB, S, 2 * T) if o is B_w_sp else o.shape, o.dtype) for o in operands] + [
        pltpu.VMEM((R, M // 2, 2 * M), U32),
        pltpu.VMEM((NJ, NA) + spectrum, F32),
        pltpu.VMEM((NJ, NA) + spectrum, F32),
        pltpu.VMEM((NJ, C, LANES), F32),
        pltpu.VMEM((NJ, HIST + C, LANES), F32),
        pltpu.VMEM((NJ, C, LANES), F32),
        pltpu.VMEM((NJ, S, LANES), F32),
        pltpu.VMEM((S, D), F32),
        pltpu.SMEM((1,), jnp.int32),
        pltpu.VMEM((16, D), F32),
        pltpu.VMEM((A_shift_k.shape[1] + 1, 8, D), F32),
        pltpu.VMEM((5, 8, D), F32),
        pltpu.VMEM((S // 2, D), U32),
        pltpu.VMEM((2, 2, FH // 4, D), U32),
        pltpu.VMEM((NB, 7 * FH // 2 + PAD, T), F32),
        pltpu.VMEM((2, 2, FH, T), F32),
        pltpu.VMEM((2, 8, 2 * T), F32),
        pltpu.VMEM((2, FH // 4, 7 * T), U32),
        pltpu.VMEM((2, 7, FH // 4, (NJ // 2) * LANES), U32),
        pltpu.VMEM((7, D // 4, (FH // (2 * LANES)) * LANES), U32),
        pltpu.VMEM((2, 7, KO, T), BF16),
        pltpu.VMEM((2, 2, FH - 2 * KO, T), BF16),
        pltpu.VMEM((2, 2, D, T), F32),
        pltpu.VMEM((2, D // 4, FH), U32),
        pltpu.VMEM((8, S), F32),
        pltpu.VMEM((S, D), A_q.dtype),
        pltpu.SemaphoreType.DMA((96,)),
    ]
    out = pl.pallas_call(
        _kernel,
        out_shape=jax.ShapeDtypeStruct((S, D), A_q.dtype),
        in_specs=[pl.BlockSpec(memory_space=pl.ANY)] * len(operands),
        out_specs=pl.BlockSpec(memory_space=pl.ANY),
        scratch_shapes=scratch,
        compiler_params=pltpu.CompilerParams(vmem_limit_bytes=124 * 2**20, flags=FLAGS),
    )(*operands)
    return out.reshape(B, S, D)
```

```python
import functools

import numpy as np

import jax
import jax.numpy as jnp
from jax import lax
import jax.experimental.pallas as pl
import jax.experimental.pallas.tpu as pltpu

LANES = 128
R = 4
M = 128
C = R * M
HIST = 16
EPS = 1e-5
GELU_C1 = float(np.sqrt(2.0 / np.pi))
GELU_C3 = float(np.sqrt(2.0 / np.pi) * 0.044715)
T = 128
PR = 32
MB = 288
NR = 288
NO = 16
FLAGS = None
PH = 'ABC'
AHEAD = 3
WAT = 4
MODAT = 1
J0 = 2
KVW = {0: (0,), 5: (1,), 10: (2,), 15: (3,)}
TW = 4
SYNC = (1, 2, 4, 6)
ORD = (1, 4, 2, 3, 0, 6, 5)
PAD = 0
PW = 0
XAT = (0, 1, 2, 3)
B8 = 1
CP = 0
DL = -1
CO = 1
NP = 8
KM = 128
KG = 16

F32 = jnp.float32
BF16 = jnp.bfloat16
U32 = jnp.uint32
NT = (((1,), (1,)), ((), ()))
QUADS = ((0, 0), (0, 1), (1, 0), (1, 1))


def _dft_matrix():
    f0 = np.arange(M)[:, None]
    m = np.arange(M)[None, :]
    fwd = np.zeros((R, 2 * M, M), np.float64)
    for r in range(R):
        n = R * m + r
        ph = -np.pi * ((n * (1 + 4 * f0)) % (4 * C)) / (2 * C)
        re = np.cos(ph).reshape(M // 8, 8, M)
        im = np.sin(ph).reshape(M // 8, 8, M)
        fwd[r] = np.stack([re, im], 1).reshape(2 * M, M)
    return fwd.astype(np.float32)


def _pack(x):
    return pltpu.bitcast(x.astype(BF16), U32)


def _unpack(w):
    return pltpu.bitcast(w, BF16)


def _join_rows(even, odd):
    return pltpu.pack_elementwise([even, odd], packed_dtype=BF16)


def _split_rows(w):
    return [pltpu.unpack_elementwise(w, index=n, packed_dtype=BF16, unpacked_dtype=F32) for n in range(2)]


def _np_pack(x):
    bits = x.astype(BF16).view(np.uint16).astype(np.uint32)
    return bits[..., 0::2, :] | (bits[..., 1::2, :] << 16)


def _dot(a, b):
    return jnp.dot(a, b, preferred_element_type=F32)


def _dot_nt(a, b):
    return lax.dot_general(a, b, NT, preferred_element_type=F32)


def _gelu2(x):
    t = jnp.tanh(x * (x * x * GELU_C3 + GELU_C1))
    return x * t + x


def _ln_rows(x):
    n = x.shape[-1]
    d = x - jnp.sum(x, axis=-1, keepdims=True) * (1.0 / n)
    var = jnp.sum(d * d, axis=-1, keepdims=True) * (1.0 / n)
    return d * lax.rsqrt(var + EPS)


def _interleave(*streams):
    order = sorted(((n + (0.5 if k else 0.0)) / len(st), k, n)
                   for k, st in enumerate(streams) for n in range(len(st)))
    for _, k, n in order:
        streams[k][n]()


def _strassen_left(a11, a12, a21, a22):
    return (a11 + a22, a21 + a22, a11, a22, a11 + a12, a21 - a11, a12 - a22)


def _strassen_right(b11, b12, b21, b22):
    f11, f12, f21, f22 = (b.astype(F32) for b in (b11, b12, b21, b22))
    return [b.astype(BF16) for b in (f11 + f22, b11, f12 - f22, f21 - f11, b22, f11 + f12, f21 + f22)]


def _strassen(product, rest):
    m2, m4 = product(1), product(3)
    yield (1, 0), m2 + m4 + rest(1, 0)
    m5, m3 = product(4), product(2)
    yield (0, 1), m3 + m5 + rest(0, 1)
    m1, m7 = product(0), product(6)
    yield (0, 0), (m4 - m5) + m1 + m7 + rest(0, 0)
    yield (1, 1), (m3 - m2) + m1 + product(5) + rest(1, 1)


def _strassen_sum(products):
    m1, m2, m3, m4, m5, m6, m7 = products
    return (m4 - m5) + m1 + m7, m3 + m5, m2 + m4, (m3 - m2) + m1 + m6


def _butterfly(x, inverse):
    (r0, i0), (r1, i1), (r2, i2), (r3, i3) = x
    ar, ai, br, bi = r0 + r2, i0 + i2, r0 - r2, i0 - i2
    cr, ci, dr, di = r1 + r3, i1 + i3, r1 - r3, i1 - i3
    lo, hi = (br + di, bi - dr), (br - di, bi + dr)
    if inverse:
        lo, hi = hi, lo
    return [(ar + cr, ai + ci), lo, (ar - cr, ai - ci), hi]


def _forward(f_v, phases):
    es = []
    for r in range(R):
        e = _dot(_unpack(f_v[r]), phases[r].astype(BF16)).reshape(M // 8, 2, 8, LANES)
        es.append((e[:, 0], e[:, 1]))
    return _butterfly(es, inverse=False)


def _kernel(q_h, k_h, v_h, sk_h, g_h, sd_h, win_h, wsp_h, bsp_h, wout_h, c_h, wmod_h, f_h,
            out_h,
            q_v, k_v, v_v, sk_v, g_v, sd_v, win_v, wsp_v, bsp_v, wout_v, c_v, wmod_v, f_v, fi_v,
            gs_v, us_v, gt_v, kf_v, vf_v, y_v, x1_v, flag_v, row_v, tap_v, mod_v, h_v, w_v, acc_v, a2_v, mean_v, zs_v,
            wis_v, wos_v, p_v, pr_v, o_v, woutt_v, brow_v, out_v, sems):
    S, D = q_v.shape
    FH = wout_v.shape[0]
    NA, NJ = S // C, D // LANES
    KS = sk_v.shape[0]
    HS, HF, HD = S // 2, FH // 2, D // 2
    nb = S // (2 * T)

    n_sem = [nb]

    def fetch(src, dst):
        cp = pltpu.make_async_copy(src, dst, sems.at[n_sem[0]])
        n_sem[0] += 1
        cp.start()
        return cp

    def rows(ref, i, n):
        return ref.at[pl.ds(i * n, n)]

    def cols(ref, i, n):
        return ref.at[:, pl.ds(i * n, n)]

    def mix_cols(i):
        cs = pl.ds(pl.multiple_of(i * 2 * T, 2 * T), 2 * T)
        return pltpu.make_async_copy(wsp_h.at[:, cs], wsp_v.at[i], sems.at[i])

    cp_g = [fetch(cols(g_h, 0, C), cols(g_v, 0, C))]
    cp_small = [fetch(f_h, f_v), fetch(sd_h, sd_v), fetch(sk_h, sk_v), fetch(c_h, c_v)]
    cp_kv = {}
    for n in range(1, NA + AHEAD):
        if n < NA:
            cp_g.append(fetch(cols(g_h, n, C), cols(g_v, n, C)))
        if n >= AHEAD:
            a = n - AHEAD
            for j0, j1 in ((0, J0), (J0, NJ)) if a == 0 else ((0, NJ),):
                at = (pl.ds(a * C, C), pl.ds(j0 * LANES, (j1 - j0) * LANES))
                cp_kv[a * NJ + j0] = [fetch(src.at[at], dst.at[at]) for src, dst in ((k_h, k_v), (v_h, v_v))]

    def q_block(i):
        return fetch(rows(q_h, i, 2 * T), rows(q_v, i, 2 * T))

    cp_q = [q_block(0)]
    cp_wmod = {0: fetch(cols(wmod_h, 0, 5 * D), cols(wmod_v, 0, 5 * D))}
    cp_win = {1: fetch(rows(win_h, 1, FH), rows(win_v, 1, FH))}
    cp_q += [q_block(1)]
    cp_rest = []

    def fetch_group(i):
        later = [n for n in SYNC if n > i]
        for n in range(i, (later + [nb + 1])[0]):
            if n + 1 < nb:
                cp_q.append(q_block(n + 1))
            mix_cols(n - 1).start()
        if not later:
            cp_wmod[5] = fetch(cols(wmod_h, 5, D), cols(wmod_v, 5, D))
            cp_win[0] = fetch(rows(win_h, 0, FH), rows(win_v, 0, FH))
            cp_rest.extend([fetch(bsp_h, bsp_v), fetch(wout_h, wout_v)])

    fetch_group(SYNC[0])
    flag_v[0] = 0

    @pl.loop(0, 2)
    def _(n):
        acc_v[n, 0:8] = jnp.zeros((8, T), F32)

    for cp in cp_small:
        cp.wait()
    sd_row = sd_v[...].astype(F32).reshape(1, D)
    sk = sk_v[...].astype(F32)
    tap_v[KS] = jnp.broadcast_to(sd_row, (8, D))
    for t in range(KS):
        tap_v[t] = jnp.broadcast_to(sk[t:t + 1] * (1.0 / C), (8, D))

    for r in range(R):
        fi_v[r] = _pack(_unpack(f_v[r]).T)

    raw = {}

    def transpose(a, j):
        gt_v[j] = g_v[j * LANES:(j + 1) * LANES, a * C:(a + 1) * C].T.astype(F32)

    def filter_spectrum(a, j):
        spec = _forward(f_v, [gt_v[j, pl.ds(r, M, stride=R), :] for r in range(R)])
        for qq in range(R):
            re, im = spec[qq]
            if a == 0:
                re = re + tap_v[KS, :, j * LANES:(j + 1) * LANES]
                spec[qq] = (re, im)
            else:
                re, im = re - raw[j][qq][1], im + raw[j][qq][0]
            gs_v[j, a, 2 * qq] = re
            gs_v[j, a, 2 * qq + 1] = im
        raw[j] = spec

    def widen(a, j):
        lanes = slice(j * LANES, (j + 1) * LANES)
        if a == 0:
            kf_v[j, 0:HIST, :] = jnp.zeros((HIST, LANES), F32)
            kf_v[j, HIST:, :] = k_v[0:C, lanes].astype(F32)
        else:
            kf_v[j] = k_v[a * C - HIST:(a + 1) * C, lanes].astype(F32)
        vf_v[j] = v_v[a * C:(a + 1) * C, lanes].astype(F32)

    def analyse(a, j):
        lanes = slice(j * LANES, (j + 1) * LANES)
        phases = [[] for _ in range(R)]
        for m0 in range(0, M, KM):
            kp = {s: kf_v[j, pl.ds(HIST + R * m0 + s, KM, stride=R), :] for s in range(1 - KS, R)}
            taps = [jnp.concatenate([tap_v[t, :, lanes]] * (KM // 8), axis=0) for t in range(KS)]
            for r in range(R):
                acc = kp[r] * taps[0]
                for t in range(1, KS):
                    acc = acc + kp[r - t] * taps[t]
                phases[r].append(acc * vf_v[j, pl.ds(R * m0 + r, KM, stride=R), :])
        spec = _forward(f_v, [jnp.concatenate(ph, axis=0) for ph in phases])
        for qq in range(R):
            us_v[j, a, 2 * qq], us_v[j, a, 2 * qq + 1] = spec[qq]

    def synthesise(a, j):
        packed = [[] for _ in range(R)]
        for g0 in range(0, M // 8, KG):
            gs = slice(g0, g0 + KG)
            ys = []
            for qq in range(R):
                yr = yi = None
                for b in range(a + 1):
                    ur, ui = us_v[j, a - b, 2 * qq, gs], us_v[j, a - b, 2 * qq + 1, gs]
                    gr, gi = gs_v[j, b, 2 * qq, gs], gs_v[j, b, 2 * qq + 1, gs]
                    tr, ti = gr * ur - gi * ui, gr * ui + gi * ur
                    yr, yi = (tr, ti) if b == 0 else (yr + tr, yi + ti)
                ys.append((yr, yi))
            for r, b in enumerate(_butterfly(ys, inverse=True)):
                packed[r].append(jnp.stack(b, axis=1).reshape(16 * KG, LANES).astype(BF16))
        for r in range(R):
            y_v[j, pl.ds(a * C + r, M, stride=R), :] = _dot(
                _unpack(fi_v[r]), jnp.concatenate(packed[r], axis=0))

    def modulation(n):
        cc = c_v[...].astype(F32)
        sc = jnp.broadcast_to(cc * jax.nn.sigmoid(cc), (16, D)).astype(BF16)
        return _dot(sc, wmod_v[:, n * D:(n + 1) * D])[0:8]

    def modulate():
        sa, ca, ga, sb, cb = (modulation(n) for n in range(5))
        mod_v[0] = ga * (1.0 + ca)
        mod_v[1] = ga * sa
        mod_v[2] = 1.0 + cb
        mod_v[3] = sb

    def scale(x, n):
        return (x.reshape(x.shape[0] // 8, 8, D) * mod_v[n]).reshape(x.shape)

    def shift(x, n):
        return (x.reshape(x.shape[0] // 8, 8, D) + mod_v[n]).reshape(x.shape)


    def halves(i, off=0, n=T):
        return [pl.ds(pl.multiple_of((2 * i + hh) * T + off, n), n) for hh in range(2)]

    def words(i, off=0, n=T):
        return [pl.ds(pl.multiple_of((2 * i + hh) * (T // 2) + off // 2, n // 2), n // 2) for hh in range(2)]

    last = []

    def paced(x, tiles=1, last=last):
        if not last:
            return x
        dep = last.pop()
        n = min(dep.shape[0], x.shape[0])
        dep = jnp.concatenate([dep[:n]] * (x.shape[0] // n), axis=0)
        cols = [x[:, c:c + LANES] for c in range(0, x.shape[1], LANES)]
        return jnp.concatenate([jnp.where(flag_v[0] > 0, dep, col) for col in cols[:tiles]] + cols[tiles:], axis=1)

    def delay(x):
        if DL < 0:
            return pltpu.roll(x, 1, 1)
        for _ in range(DL):
            x = jnp.tanh(x)
        return x

    def prepare(i):
        def piece(hh, off):
            rs = halves(i, off, PR)[hh]
            x = paced(q_v[rs, :].astype(F32))
            y = jnp.concatenate([y_v[j, rs, :] for j in range(NJ)], axis=1)
            x1 = x + shift(scale(_ln_rows(x), 0), 1) * y
            x1_v[rs, :] = x1
            h = shift(scale(_ln_rows(x1), 2), 3)
            h_v[words(i, off, PR)[hh], :] = _pack(h)
            last.append(h[:, -LANES:])

        return [functools.partial(piece, hh, off) for hh in range(2) for off in range(0, T, PR)]

    KI, KO = (NJ // 2) * LANES, (FH // (2 * LANES)) * LANES

    def project(i, fh):
        h1, h2 = (_unpack(h_v[hs, :]) for hs in words(i))
        right = _strassen_right(h1[:, :KI], h2[:, :KI], h1[:, KI:2 * KI], h2[:, KI:2 * KI])
        return _strassen(
            lambda n: _dot_nt(_unpack(wis_v[fh, n]), right[n]),
            lambda qh, hh: _dot_nt(_unpack(w_v[fh, qh, :, 2 * KI:]), (h1, h2)[hh][:, 2 * KI:]))

    def activate(i):
        for _ in activation(i):
            pass

    def activation(i):
        tot = {}
        for (qh, hh), z in project(i, 1):
            a2 = _gelu2(z)
            a2_v[i % 2, hh, qh * HF:(qh + 1) * HF, :] = a2
            tot[hh] = tot.get(hh, 0.0) + jnp.sum(a2.reshape(HF // 8, 8, T), axis=0)
            yield
        for hh in range(2):
            mean = jnp.sum(tot[hh], axis=0, keepdims=True) * (1.0 / FH)
            mean_v[i % 2, :, hh * T:(hh + 1) * T] = jnp.broadcast_to(mean, (8, T))

    def normalize(i):
        state = {}

        def centred(rs, n, mean):
            a2 = jnp.concatenate([a2_v[i % 2, hh, rs, :] for hh in range(2)], axis=1)
            return a2.reshape(n // 8, 8, 2 * T) - mean

        def var_piece(r0):
            d = centred(pl.ds(r0, NR), NR, paced(mean_v[i % 2], 2))
            part = jnp.sum(d * d, axis=0)
            state["ss"] = part if r0 == 0 else state["ss"] + part
            last.append(delay(state["ss"][:, :LANES]))
            if r0 + NR == FH:
                var = jnp.sum(state["ss"], axis=0, keepdims=True) * (1.0 / FH)
                state["rstd"] = jnp.broadcast_to(lax.rsqrt(var + 4.0 * EPS), (8, 2 * T))

        def out_piece(r0):
            mean = paced(mean_v[i % 2], 2)
            parts = []
            for odd in range(2):
                za, zb = ((centred(pl.ds(r + odd, NO // 2, stride=2), NO // 2, mean) * state["rstd"]
                           ).reshape(NO // 2, 2 * T) for r in (r0, HF + r0))
                parts.append(jnp.concatenate(
                    _strassen_left(za[:, :T], za[:, T:], zb[:, :T], zb[:, T:]), axis=1))
            words = _join_rows(*parts)
            zs_v[i % 2, r0 // 2:(r0 + NO) // 2, :] = words
            last.append(delay(pltpu.bitcast(words[-8:, :T], F32)))

        return ([functools.partial(var_piece, r0) for r0 in range(0, FH, NR)]
                + [functools.partial(out_piece, r0) for r0 in range(0, HF, NO)])

    def mix(i, extra=iter(())):
        def block(k0, th, sh, n):
            return jnp.concatenate([wsp_v[i, (2 * k + th) * T:(2 * k + th + 1) * T, sh * T:(sh + 1) * T]
                                    for k in range(k0, k0 + TW)], axis=0)

        for k0 in range(0, nb, TW):
            for n in ORD:
                for _ in range(XAT.count(ORD.index(n)) if k0 == 0 else 0):
                    next(extra, None)
                right = _strassen_right(*(block(k0, th, sh, n) for sh in range(2) for th in range(2)))[n]
                m = _dot_nt(_unpack(zs_v[i % 2, :, n * T:(n + 1) * T]), right)
                for k in range(TW):
                    at = (k0 + k, slice(n * HF, (n + 1) * HF))
                    part = m[:, k * T:(k + 1) * T]
                    acc_v[at] = acc_v[at] + part if i else part

    def step_b(i):
        if i in SYNC:
            upto = ([n for n in SYNC if n > i] + [nb + 1])[0]
            if upto <= nb:
                fetch_group(upto)
            for n in range(i, upto):
                mix_cols(n - 1).wait()
                if n + 1 < nb:
                    cp_q[n + 1].wait()
            if upto > nb:
                for cp in [cp_wmod[5], cp_win[0]] + cp_rest:
                    cp.wait()
        if i == 1:
            unpaced(normalize(0))
            last.clear()
        extra = activation(i)
        if i == 1:
            activate(i)
        mix(i - 1, iter(()) if i == 1 else extra)
        if i > 1:
            for _ in extra:
                pass
        side = prepare(i + 1) if i + 1 < nb else []
        if i == 1:
            last.clear()
        _interleave(side + normalize(i))

    def unpaced(pieces):
        for piece in pieces:
            last.clear()
            piece()

    def split_left(dst, top, bottom, width, pace):
        last.clear()
        for r0 in range(0, top.shape[0], 8):
            blk = [src[r0:r0 + 8, k:k + width] for src in (top, bottom) for k in (0, width)]
            if pace:
                blk = [paced(w, width // LANES, list(last)) for w in blk]
            blk = [_split_rows(w) for w in blk]
            even, odd = (_strassen_left(*(b[n] for b in blk)) for n in range(2))
            for n in range(7):
                words = dst[n, r0:r0 + 8, :] = _join_rows(even[n], odd[n])
            last[:] = [delay(words[:, :LANES])]

    def load_w_in(fh):
        for qh in range(2):
            for dst, src, n in ((0, qh * KO, KO), (KO, 2 * KO + qh * (HF - KO), HF - KO)):
                w_v[fh, qh, dst // 2:(dst + n) // 2] = _pack(win_v[fh * FH + src:fh * FH + src + n, :])
        split_left(wis_v.at[fh], w_v.at[fh, 0], w_v.at[fh, 1], KI, fh == 0 and PW)

    tiles = [(a, j) for a in range(NA) for j in range(NJ)]
    lead = AHEAD * NJ
    stages = ((transpose, 0), (filter_spectrum, 1), (widen, lead), (analyse, lead + 1), (synthesise, lead + 2))
    def await_inputs(n):
        todo = []
        if n % NJ == 0 and n < len(tiles):
            todo += [cp_g[n // NJ]]
        todo += cp_kv.get(n - lead, [])
        if n == len(tiles) + lead + MODAT:
            todo += [cp_q[0], cp_wmod[0]]
        if todo:
            for cp in todo:
                cp.wait()

    await_inputs(0)
    for n in range(len(tiles) + lead + 2 if "A" in PH else 0):
        if n == len(tiles) + lead + MODAT:
            modulate()
            unpaced(prepare(0))
        for k, (fn, lag) in enumerate(stages):
            if k == WAT:
                await_inputs(n + 1)
            if 0 <= n - lag < len(tiles):
                fn(*tiles[n - lag])
        if WAT == len(stages):
            await_inputs(n + 1)

    cp_win[1].wait()
    cp_q[1].wait()
    load_w_in(1)
    activate(0)
    unpaced(prepare(1))
    if 'S' in PH:
        mix_cols(0).wait()
        cp_q[2].wait()
        _interleave(normalize(0))
        activate(1)
        pltpu.sync_copy(out_v.at[pl.ds(0, 8)], out_h.at[pl.ds(0, 8)])
        pltpu.sync_copy(zs_v.at[0, pl.ds(0, 8), pl.ds(0, 640)], h_v.at[pl.ds(0, 8)])
        return
    if 'B' in PH:
        for i in range(1, nb if 'F' not in PH else 4):
            step_b(i)
    if 'F' in PH:
        out_v[0:16, 0:128] = (x1_v[0:16, 0:128] + y_v[1, 0:16, :] + acc_v[1, 0:16, :]).astype(BF16) + _unpack(h_v[0:8, 0:128] + zs_v[0, 0:8, 0:128])
        pltpu.sync_copy(out_v, out_h)
        pltpu.sync_copy(zs_v.at[0, pl.ds(0, 8), pl.ds(0, 640)], h_v.at[pl.ds(0, 8)])
        return

    out_sem0 = n_sem[0]

    def out_copy(i, hh):
        rs = halves(i)[hh]
        return pltpu.make_async_copy(out_v.at[rs], out_h.at[rs], sems.at[out_sem0 + 2 * i + hh])

    def gate(i, slot, zs):
        gates = _strassen_sum([acc_v[i, n * HF:(n + 1) * HF] for n in range(7)])
        ps = [None] * 4
        for (qh, hh), z in zs:
            g = gates[2 * qh + hh]
            g = (g.reshape(HF // 8, 8, T) + brow_v[:, halves(i)[hh]]).reshape(HF, T)
            ps[2 * qh + hh] = _gelu2(z) * g
        for n, val in enumerate(_strassen_right(*(p[:KO] for p in ps))):
            p_v[slot, n] = val
        for hh in range(2):
            pr_v[slot, hh] = jnp.concatenate([ps[hh][KO:], ps[2 + hh][KO:]], axis=0).astype(BF16)

    def project_out(slot):
        for (dh, hh), o in _strassen(
                lambda n: _dot(_unpack(wos_v[n]), p_v[slot, n]),
                lambda dh, hh: _dot(_unpack(woutt_v[dh, :, 2 * KO:]), pr_v[slot, hh])):
            o_v[slot, hh, dh * HD:(dh + 1) * HD] = o

    def finish(i, slot):
        for hh, rs in enumerate(halves(i)):
            out_v[rs, :] = (x1_v[rs, :] + scale(o_v[slot, hh].T, 4)).astype(out_v.dtype)
            out_copy(i, hh).start()

    def step_c(i, slot, n_done):
        if n_done >= 2:
            finish(i - 2, slot)
        gate(i, slot, project(i, 0))
        project_out(1 - slot)

    if 'B' not in PH:
        cp_q[2].wait()
    def load_w_out():
        woutt = _pack(wout_v[...].T)
        for dh in range(2):
            woutt_v[dh] = woutt[dh * HD // 2:(dh + 1) * HD // 2]
        split_left(wos_v, woutt_v.at[0], woutt_v.at[1], KO, True)

    load_w_in(0)
    brow_v[...] = jnp.broadcast_to(bsp_v[...].astype(F32).reshape(1, S), (8, S))
    mod_v[4] = 0.5 * modulation(5)
    z_first = list(project(0, 0))
    mix(nb - 1)
    gate(0, 0, z_first)
    load_w_out()
    for i in range(1, nb):
        step_c(i, i % 2, i)
    project_out(1)
    finish(nb - 2, 0)
    finish(nb - 1, 1)
    for i in range(nb):
        for hh in range(2):
            out_copy(i, hh).wait()


@jax.jit
def pallas_adaLN_cond__ssm_conv_h3__mixer_gmlp__prompt_kernel(
    A_q: jax.Array,
    A_k: jax.Array,
    A_v: jax.Array,
    A_shift_k: jax.Array,
    A_ssm_k: jax.Array,
    A_ssm_D: jax.Array,
    B_x: jax.Array,
    B_w_in: jax.Array,
    B_w_sp: jax.Array,
    B_b_sp: jax.Array,
    B_w_out: jax.Array,
    c: jax.Array,
    w_mod: jax.Array,
):
    del B_x
    B, S, D = A_q.shape
    FH = B_w_out.shape[0]
    assert B == 1 and S % C == 0 and D % LANES == 0 and B_w_in.shape[1] == 2 * FH
    NA, NJ, NB = S // C, D // LANES, S // (2 * T)
    KO = (FH // (2 * LANES)) * LANES
    operands = (
        A_q.reshape(S, D), A_k.reshape(S, D), A_v.reshape(S, D), A_shift_k.T, A_ssm_k, A_ssm_D,
        B_w_in.T, B_w_sp, B_b_sp, B_w_out, c, w_mod,
        _np_pack(_dft_matrix()),
    )
    spectrum = (2 * R, M // 8, 8, LANES)
    scratch = [pltpu.VMEM((NB, S, 2 * T) if o is B_w_sp else o.shape, o.dtype) for o in operands] + [
        pltpu.VMEM((R, M // 2, 2 * M), U32),
        pltpu.VMEM((NJ, NA) + spectrum, F32),
        pltpu.VMEM((NJ, NA) + spectrum, F32),
        pltpu.VMEM((NJ, C, LANES), F32),
        pltpu.VMEM((NJ, HIST + C, LANES), F32),
        pltpu.VMEM((NJ, C, LANES), F32),
        pltpu.VMEM((NJ, S, LANES), F32),
        pltpu.VMEM((S, D), F32),
        pltpu.SMEM((1,), jnp.int32),
        pltpu.VMEM((16, D), F32),
        pltpu.VMEM((A_shift_k.shape[1] + 1, 8, D), F32),
        pltpu.VMEM((5, 8, D), F32),
        pltpu.VMEM((S // 2, D), U32),
        pltpu.VMEM((2, 2, FH // 4, D), U32),
        pltpu.VMEM((NB, 7 * FH // 2 + PAD, T), F32),
        pltpu.VMEM((2, 2, FH, T), F32),
        pltpu.VMEM((2, 8, 2 * T), F32),
        pltpu.VMEM((2, FH // 4, 7 * T), U32),
        pltpu.VMEM((2, 7, FH // 4, (NJ // 2) * LANES), U32),
        pltpu.VMEM((7, D // 4, (FH // (2 * LANES)) * LANES), U32),
        pltpu.VMEM((2, 7, KO, T), BF16),
        pltpu.VMEM((2, 2, FH - 2 * KO, T), BF16),
        pltpu.VMEM((2, 2, D, T), F32),
        pltpu.VMEM((2, D // 4, FH), U32),
        pltpu.VMEM((8, S), F32),
        pltpu.VMEM((S, D), A_q.dtype),
        pltpu.SemaphoreType.DMA((96,)),
    ]
    out = pl.pallas_call(
        _kernel,
        out_shape=jax.ShapeDtypeStruct((S, D), A_q.dtype),
        in_specs=[pl.BlockSpec(memory_space=pl.ANY)] * len(operands),
        out_specs=pl.BlockSpec(memory_space=pl.ANY),
        scratch_shapes=scratch,
        compiler_params=pltpu.CompilerParams(vmem_limit_bytes=124 * 2**20, flags=FLAGS),
    )(*operands)
    return out.reshape(B, S, D)
```

```python
import functools

import numpy as np

import jax
import jax.numpy as jnp
from jax import lax
import jax.experimental.pallas as pl
import jax.experimental.pallas.tpu as pltpu

LANES = 128
R = 4
M = 128
C = R * M
HIST = 16
EPS = 1e-5
GELU_C1 = float(np.sqrt(2.0 / np.pi))
GELU_C3 = float(np.sqrt(2.0 / np.pi) * 0.044715)
T = 128
PR = 32
MB = 288
NR = 288
NO = 16
FLAGS = None
PH = 'ABC'
AHEAD = 3
WAT = 4
MODAT = 1
J0 = 2
KVW = {0: (0,), 5: (1,), 10: (2,), 15: (3,)}
TW = 4
SYNC = (1, 2, 4, 6)
ORD = (1, 4, 2, 3, 0, 6, 5)
PAD = 0
PW = 0
CUT = (2,)
XAT = (0, 1, 2, 3)
B8 = 1
CP = 0
DL = -1
CO = 1
NP = 8
KM = 128
KG = 16

F32 = jnp.float32
BF16 = jnp.bfloat16
U32 = jnp.uint32
NT = (((1,), (1,)), ((), ()))
QUADS = ((0, 0), (0, 1), (1, 0), (1, 1))


def _dft_matrix():
    f0 = np.arange(M)[:, None]
    m = np.arange(M)[None, :]
    fwd = np.zeros((R, 2 * M, M), np.float64)
    for r in range(R):
        n = R * m + r
        ph = -np.pi * ((n * (1 + 4 * f0)) % (4 * C)) / (2 * C)
        re = np.cos(ph).reshape(M // 8, 8, M)
        im = np.sin(ph).reshape(M // 8, 8, M)
        fwd[r] = np.stack([re, im], 1).reshape(2 * M, M)
    return fwd.astype(np.float32)


def _pack(x):
    return pltpu.bitcast(x.astype(BF16), U32)


def _unpack(w):
    return pltpu.bitcast(w, BF16)


def _join_rows(even, odd):
    return pltpu.pack_elementwise([even, odd], packed_dtype=BF16)


def _split_rows(w):
    return [pltpu.unpack_elementwise(w, index=n, packed_dtype=BF16, unpacked_dtype=F32) for n in range(2)]


def _np_pack(x):
    bits = x.astype(BF16).view(np.uint16).astype(np.uint32)
    return bits[..., 0::2, :] | (bits[..., 1::2, :] << 16)


def _dot(a, b):
    return jnp.dot(a, b, preferred_element_type=F32)


def _dot_nt(a, b):
    return lax.dot_general(a, b, NT, preferred_element_type=F32)


def _gelu2(x):
    t = jnp.tanh(x * (x * x * GELU_C3 + GELU_C1))
    return x * t + x


def _ln_rows(x):
    n = x.shape[-1]
    d = x - jnp.sum(x, axis=-1, keepdims=True) * (1.0 / n)
    var = jnp.sum(d * d, axis=-1, keepdims=True) * (1.0 / n)
    return d * lax.rsqrt(var + EPS)


def _interleave(*streams):
    order = sorted(((n + (0.5 if k else 0.0)) / len(st), k, n)
                   for k, st in enumerate(streams) for n in range(len(st)))
    for _, k, n in order:
        streams[k][n]()


def _strassen_left(a11, a12, a21, a22):
    return (a11 + a22, a21 + a22, a11, a22, a11 + a12, a21 - a11, a12 - a22)


def _strassen_right(b11, b12, b21, b22):
    f11, f12, f21, f22 = (b.astype(F32) for b in (b11, b12, b21, b22))
    return [b.astype(BF16) for b in (f11 + f22, b11, f12 - f22, f21 - f11, b22, f11 + f12, f21 + f22)]


def _strassen(product, rest):
    m2, m4 = product(1), product(3)
    yield (1, 0), m2 + m4 + rest(1, 0)
    m5, m3 = product(4), product(2)
    yield (0, 1), m3 + m5 + rest(0, 1)
    m1, m7 = product(0), product(6)
    yield (0, 0), (m4 - m5) + m1 + m7 + rest(0, 0)
    yield (1, 1), (m3 - m2) + m1 + product(5) + rest(1, 1)


def _strassen_sum(products):
    m1, m2, m3, m4, m5, m6, m7 = products
    return (m4 - m5) + m1 + m7, m3 + m5, m2 + m4, (m3 - m2) + m1 + m6


def _butterfly(x, inverse):
    (r0, i0), (r1, i1), (r2, i2), (r3, i3) = x
    ar, ai, br, bi = r0 + r2, i0 + i2, r0 - r2, i0 - i2
    cr, ci, dr, di = r1 + r3, i1 + i3, r1 - r3, i1 - i3
    lo, hi = (br + di, bi - dr), (br - di, bi + dr)
    if inverse:
        lo, hi = hi, lo
    return [(ar + cr, ai + ci), lo, (ar - cr, ai - ci), hi]


def _forward(f_v, phases):
    es = []
    for r in range(R):
        e = _dot(_unpack(f_v[r]), phases[r].astype(BF16)).reshape(M // 8, 2, 8, LANES)
        es.append((e[:, 0], e[:, 1]))
    return _butterfly(es, inverse=False)


def _kernel(q_h, k_h, v_h, sk_h, g_h, sd_h, win_h, wsp_h, bsp_h, wout_h, c_h, wmod_h, f_h,
            out_h,
            q_v, k_v, v_v, sk_v, g_v, sd_v, win_v, wsp_v, bsp_v, wout_v, c_v, wmod_v, f_v, fi_v,
            gs_v, us_v, gt_v, kf_v, vf_v, y_v, x1_v, flag_v, row_v, tap_v, mod_v, h_v, w_v, acc_v, a2_v, mean_v, zs_v,
            wis_v, wos_v, p_v, pr_v, o_v, woutt_v, brow_v, out_v, sems):
    S, D = q_v.shape
    FH = wout_v.shape[0]
    NA, NJ = S // C, D // LANES
    KS = sk_v.shape[0]
    HS, HF, HD = S // 2, FH // 2, D // 2
    nb = S // (2 * T)

    n_sem = [nb]

    def fetch(src, dst):
        cp = pltpu.make_async_copy(src, dst, sems.at[n_sem[0]])
        n_sem[0] += 1
        cp.start()
        return cp

    def rows(ref, i, n):
        return ref.at[pl.ds(i * n, n)]

    def cols(ref, i, n):
        return ref.at[:, pl.ds(i * n, n)]

    def mix_cols(i):
        cs = pl.ds(pl.multiple_of(i * 2 * T, 2 * T), 2 * T)
        return pltpu.make_async_copy(wsp_h.at[:, cs], wsp_v.at[i], sems.at[i])

    cp_g = [fetch(cols(g_h, 0, C), cols(g_v, 0, C))]
    cp_small = [fetch(f_h, f_v), fetch(sd_h, sd_v), fetch(sk_h, sk_v), fetch(c_h, c_v)]
    cp_kv = {}
    for n in range(1, NA + AHEAD):
        if n < NA:
            cp_g.append(fetch(cols(g_h, n, C), cols(g_v, n, C)))
        if n >= AHEAD:
            a = n - AHEAD
            for j0, j1 in ((0, J0), (J0, NJ)) if a == 0 else ((0, NJ),):
                at = (pl.ds(a * C, C), pl.ds(j0 * LANES, (j1 - j0) * LANES))
                cp_kv[a * NJ + j0] = [fetch(src.at[at], dst.at[at]) for src, dst in ((k_h, k_v), (v_h, v_v))]

    def q_block(i):
        return fetch(rows(q_h, i, 2 * T), rows(q_v, i, 2 * T))

    cp_q = [q_block(0)]
    cp_wmod = {0: fetch(cols(wmod_h, 0, 5 * D), cols(wmod_v, 0, 5 * D))}
    cp_win = {1: fetch(rows(win_h, 1, FH), rows(win_v, 1, FH))}
    cp_q += [q_block(1)]
    cp_rest = []

    def fetch_group(i):
        later = [n for n in SYNC if n > i]
        for n in range(i, (later + [nb + 1])[0]):
            if n + 1 < nb:
                cp_q.append(q_block(n + 1))
            mix_cols(n - 1).start()
        if not later:
            cp_wmod[5] = fetch(cols(wmod_h, 5, D), cols(wmod_v, 5, D))
            cp_win[0] = fetch(rows(win_h, 0, FH), rows(win_v, 0, FH))
            cp_rest.extend([fetch(bsp_h, bsp_v), fetch(wout_h, wout_v)])

    fetch_group(SYNC[0])
    flag_v[0] = 0

    def split_code():
        @pl.loop(0, 2)
        def _(n):
            acc_v[n, 7 * HF:] = jnp.zeros((8, T), F32)

    split_code()

    for cp in cp_small:
        cp.wait()
    sd_row = sd_v[...].astype(F32).reshape(1, D)
    sk = sk_v[...].astype(F32)
    tap_v[KS] = jnp.broadcast_to(sd_row, (8, D))
    for t in range(KS):
        tap_v[t] = jnp.broadcast_to(sk[t:t + 1] * (1.0 / C), (8, D))

    for r in range(R):
        fi_v[r] = _pack(_unpack(f_v[r]).T)

    raw = {}

    def transpose(a, j):
        gt_v[j] = g_v[j * LANES:(j + 1) * LANES, a * C:(a + 1) * C].T.astype(F32)

    def filter_spectrum(a, j):
        spec = _forward(f_v, [gt_v[j, pl.ds(r, M, stride=R), :] for r in range(R)])
        for qq in range(R):
            re, im = spec[qq]
            if a == 0:
                re = re + tap_v[KS, :, j * LANES:(j + 1) * LANES]
                spec[qq] = (re, im)
            else:
                re, im = re - raw[j][qq][1], im + raw[j][qq][0]
            gs_v[j, a, 2 * qq] = re
            gs_v[j, a, 2 * qq + 1] = im
        raw[j] = spec

    def widen(a, j):
        lanes = slice(j * LANES, (j + 1) * LANES)
        if a == 0:
            kf_v[j, 0:HIST, :] = jnp.zeros((HIST, LANES), F32)
            kf_v[j, HIST:, :] = k_v[0:C, lanes].astype(F32)
        else:
            kf_v[j] = k_v[a * C - HIST:(a + 1) * C, lanes].astype(F32)
        vf_v[j] = v_v[a * C:(a + 1) * C, lanes].astype(F32)

    def analyse(a, j):
        lanes = slice(j * LANES, (j + 1) * LANES)
        phases = [[] for _ in range(R)]
        for m0 in range(0, M, KM):
            kp = {s: kf_v[j, pl.ds(HIST + R * m0 + s, KM, stride=R), :] for s in range(1 - KS, R)}
            taps = [jnp.concatenate([tap_v[t, :, lanes]] * (KM // 8), axis=0) for t in range(KS)]
            for r in range(R):
                acc = kp[r] * taps[0]
                for t in range(1, KS):
                    acc = acc + kp[r - t] * taps[t]
                phases[r].append(acc * vf_v[j, pl.ds(R * m0 + r, KM, stride=R), :])
        spec = _forward(f_v, [jnp.concatenate(ph, axis=0) for ph in phases])
        for qq in range(R):
            us_v[j, a, 2 * qq], us_v[j, a, 2 * qq + 1] = spec[qq]

    def synthesise(a, j):
        packed = [[] for _ in range(R)]
        for g0 in range(0, M // 8, KG):
            gs = slice(g0, g0 + KG)
            ys = []
            for qq in range(R):
                yr = yi = None
                for b in range(a + 1):
                    ur, ui = us_v[j, a - b, 2 * qq, gs], us_v[j, a - b, 2 * qq + 1, gs]
                    gr, gi = gs_v[j, b, 2 * qq, gs], gs_v[j, b, 2 * qq + 1, gs]
                    tr, ti = gr * ur - gi * ui, gr * ui + gi * ur
                    yr, yi = (tr, ti) if b == 0 else (yr + tr, yi + ti)
                ys.append((yr, yi))
            for r, b in enumerate(_butterfly(ys, inverse=True)):
                packed[r].append(jnp.stack(b, axis=1).reshape(16 * KG, LANES).astype(BF16))
        for r in range(R):
            y_v[j, pl.ds(a * C + r, M, stride=R), :] = _dot(
                _unpack(fi_v[r]), jnp.concatenate(packed[r], axis=0))

    def modulation(n):
        cc = c_v[...].astype(F32)
        sc = jnp.broadcast_to(cc * jax.nn.sigmoid(cc), (16, D)).astype(BF16)
        return _dot(sc, wmod_v[:, n * D:(n + 1) * D])[0:8]

    def modulate():
        sa, ca, ga, sb, cb = (modulation(n) for n in range(5))
        mod_v[0] = ga * (1.0 + ca)
        mod_v[1] = ga * sa
        mod_v[2] = 1.0 + cb
        mod_v[3] = sb

    def scale(x, n):
        return (x.reshape(x.shape[0] // 8, 8, D) * mod_v[n]).reshape(x.shape)

    def shift(x, n):
        return (x.reshape(x.shape[0] // 8, 8, D) + mod_v[n]).reshape(x.shape)


    def halves(i, off=0, n=T):
        return [pl.ds(pl.multiple_of((2 * i + hh) * T + off, n), n) for hh in range(2)]

    def words(i, off=0, n=T):
        return [pl.ds(pl.multiple_of((2 * i + hh) * (T // 2) + off // 2, n // 2), n // 2) for hh in range(2)]

    last = []

    def paced(x, tiles=1, last=last):
        if not last:
            return x
        dep = last.pop()
        n = min(dep.shape[0], x.shape[0])
        dep = jnp.concatenate([dep[:n]] * (x.shape[0] // n), axis=0)
        cols = [x[:, c:c + LANES] for c in range(0, x.shape[1], LANES)]
        return jnp.concatenate([jnp.where(flag_v[0] > 0, dep, col) for col in cols[:tiles]] + cols[tiles:], axis=1)

    def delay(x):
        if DL < 0:
            return pltpu.roll(x, 1, 1)
        for _ in range(DL):
            x = jnp.tanh(x)
        return x

    def prepare(i):
        def piece(hh, off):
            rs = halves(i, off, PR)[hh]
            x = paced(q_v[rs, :].astype(F32))
            y = jnp.concatenate([y_v[j, rs, :] for j in range(NJ)], axis=1)
            x1 = x + shift(scale(_ln_rows(x), 0), 1) * y
            x1_v[rs, :] = x1
            h = shift(scale(_ln_rows(x1), 2), 3)
            h_v[words(i, off, PR)[hh], :] = _pack(h)
            last.append(h[:, -LANES:])

        return [functools.partial(piece, hh, off) for hh in range(2) for off in range(0, T, PR)]

    KI, KO = (NJ // 2) * LANES, (FH // (2 * LANES)) * LANES

    def project(i, fh):
        h1, h2 = (_unpack(h_v[hs, :]) for hs in words(i))
        right = _strassen_right(h1[:, :KI], h2[:, :KI], h1[:, KI:2 * KI], h2[:, KI:2 * KI])
        return _strassen(
            lambda n: _dot_nt(_unpack(wis_v[fh, n]), right[n]),
            lambda qh, hh: _dot_nt(_unpack(w_v[fh, qh, :, 2 * KI:]), (h1, h2)[hh][:, 2 * KI:]))

    def activate(i):
        for _ in activation(i):
            pass

    def activation(i):
        tot = {}
        for (qh, hh), z in project(i, 1):
            a2 = _gelu2(z)
            a2_v[i % 2, hh, qh * HF:(qh + 1) * HF, :] = a2
            tot[hh] = tot.get(hh, 0.0) + jnp.sum(a2.reshape(HF // 8, 8, T), axis=0)
            yield
        for hh in range(2):
            mean = jnp.sum(tot[hh], axis=0, keepdims=True) * (1.0 / FH)
            mean_v[i % 2, :, hh * T:(hh + 1) * T] = jnp.broadcast_to(mean, (8, T))

    def normalize(i):
        state = {}

        def centred(rs, n, mean):
            a2 = jnp.concatenate([a2_v[i % 2, hh, rs, :] for hh in range(2)], axis=1)
            return a2.reshape(n // 8, 8, 2 * T) - mean

        def var_piece(r0):
            d = centred(pl.ds(r0, NR), NR, paced(mean_v[i % 2], 2))
            part = jnp.sum(d * d, axis=0)
            state["ss"] = part if r0 == 0 else state["ss"] + part
            last.append(delay(state["ss"][:, :LANES]))
            if r0 + NR == FH:
                var = jnp.sum(state["ss"], axis=0, keepdims=True) * (1.0 / FH)
                state["rstd"] = jnp.broadcast_to(lax.rsqrt(var + 4.0 * EPS), (8, 2 * T))

        def out_piece(r0):
            mean = paced(mean_v[i % 2], 2)
            parts = []
            for odd in range(2):
                za, zb = ((centred(pl.ds(r + odd, NO // 2, stride=2), NO // 2, mean) * state["rstd"]
                           ).reshape(NO // 2, 2 * T) for r in (r0, HF + r0))
                parts.append(jnp.concatenate(
                    _strassen_left(za[:, :T], za[:, T:], zb[:, :T], zb[:, T:]), axis=1))
            words = _join_rows(*parts)
            zs_v[i % 2, r0 // 2:(r0 + NO) // 2, :] = words
            last.append(delay(pltpu.bitcast(words[-8:, :T], F32)))

        return ([functools.partial(var_piece, r0) for r0 in range(0, FH, NR)]
                + [functools.partial(out_piece, r0) for r0 in range(0, HF, NO)])

    def mix(i, extra=iter(())):
        def block(k0, th, sh, n):
            return jnp.concatenate([wsp_v[i, (2 * k + th) * T:(2 * k + th + 1) * T, sh * T:(sh + 1) * T]
                                    for k in range(k0, k0 + TW)], axis=0)

        for k0 in range(0, nb, TW):
            for n in ORD:
                for _ in range(XAT.count(ORD.index(n)) if k0 == 0 else 0):
                    next(extra, None)
                right = _strassen_right(*(block(k0, th, sh, n) for sh in range(2) for th in range(2)))[n]
                m = _dot_nt(_unpack(zs_v[i % 2, :, n * T:(n + 1) * T]), right)
                for k in range(TW):
                    at = (k0 + k, slice(n * HF, (n + 1) * HF))
                    part = m[:, k * T:(k + 1) * T]
                    acc_v[at] = acc_v[at] + part if i else part

    def step_b(i):
        if i in SYNC:
            if i in CUT:
                split_code()
            upto = ([n for n in SYNC if n > i] + [nb + 1])[0]
            if upto <= nb:
                fetch_group(upto)
            for n in range(i, upto):
                mix_cols(n - 1).wait()
                if n + 1 < nb:
                    cp_q[n + 1].wait()
            if upto > nb:
                for cp in [cp_wmod[5], cp_win[0]] + cp_rest:
                    cp.wait()
        if i == 1:
            unpaced(normalize(0))
            last.clear()
        extra = activation(i)
        if i == 1:
            activate(i)
        mix(i - 1, iter(()) if i == 1 else extra)
        if i > 1:
            for _ in extra:
                pass
        side = prepare(i + 1) if i + 1 < nb else []
        if i == 1:
            last.clear()
        _interleave(side + normalize(i))

    def unpaced(pieces):
        for piece in pieces:
            last.clear()
            piece()

    def split_left(dst, top, bottom, width, pace):
        last.clear()
        for r0 in range(0, top.shape[0], 8):
            blk = [src[r0:r0 + 8, k:k + width] for src in (top, bottom) for k in (0, width)]
            if pace:
                blk = [paced(w, width // LANES, list(last)) for w in blk]
            blk = [_split_rows(w) for w in blk]
            even, odd = (_strassen_left(*(b[n] for b in blk)) for n in range(2))
            for n in range(7):
                words = dst[n, r0:r0 + 8, :] = _join_rows(even[n], odd[n])
            last[:] = [delay(words[:, :LANES])]

    def load_w_in(fh):
        for qh in range(2):
            for dst, src, n in ((0, qh * KO, KO), (KO, 2 * KO + qh * (HF - KO), HF - KO)):
                w_v[fh, qh, dst // 2:(dst + n) // 2] = _pack(win_v[fh * FH + src:fh * FH + src + n, :])
        split_left(wis_v.at[fh], w_v.at[fh, 0], w_v.at[fh, 1], KI, fh == 0 and PW)

    tiles = [(a, j) for a in range(NA) for j in range(NJ)]
    lead = AHEAD * NJ
    stages = ((transpose, 0), (filter_spectrum, 1), (widen, lead), (analyse, lead + 1), (synthesise, lead + 2))
    def await_inputs(n):
        todo = []
        if n % NJ == 0 and n < len(tiles):
            todo += [cp_g[n // NJ]]
        todo += cp_kv.get(n - lead, [])
        if n == len(tiles) + lead + MODAT:
            todo += [cp_q[0], cp_wmod[0]]
        if todo:
            for cp in todo:
                cp.wait()

    await_inputs(0)
    for n in range(len(tiles) + lead + 2 if "A" in PH else 0):
        if n == len(tiles) + lead + MODAT:
            modulate()
            unpaced(prepare(0))
        for k, (fn, lag) in enumerate(stages):
            if k == WAT:
                await_inputs(n + 1)
            if 0 <= n - lag < len(tiles):
                fn(*tiles[n - lag])
        if WAT == len(stages):
            await_inputs(n + 1)

    cp_win[1].wait()
    cp_q[1].wait()
    load_w_in(1)
    activate(0)
    unpaced(prepare(1))
    if 'S' in PH:
        mix_cols(0).wait()
        cp_q[2].wait()
        _interleave(normalize(0))
        activate(1)
        pltpu.sync_copy(out_v.at[pl.ds(0, 8)], out_h.at[pl.ds(0, 8)])
        pltpu.sync_copy(zs_v.at[0, pl.ds(0, 8), pl.ds(0, 640)], h_v.at[pl.ds(0, 8)])
        return
    if 'B' in PH:
        for i in range(1, nb if 'F' not in PH else 4):
            step_b(i)
    if 'F' in PH:
        out_v[0:16, 0:128] = (x1_v[0:16, 0:128] + y_v[1, 0:16, :] + acc_v[1, 0:16, :]).astype(BF16) + _unpack(h_v[0:8, 0:128] + zs_v[0, 0:8, 0:128])
        pltpu.sync_copy(out_v, out_h)
        pltpu.sync_copy(zs_v.at[0, pl.ds(0, 8), pl.ds(0, 640)], h_v.at[pl.ds(0, 8)])
        return

    out_sem0 = n_sem[0]

    def out_copy(i, hh):
        rs = halves(i)[hh]
        return pltpu.make_async_copy(out_v.at[rs], out_h.at[rs], sems.at[out_sem0 + 2 * i + hh])

    def gate(i, slot, zs):
        gates = _strassen_sum([acc_v[i, n * HF:(n + 1) * HF] for n in range(7)])
        ps = [None] * 4
        for (qh, hh), z in zs:
            g = gates[2 * qh + hh]
            g = (g.reshape(HF // 8, 8, T) + brow_v[:, halves(i)[hh]]).reshape(HF, T)
            ps[2 * qh + hh] = _gelu2(z) * g
        for n, val in enumerate(_strassen_right(*(p[:KO] for p in ps))):
            p_v[slot, n] = val
        for hh in range(2):
            pr_v[slot, hh] = jnp.concatenate([ps[hh][KO:], ps[2 + hh][KO:]], axis=0).astype(BF16)

    def project_out(slot):
        for (dh, hh), o in _strassen(
                lambda n: _dot(_unpack(wos_v[n]), p_v[slot, n]),
                lambda dh, hh: _dot(_unpack(woutt_v[dh, :, 2 * KO:]), pr_v[slot, hh])):
            o_v[slot, hh, dh * HD:(dh + 1) * HD] = o

    def finish(i, slot):
        for hh, rs in enumerate(halves(i)):
            out_v[rs, :] = (x1_v[rs, :] + scale(o_v[slot, hh].T, 4)).astype(out_v.dtype)
            out_copy(i, hh).start()

    def step_c(i, slot, n_done):
        if n_done >= 2:
            finish(i - 2, slot)
        gate(i, slot, project(i, 0))
        project_out(1 - slot)

    if 'B' not in PH:
        cp_q[2].wait()
    def load_w_out():
        woutt = _pack(wout_v[...].T)
        for dh in range(2):
            woutt_v[dh] = woutt[dh * HD // 2:(dh + 1) * HD // 2]
        split_left(wos_v, woutt_v.at[0], woutt_v.at[1], KO, True)

    load_w_in(0)
    brow_v[...] = jnp.broadcast_to(bsp_v[...].astype(F32).reshape(1, S), (8, S))
    mod_v[4] = 0.5 * modulation(5)
    z_first = list(project(0, 0))
    mix(nb - 1)
    gate(0, 0, z_first)
    load_w_out()
    for i in range(1, nb):
        step_c(i, i % 2, i)
    project_out(1)
    finish(nb - 2, 0)
    finish(nb - 1, 1)
    for i in range(nb):
        for hh in range(2):
            out_copy(i, hh).wait()


@jax.jit
def pallas_adaLN_cond__ssm_conv_h3__mixer_gmlp__prompt_kernel(
    A_q: jax.Array,
    A_k: jax.Array,
    A_v: jax.Array,
    A_shift_k: jax.Array,
    A_ssm_k: jax.Array,
    A_ssm_D: jax.Array,
    B_x: jax.Array,
    B_w_in: jax.Array,
    B_w_sp: jax.Array,
    B_b_sp: jax.Array,
    B_w_out: jax.Array,
    c: jax.Array,
    w_mod: jax.Array,
):
    del B_x
    B, S, D = A_q.shape
    FH = B_w_out.shape[0]
    assert B == 1 and S % C == 0 and D % LANES == 0 and B_w_in.shape[1] == 2 * FH
    NA, NJ, NB = S // C, D // LANES, S // (2 * T)
    KO = (FH // (2 * LANES)) * LANES
    operands = (
        A_q.reshape(S, D), A_k.reshape(S, D), A_v.reshape(S, D), A_shift_k.T, A_ssm_k, A_ssm_D,
        B_w_in.T, B_w_sp, B_b_sp, B_w_out, c, w_mod,
        _np_pack(_dft_matrix()),
    )
    spectrum = (2 * R, M // 8, 8, LANES)
    scratch = [pltpu.VMEM((NB, S, 2 * T) if o is B_w_sp else o.shape, o.dtype) for o in operands] + [
        pltpu.VMEM((R, M // 2, 2 * M), U32),
        pltpu.VMEM((NJ, NA) + spectrum, F32),
        pltpu.VMEM((NJ, NA) + spectrum, F32),
        pltpu.VMEM((NJ, C, LANES), F32),
        pltpu.VMEM((NJ, HIST + C, LANES), F32),
        pltpu.VMEM((NJ, C, LANES), F32),
        pltpu.VMEM((NJ, S, LANES), F32),
        pltpu.VMEM((S, D), F32),
        pltpu.SMEM((1,), jnp.int32),
        pltpu.VMEM((16, D), F32),
        pltpu.VMEM((A_shift_k.shape[1] + 1, 8, D), F32),
        pltpu.VMEM((5, 8, D), F32),
        pltpu.VMEM((S // 2, D), U32),
        pltpu.VMEM((2, 2, FH // 4, D), U32),
        pltpu.VMEM((NB, 7 * FH // 2 + 8, T), F32),
        pltpu.VMEM((2, 2, FH, T), F32),
        pltpu.VMEM((2, 8, 2 * T), F32),
        pltpu.VMEM((2, FH // 4, 7 * T), U32),
        pltpu.VMEM((2, 7, FH // 4, (NJ // 2) * LANES), U32),
        pltpu.VMEM((7, D // 4, (FH // (2 * LANES)) * LANES), U32),
        pltpu.VMEM((2, 7, KO, T), BF16),
        pltpu.VMEM((2, 2, FH - 2 * KO, T), BF16),
        pltpu.VMEM((2, 2, D, T), F32),
        pltpu.VMEM((2, D // 4, FH), U32),
        pltpu.VMEM((8, S), F32),
        pltpu.VMEM((S, D), A_q.dtype),
        pltpu.SemaphoreType.DMA((96,)),
    ]
    out = pl.pallas_call(
        _kernel,
        out_shape=jax.ShapeDtypeStruct((S, D), A_q.dtype),
        in_specs=[pl.BlockSpec(memory_space=pl.ANY)] * len(operands),
        out_specs=pl.BlockSpec(memory_space=pl.ANY),
        scratch_shapes=scratch,
        compiler_params=pltpu.CompilerParams(vmem_limit_bytes=124 * 2**20, flags=FLAGS),
    )(*operands)
    return out.reshape(B, S, D)
```

```python
import functools

import numpy as np

import jax
import jax.numpy as jnp
from jax import lax
import jax.experimental.pallas as pl
import jax.experimental.pallas.tpu as pltpu

LANES = 128
R = 4
M = 128
C = R * M
HIST = 16
T = 128
EPS = 1e-5
GELU_C1 = float(np.sqrt(2.0 / np.pi))
GELU_C3 = float(np.sqrt(2.0 / np.pi) * 0.044715)

PR = 32
NR = 288
NO = 16
TW = 4
SYNC = (1, 2, 4, 6)
XAT = (0, 1, 2, 3)
ORDER = (1, 4, 2, 3, 0, 6, 5)

F32 = jnp.float32
BF16 = jnp.bfloat16
U32 = jnp.uint32
NT = (((1,), (1,)), ((), ()))


def _dft_matrix():
    f0 = np.arange(M)[:, None]
    m = np.arange(M)[None, :]
    fwd = np.zeros((R, 2 * M, M), np.float32)
    for r in range(R):
        ph = -np.pi * (((R * m + r) * (1 + 4 * f0)) % (4 * C)) / (2 * C)
        parts = [fn(ph).reshape(M // 8, 8, M) for fn in (np.cos, np.sin)]
        fwd[r] = np.stack(parts, 1).reshape(2 * M, M)
    return fwd


def _pack(x):
    return pltpu.bitcast(x.astype(BF16), U32)


def _unpack(w):
    return pltpu.bitcast(w, BF16)


def _split_rows(w):
    return [lax.bitcast_convert_type(x, F32) for x in (w << 16, w & np.uint32(0xFFFF0000))]


def _np_pack(x):
    bits = x.astype(BF16).view(np.uint16).astype(np.uint32)
    return bits[..., 0::2, :] | (bits[..., 1::2, :] << 16)


def _dot(a, b):
    return jnp.dot(a, b, preferred_element_type=F32)


def _dot_nt(a, b):
    return lax.dot_general(a, b, NT, preferred_element_type=F32)


def _gelu2(x):
    t = jnp.tanh(x * (x * x * GELU_C3 + GELU_C1))
    return x * t + x


def _ln_rows(x):
    n = x.shape[-1]
    d = x - jnp.sum(x, axis=-1, keepdims=True) * (1.0 / n)
    var = jnp.sum(d * d, axis=-1, keepdims=True) * (1.0 / n)
    return d * lax.rsqrt(var + EPS)


def _strassen_left(a11, a12, a21, a22):
    return (a11 + a22, a21 + a22, a11, a22, a11 + a12, a21 - a11, a12 - a22)


def _strassen_right(b11, b12, b21, b22):
    f11, f12, f21, f22 = (b.astype(F32) for b in (b11, b12, b21, b22))
    return [b.astype(BF16) for b in (f11 + f22, b11, f12 - f22, f21 - f11, b22, f11 + f12, f21 + f22)]


def _strassen(product, rest=None):
    def block(row, col, value):
        return (row, col), value if rest is None else value + rest(row, col)

    m2, m4 = product(1), product(3)
    yield block(1, 0, m2 + m4)
    m5, m3 = product(4), product(2)
    yield block(0, 1, m3 + m5)
    m1, m7 = product(0), product(6)
    yield block(0, 0, (m4 - m5) + m1 + m7)
    yield block(1, 1, (m3 - m2) + m1 + product(5))


def _butterfly(x, inverse):
    (r0, i0), (r1, i1), (r2, i2), (r3, i3) = x
    ar, ai, br, bi = r0 + r2, i0 + i2, r0 - r2, i0 - i2
    cr, ci, dr, di = r1 + r3, i1 + i3, r1 - r3, i1 - i3
    lo, hi = (br + di, bi - dr), (br - di, bi + dr)
    if inverse:
        lo, hi = hi, lo
    return [(ar + cr, ai + ci), lo, (ar - cr, ai - ci), hi]


def _forward(f_v, phases):
    es = []
    for r in range(R):
        e = _dot(_unpack(f_v[r]), phases[r].astype(BF16)).reshape(M // 8, 2, 8, LANES)
        es.append((e[:, 0], e[:, 1]))
    return _butterfly(es, inverse=False)


def _kernel(q_h, k_h, v_h, sk_h, g_h, sd_h, win_h, wsp_h, bsp_h, wout_h, c_h, wmod_h, f_h,
            out_h,
            q_v, k_v, v_v, sk_v, g_v, sd_v, win_v, wsp_v, bsp_v, wout_v, c_v, wmod_v, f_v,
            fi_v, gs_v, us_v, gt_v, kf_v, vf_v, tap_v, y_v, x1_v, mod_v, h_v, w_v, wis_v, a2_v,
            mean_v, zs_v, acc_v, brow_v, woutt_v, wos_v, p_v, pr_v, o_v, out_v, flag_v, sems):
    S, D = q_v.shape
    FH = wout_v.shape[0]
    KS = sk_v.shape[0]
    NA, NJ, NB = S // C, D // LANES, S // (2 * T)
    HF, HD = FH // 2, D // 2
    KI, KO = wis_v.shape[-1], wos_v.shape[-1]

    n_sem = [0]

    def fetch(src, dst):
        cp = pltpu.make_async_copy(src, dst, sems.at[n_sem[0]])
        n_sem[0] += 1
        cp.start()
        return cp

    def fetch_rows(src, dst, i, n):
        return fetch(src.at[pl.ds(i * n, n)], dst.at[pl.ds(i * n, n)])

    def fetch_cols(src, dst, i, n):
        return fetch(src.at[:, pl.ds(i * n, n)], dst.at[:, pl.ds(i * n, n)])

    def wait(copies):
        for cp in copies:
            cp.wait()

    def fetch_for_steps(first):
        later = [n for n in SYNC if n > first]
        copies = []
        for i in range(first, (later + [NB + 1])[0]):
            if i + 1 < NB:
                copies.append(fetch_rows(q_h, q_v, i + 1, 2 * T))
            copies.append(fetch(wsp_h.at[:, pl.ds((i - 1) * 2 * T, 2 * T)], wsp_v.at[i - 1]))
        if not later:
            copies += [fetch_cols(wmod_h, wmod_v, 5, D), fetch_rows(win_h, win_v, 0, FH),
                       fetch(bsp_h, bsp_v), fetch(wout_h, wout_v)]
        return copies

    cp_g = [[fetch_cols(g_h, g_v, 0, C), fetch(f_h, f_v), fetch(sd_h, sd_v), fetch(sk_h, sk_v),
             fetch(c_h, c_v)]]
    cp_g += [[fetch_cols(g_h, g_v, a, C)] for a in range(1, NA)]
    cp_kv = [[fetch_rows(k_h, k_v, a, C), fetch_rows(v_h, v_v, a, C)] for a in range(NA)]
    cp_mod = [fetch_rows(q_h, q_v, 0, 2 * T), fetch_cols(wmod_h, wmod_v, 0, 5 * D)]
    cp_proj = [fetch_rows(win_h, win_v, 1, FH), fetch_rows(q_h, q_v, 1, 2 * T)]
    cp_step = {SYNC[0]: fetch_for_steps(SYNC[0])}

    flag_v[0] = 0

    def split_code():
        @pl.loop(0, 2)
        def _(n):
            acc_v[n, 7 * HF:] = jnp.zeros((8, T), F32)

    last = []

    def paced(x, tiles=1, token=last):
        if not token:
            return x
        dep = token.pop()
        n = min(dep.shape[0], x.shape[0])
        dep = jnp.concatenate([dep[:n]] * (x.shape[0] // n), axis=0)
        cols = [x[:, c:c + LANES] for c in range(0, x.shape[1], LANES)]
        return jnp.concatenate(
            [jnp.where(flag_v[0] > 0, dep, col) for col in cols[:tiles]] + cols[tiles:], axis=1)

    def delayed(x):
        return pltpu.roll(x, 1, 1)

    def run(pieces, chained=True):
        for piece in pieces:
            if not chained:
                last.clear()
            piece()

    split_code()

    def transpose(a, j):
        gt_v[j] = _pack(g_v[j * LANES:(j + 1) * LANES, a * C:(a + 1) * C].T)

    def filter_spectrum(a, j):
        spec = _forward(f_v, [ph for r in range(R // 2)
                              for ph in _split_rows(gt_v[j, pl.ds(r, M, stride=R // 2), :])])
        for q in range(R):
            re, im = spec[q]
            if a == 0:
                re = re + tap_v[KS, :, j * LANES:(j + 1) * LANES]
            else:
                pr, pi = gs_v[j, 0, 2 * q], gs_v[j, 0, 2 * q + 1]
                for b in range(1, a):
                    pr, pi = gs_v[j, b, 2 * q] + pi, gs_v[j, b, 2 * q + 1] - pr
                re, im = re - pi, im + pr
            gs_v[j, a, 2 * q], gs_v[j, a, 2 * q + 1] = re, im

    def widen(a, j):
        lanes = slice(j * LANES, (j + 1) * LANES)
        if a == 0:
            kf_v[j, 0:HIST, :] = jnp.zeros((HIST, LANES), F32)
            kf_v[j, HIST:, :] = k_v[0:C, lanes].astype(F32)
        else:
            kf_v[j] = k_v[a * C - HIST:(a + 1) * C, lanes].astype(F32)
        vf_v[j] = v_v[a * C:(a + 1) * C, lanes].astype(F32)

    def analyse(a, j):
        lanes = slice(j * LANES, (j + 1) * LANES)
        kp = {s: kf_v[j, pl.ds(HIST + s, M, stride=R), :] for s in range(1 - KS, R)}
        taps = [jnp.concatenate([tap_v[t, :, lanes]] * (M // 8), axis=0) for t in range(KS)]
        phases = []
        for r in range(R):
            acc = kp[r] * taps[0]
            for t in range(1, KS):
                acc = acc + kp[r - t] * taps[t]
            phases.append(acc * vf_v[j, pl.ds(r, M, stride=R), :])
        spec = _forward(f_v, phases)
        for q in range(R):
            us_v[j, a, 2 * q], us_v[j, a, 2 * q + 1] = spec[q]

    def synthesise(a, j):
        ys = []
        for q in range(R):
            yr = yi = None
            for b in range(a + 1):
                ur, ui = us_v[j, a - b, 2 * q], us_v[j, a - b, 2 * q + 1]
                gr, gi = gs_v[j, b, 2 * q], gs_v[j, b, 2 * q + 1]
                tr, ti = gr * ur - gi * ui, gr * ui + gi * ur
                yr, yi = (tr, ti) if b == 0 else (yr + tr, yi + ti)
            ys.append((yr, yi))
        for r, pair in enumerate(_butterfly(ys, inverse=True)):
            spec = jnp.stack(pair, axis=1).reshape(2 * M, LANES).astype(BF16)
            y_v[j, pl.ds(a * C + r, M, stride=R), :] = _dot(_unpack(fi_v[r]), spec)

    def modulation(n):
        cc = c_v[...].astype(F32)
        sc = jnp.broadcast_to(cc * jax.nn.sigmoid(cc), (16, D)).astype(BF16)
        return _dot(sc, wmod_v[:, n * D:(n + 1) * D])[0:8]

    def scale(x, n):
        return (x.reshape(x.shape[0] // 8, 8, D) * mod_v[n]).reshape(x.shape)

    def shift(x, n):
        return (x.reshape(x.shape[0] // 8, 8, D) + mod_v[n]).reshape(x.shape)

    def prepare(i):
        def piece(r0):
            rs = slice(r0, r0 + PR)
            x = paced(q_v[rs, :].astype(F32))
            y = jnp.concatenate([y_v[j, rs, :] for j in range(NJ)], axis=1)
            x1 = x + shift(scale(_ln_rows(x), 0), 1) * y
            x1_v[rs, :] = x1
            h = shift(scale(_ln_rows(x1), 2), 3)
            h_v[r0 // 2:(r0 + PR) // 2, :] = _pack(h)
            last.append(h[:, -LANES:])

        return [functools.partial(piece, r0) for r0 in range(2 * i * T, 2 * (i + 1) * T, PR)]

    def split_left(dst, top, bottom, width, pace):
        last.clear()
        for r0 in range(0, top.shape[0], 8):
            blk = [src[r0:r0 + 8, k:k + width] for src in (top, bottom) for k in (0, width)]
            if pace:
                blk = [paced(w, width // LANES, list(last)) for w in blk]
            blk = [_unpack(w).astype(F32).reshape(2, 8, width) for w in blk]
            for n, val in enumerate(_strassen_left(*blk)):
                words = dst[n, r0:r0 + 8, :] = _pack(val.reshape(16, width))
            last[:] = [delayed(words[:, :LANES])]

    def load_w_in(fh):
        for qh in range(2):
            for dst, src, n in ((0, qh * KO, KO), (KO, 2 * KO + qh * (HF - KO), HF - KO)):
                w_v[fh, qh, dst // 2:(dst + n) // 2] = _pack(win_v[fh * FH + src:fh * FH + src + n, :])
        split_left(wis_v.at[fh], w_v.at[fh, 0], w_v.at[fh, 1], KI, False)

    def project(i, fh):
        hs = [_unpack(h_v[(2 * i + hh) * T // 2:(2 * i + hh + 1) * T // 2, :]) for hh in range(2)]
        right = _strassen_right(*(h[:, k:k + KI] for k in (0, KI) for h in hs))
        return _strassen(lambda n: _dot_nt(_unpack(wis_v[fh, n]), right[n]),
                         lambda qh, hh: _dot_nt(_unpack(w_v[fh, qh, :, 2 * KI:]), hs[hh][:, 2 * KI:]))

    def activate(i):
        tot = {}
        for (qh, hh), z in project(i, 1):
            a2 = _gelu2(z)
            a2_v[i % 2, qh * HF:(qh + 1) * HF, hh * T:(hh + 1) * T] = a2
            part = jnp.sum(a2.reshape(HF // 8, 8, T), axis=0)
            tot[hh] = tot[hh] + part if hh in tot else part
            yield
        for hh in range(2):
            mean = jnp.sum(tot[hh], axis=0, keepdims=True) * (1.0 / FH)
            mean_v[i % 2, :, hh * T:(hh + 1) * T] = jnp.broadcast_to(mean, (8, T))

    def normalize(i):
        state = {}

        def centred(r0, n, mean):
            return a2_v[i % 2, r0:r0 + n, :].reshape(n // 8, 8, 2 * T) - mean

        def var_piece(r0):
            d = centred(r0, NR, paced(mean_v[i % 2], 2))
            part = jnp.sum(d * d, axis=0)
            state["ss"] = part if r0 == 0 else state["ss"] + part
            last.append(delayed(state["ss"][:, :LANES]))
            if r0 + NR == FH:
                var = jnp.sum(state["ss"], axis=0, keepdims=True) * (1.0 / FH)
                state["rstd"] = jnp.broadcast_to(lax.rsqrt(var + 4.0 * EPS), (8, 2 * T))

        def out_piece(r0):
            mean = paced(mean_v[i % 2], 2)
            za, zb = (centred(r, NO, mean) * state["rstd"] for r in (r0, HF + r0))
            left = _strassen_left(za[..., :T], za[..., T:], zb[..., :T], zb[..., T:])
            words = _pack(jnp.concatenate(left, axis=2).reshape(NO, 7 * T))
            zs_v[i % 2, r0 // 2:(r0 + NO) // 2, :] = words
            last.append(delayed(lax.bitcast_convert_type(words[-8:, :T], F32)))

        return ([functools.partial(var_piece, r0) for r0 in range(0, FH, NR)]
                + [functools.partial(out_piece, r0) for r0 in range(0, HF, NO)])

    def mix(i, extra=iter(())):
        def block(k0, th, sh):
            return jnp.concatenate(
                [wsp_v[i, (2 * k + th) * T:(2 * k + th + 1) * T, sh * T:(sh + 1) * T]
                 for k in range(k0, k0 + TW)], axis=0)

        for k0 in range(0, NB, TW):
            for pos, n in enumerate(ORDER):
                for _ in range(XAT.count(pos) if k0 == 0 else 0):
                    next(extra, None)
                right = _strassen_right(*(block(k0, th, sh) for sh in range(2) for th in range(2)))[n]
                m = _dot_nt(_unpack(zs_v[i % 2, :, n * T:(n + 1) * T]), right)
                for k in range(TW):
                    at = (k0 + k, slice(n * HF, (n + 1) * HF))
                    part = m[:, k * T:(k + 1) * T]
                    acc_v[at] = acc_v[at] + part if i else part
        for _ in extra:
            pass

    def step_b(i):
        if i in SYNC:
            if i == SYNC[1]:
                split_code()
            for n in [n for n in SYNC if n > i][:1]:
                cp_step[n] = fetch_for_steps(n)
            wait(cp_step[i])
        extra = activate(i)
        if i == 1:
            run(normalize(0), chained=False)
            last.clear()
            for _ in extra:
                pass
        mix(i - 1, extra)
        run((prepare(i + 1) if i + 1 < NB else []) + normalize(i))

    def gate(i, zs):
        gates = dict(_strassen(lambda n: acc_v[i, n * HF:(n + 1) * HF]))
        ps = {}
        for (qh, hh), z in zs:
            bias = brow_v[:, (2 * i + hh) * T:(2 * i + hh + 1) * T]
            ps[qh, hh] = _gelu2(z) * (gates[qh, hh].reshape(HF // 8, 8, T) + bias).reshape(HF, T)
        for n, val in enumerate(_strassen_right(*(ps[qh, hh][:KO] for qh in range(2) for hh in range(2)))):
            p_v[i % 2, n] = val
        for hh in range(2):
            pr_v[i % 2, hh] = jnp.concatenate([ps[0, hh][KO:], ps[1, hh][KO:]], axis=0).astype(BF16)

    def project_out(i):
        for (dh, hh), o in _strassen(
                lambda n: _dot(_unpack(wos_v[n]), p_v[i % 2, n]),
                lambda dh, hh: _dot(_unpack(woutt_v[dh, :, 2 * KO:]), pr_v[i % 2, hh])):
            o_v[i % 2, hh, dh * HD:(dh + 1) * HD] = o

    cp_out = []

    def finish(i):
        for hh in range(2):
            rs = slice((2 * i + hh) * T, (2 * i + hh + 1) * T)
            out_v[rs, :] = (x1_v[rs, :] + scale(o_v[i % 2, hh].T, 4)).astype(out_v.dtype)
            cp_out.append(fetch_rows(out_v, out_h, 2 * i + hh, T))

    wait(cp_g[0])
    tap_v[KS] = jnp.broadcast_to(sd_v[...].astype(F32).reshape(1, D), (8, D))
    sk = sk_v[...].astype(F32)
    for t in range(KS):
        tap_v[t] = jnp.broadcast_to(sk[t:t + 1] * (1.0 / C), (8, D))
    for r in range(R):
        fi_v[r] = _pack(_unpack(f_v[r]).T)

    tiles = [(a, j) for a in range(NA) for j in range(NJ)]
    nt = len(tiles)
    needed = {a * NJ: cp_g[a] for a in range(1, NA)}
    needed.update({nt + a * NJ: cp_kv[a] for a in range(NA)})
    needed[2 * nt + 1] = cp_mod
    stages = ((transpose, 0), (filter_spectrum, 1), (widen, nt), (analyse, nt + 1), (synthesise, nt + 2))
    for n in range(2 * nt + 2):
        if n == 2 * nt + 1:
            sa, ca, ga, sb, cb = (modulation(m) for m in range(5))
            mod_v[0], mod_v[1], mod_v[2], mod_v[3] = ga * (1.0 + ca), ga * sa, 1.0 + cb, sb
            run(prepare(0), chained=False)
        for fn, lag in stages:
            if fn is synthesise and n + 1 in needed:
                wait(needed[n + 1])
            if 0 <= n - lag < nt:
                fn(*tiles[n - lag])

    wait(cp_proj)
    load_w_in(1)
    for _ in activate(0):
        pass
    run(prepare(1), chained=False)
    for i in range(1, NB):
        step_b(i)

    load_w_in(0)
    brow_v[...] = jnp.broadcast_to(bsp_v[...].astype(F32).reshape(1, S), (8, S))
    mod_v[4] = 0.5 * modulation(5)
    z_first = list(project(0, 0))
    mix(NB - 1)
    gate(0, z_first)
    woutt = _pack(wout_v[...].T)
    for dh in range(2):
        woutt_v[dh] = woutt[dh * HD // 2:(dh + 1) * HD // 2]
    split_left(wos_v, woutt_v.at[0], woutt_v.at[1], KO, True)

    for i in range(1, NB + 2):
        if i >= 2:
            finish(i - 2)
        if i < NB:
            gate(i, project(i, 0))
        if i <= NB:
            project_out(i - 1)
    wait(cp_out)


@jax.jit
def pallas_adaLN_cond__ssm_conv_h3__mixer_gmlp__prompt_kernel(
    A_q: jax.Array,
    A_k: jax.Array,
    A_v: jax.Array,
    A_shift_k: jax.Array,
    A_ssm_k: jax.Array,
    A_ssm_D: jax.Array,
    B_x: jax.Array,
    B_w_in: jax.Array,
    B_w_sp: jax.Array,
    B_b_sp: jax.Array,
    B_w_out: jax.Array,
    c: jax.Array,
    w_mod: jax.Array,
):
    del B_x
    B, S, D = A_q.shape
    FH = B_w_out.shape[0]
    KS = A_shift_k.shape[1]
    assert B == 1 and S % C == 0 and D % LANES == 0 and B_w_in.shape[1] == 2 * FH
    NA, NJ, NB = S // C, D // LANES, S // (2 * T)
    KI, KO = (D // (2 * LANES)) * LANES, (FH // (2 * LANES)) * LANES
    operands = (
        A_q.reshape(S, D), A_k.reshape(S, D), A_v.reshape(S, D), A_shift_k.T, A_ssm_k, A_ssm_D,
        B_w_in.T, B_w_sp, B_b_sp, B_w_out, c, w_mod, _np_pack(_dft_matrix()),
    )
    spectra = (NJ, NA, 2 * R, M // 8, 8, LANES)
    scratch = [pltpu.VMEM((NB, S, 2 * T) if o is B_w_sp else o.shape, o.dtype) for o in operands] + [
        pltpu.VMEM((R, M // 2, 2 * M), U32),
        pltpu.VMEM(spectra, F32),
        pltpu.VMEM(spectra, F32),
        pltpu.VMEM((NJ, C // 2, LANES), U32),
        pltpu.VMEM((NJ, HIST + C, LANES), F32),
        pltpu.VMEM((NJ, C, LANES), F32),
        pltpu.VMEM((KS + 1, 8, D), F32),
        pltpu.VMEM((NJ, S, LANES), F32),
        pltpu.VMEM((S, D), F32),
        pltpu.VMEM((5, 8, D), F32),
        pltpu.VMEM((S // 2, D), U32),
        pltpu.VMEM((2, 2, FH // 4, D), U32),
        pltpu.VMEM((2, 7, FH // 4, KI), U32),
        pltpu.VMEM((2, FH, 2 * T), F32),
        pltpu.VMEM((2, 8, 2 * T), F32),
        pltpu.VMEM((2, FH // 4, 7 * T), U32),
        pltpu.VMEM((NB, 7 * FH // 2 + 8, T), F32),
        pltpu.VMEM((8, S), F32),
        pltpu.VMEM((2, D // 4, FH), U32),
        pltpu.VMEM((7, D // 4, KO), U32),
        pltpu.VMEM((2, 7, KO, T), BF16),
        pltpu.VMEM((2, 2, FH - 2 * KO, T), BF16),
        pltpu.VMEM((2, 2, D, T), F32),
        pltpu.VMEM((S, D), A_q.dtype),
        pltpu.SMEM((1,), jnp.int32),
        pltpu.SemaphoreType.DMA((16 + 3 * NA + 4 * NB,)),
    ]
    out = pl.pallas_call(
        _kernel,
        out_shape=jax.ShapeDtypeStruct((S, D), A_q.dtype),
        in_specs=[pl.BlockSpec(memory_space=pl.ANY)] * len(operands),
        out_specs=pl.BlockSpec(memory_space=pl.ANY),
        scratch_shapes=scratch,
        compiler_params=pltpu.CompilerParams(vmem_limit_bytes=124 * 2**20),
    )(*operands)
    return out.reshape(B, S, D)
```

```python
import functools

import numpy as np

import jax
import jax.numpy as jnp
from jax import lax
import jax.experimental.pallas as pl
import jax.experimental.pallas.tpu as pltpu

LANES = 128
R = 4
M = 128
C = R * M
HIST = 16
T = 128
EPS = 1e-5
GELU_C1 = float(np.sqrt(2.0 / np.pi))
GELU_C3 = float(np.sqrt(2.0 / np.pi) * 0.044715)

PR = 32
NR = 288
NO = 16
TW = 2
SYNC = (1, 2, 4, 6)
XAT = (0, 1, 2, 3)
ORDER = (1, 4, 2, 3, 0, 6, 5)

F32 = jnp.float32
BF16 = jnp.bfloat16
U32 = jnp.uint32
NT = (((1,), (1,)), ((), ()))


def _dft_matrix():
    f0 = np.arange(M)[:, None]
    m = np.arange(M)[None, :]
    fwd = np.zeros((R, 2 * M, M), np.float32)
    for r in range(R):
        ph = -np.pi * (((R * m + r) * (1 + 4 * f0)) % (4 * C)) / (2 * C)
        parts = [fn(ph).reshape(M // 8, 8, M) for fn in (np.cos, np.sin)]
        fwd[r] = np.stack(parts, 1).reshape(2 * M, M)
    return fwd


def _pack(x):
    return pltpu.bitcast(x.astype(BF16), U32)


def _unpack(w):
    return pltpu.bitcast(w, BF16)


def _split_rows(w):
    return [lax.bitcast_convert_type(x, F32) for x in (w << 16, w & np.uint32(0xFFFF0000))]


def _np_pack(x):
    bits = x.astype(BF16).view(np.uint16).astype(np.uint32)
    return bits[..., 0::2, :] | (bits[..., 1::2, :] << 16)


def _dot(a, b):
    return jnp.dot(a, b, preferred_element_type=F32)


def _dot_nt(a, b):
    return lax.dot_general(a, b, NT, preferred_element_type=F32)


def _gelu2(x):
    t = jnp.tanh(x * (x * x * GELU_C3 + GELU_C1))
    return x * t + x


def _ln_rows(x):
    n = x.shape[-1]
    d = x - jnp.sum(x, axis=-1, keepdims=True) * (1.0 / n)
    var = jnp.sum(d * d, axis=-1, keepdims=True) * (1.0 / n)
    return d * lax.rsqrt(var + EPS)


def _strassen_left(a11, a12, a21, a22):
    return (a11 + a22, a21 + a22, a11, a22, a11 + a12, a21 - a11, a12 - a22)


def _strassen_right(b11, b12, b21, b22):
    f11, f12, f21, f22 = (b.astype(F32) for b in (b11, b12, b21, b22))
    return [b.astype(BF16) for b in (f11 + f22, b11, f12 - f22, f21 - f11, b22, f11 + f12, f21 + f22)]


def _strassen(product, rest=None):
    def block(row, col, value):
        return (row, col), value if rest is None else value + rest(row, col)

    m2, m4 = product(1), product(3)
    yield block(1, 0, m2 + m4)
    m5, m3 = product(4), product(2)
    yield block(0, 1, m3 + m5)
    m1, m7 = product(0), product(6)
    yield block(0, 0, (m4 - m5) + m1 + m7)
    yield block(1, 1, (m3 - m2) + m1 + product(5))


def _butterfly(x, inverse):
    (r0, i0), (r1, i1), (r2, i2), (r3, i3) = x
    ar, ai, br, bi = r0 + r2, i0 + i2, r0 - r2, i0 - i2
    cr, ci, dr, di = r1 + r3, i1 + i3, r1 - r3, i1 - i3
    lo, hi = (br + di, bi - dr), (br - di, bi + dr)
    if inverse:
        lo, hi = hi, lo
    return [(ar + cr, ai + ci), lo, (ar - cr, ai - ci), hi]


def _forward(f_v, phases):
    es = []
    for r in range(R):
        e = _dot(_unpack(f_v[r]), phases[r].astype(BF16)).reshape(M // 8, 2, 8, LANES)
        es.append((e[:, 0], e[:, 1]))
    return _butterfly(es, inverse=False)


def _kernel(q_h, k_h, v_h, sk_h, g_h, sd_h, win_h, wsp_h, bsp_h, wout_h, c_h, wmod_h, f_h,
            out_h,
            q_v, k_v, v_v, sk_v, g_v, sd_v, win_v, wsp_v, bsp_v, wout_v, c_v, wmod_v, f_v,
            fi_v, gs_v, us_v, gt_v, kf_v, vf_v, tap_v, y_v, x1_v, mod_v, h_v, w_v, wis_v, a2_v,
            mean_v, zs_v, acc_v, brow_v, woutt_v, wos_v, p_v, pr_v, o_v, out_v, flag_v, sems):
    S, D = q_v.shape
    FH = wout_v.shape[0]
    KS = sk_v.shape[0]
    NA, NJ, NB = S // C, D // LANES, S // (2 * T)
    HF, HD = FH // 2, D // 2
    KI, KO = wis_v.shape[-1], wos_v.shape[-1]

    n_sem = [0]

    def fetch(src, dst):
        cp = pltpu.make_async_copy(src, dst, sems.at[n_sem[0]])
        n_sem[0] += 1
        cp.start()
        return cp

    def fetch_rows(src, dst, i, n):
        return fetch(src.at[pl.ds(i * n, n)], dst.at[pl.ds(i * n, n)])

    def fetch_cols(src, dst, i, n):
        return fetch(src.at[:, pl.ds(i * n, n)], dst.at[:, pl.ds(i * n, n)])

    def wait(copies):
        for cp in copies:
            cp.wait()

    def fetch_for_steps(first):
        later = [n for n in SYNC if n > first]
        copies = []
        for i in range(first, (later + [NB + 1])[0]):
            if i + 1 < NB:
                copies.append(fetch_rows(q_h, q_v, i + 1, 2 * T))
            copies.append(fetch(wsp_h.at[:, pl.ds((i - 1) * 2 * T, 2 * T)], wsp_v.at[i - 1]))
        if not later:
            copies += [fetch_cols(wmod_h, wmod_v, 5, D), fetch_rows(win_h, win_v, 0, FH),
                       fetch(bsp_h, bsp_v), fetch(wout_h, wout_v)]
        return copies

    cp_g = [[fetch_cols(g_h, g_v, 0, C), fetch(f_h, f_v), fetch(sd_h, sd_v), fetch(sk_h, sk_v),
             fetch(c_h, c_v)]]
    cp_g += [[fetch_cols(g_h, g_v, a, C)] for a in range(1, NA)]
    cp_kv = [[fetch_rows(k_h, k_v, a, C), fetch_rows(v_h, v_v, a, C)] for a in range(NA)]
    cp_mod = [fetch_rows(q_h, q_v, 0, 2 * T), fetch_cols(wmod_h, wmod_v, 0, 5 * D)]
    cp_proj = [fetch_rows(win_h, win_v, 1, FH), fetch_rows(q_h, q_v, 1, 2 * T)]
    cp_step = {SYNC[0]: fetch_for_steps(SYNC[0])}

    flag_v[0] = 0

    def split_code():
        @pl.loop(0, 2)
        def _(n):
            acc_v[n, 7 * HF:] = jnp.zeros((8, T), F32)

    last = []

    def paced(x, tiles=1, token=last):
        if not token:
            return x
        dep = token.pop()
        n = min(dep.shape[0], x.shape[0])
        dep = jnp.concatenate([dep[:n]] * (x.shape[0] // n), axis=0)
        cols = [x[:, c:c + LANES] for c in range(0, x.shape[1], LANES)]
        return jnp.concatenate(
            [jnp.where(flag_v[0] > 0, dep, col) for col in cols[:tiles]] + cols[tiles:], axis=1)

    def delayed(x):
        return pltpu.roll(x, 1, 1)

    def run(pieces, chained=True):
        for piece in pieces:
            if not chained:
                last.clear()
            piece()

    split_code()

    def transpose(a, j):
        gt_v[j] = _pack(g_v[j * LANES:(j + 1) * LANES, a * C:(a + 1) * C].T)

    def filter_spectrum(a, j):
        spec = _forward(f_v, [ph for r in range(R // 2)
                              for ph in _split_rows(gt_v[j, pl.ds(r, M, stride=R // 2), :])])
        for q in range(R):
            re, im = spec[q]
            if a == 0:
                re = re + tap_v[KS, :, j * LANES:(j + 1) * LANES]
            else:
                pr, pi = gs_v[j, 0, 2 * q], gs_v[j, 0, 2 * q + 1]
                for b in range(1, a):
                    pr, pi = gs_v[j, b, 2 * q] + pi, gs_v[j, b, 2 * q + 1] - pr
                re, im = re - pi, im + pr
            gs_v[j, a, 2 * q], gs_v[j, a, 2 * q + 1] = re, im

    def widen(a, j):
        lanes = slice(j * LANES, (j + 1) * LANES)
        if a == 0:
            kf_v[j, 0:HIST, :] = jnp.zeros((HIST, LANES), F32)
            kf_v[j, HIST:, :] = k_v[0:C, lanes].astype(F32)
        else:
            kf_v[j] = k_v[a * C - HIST:(a + 1) * C, lanes].astype(F32)
        vf_v[j] = v_v[a * C:(a + 1) * C, lanes].astype(F32)

    def analyse(a, j):
        lanes = slice(j * LANES, (j + 1) * LANES)
        kp = {s: kf_v[j, pl.ds(HIST + s, M, stride=R), :] for s in range(1 - KS, R)}
        vp = [vf_v[j, pl.ds(r, M, stride=R), :] for r in range(R)]
        taps = [jnp.concatenate([tap_v[t, :, lanes]] * (M // 8), axis=0) for t in range(KS)]
        phases = []
        for r in range(R):
            acc = kp[r] * taps[0]
            for t in range(1, KS):
                acc = acc + kp[r - t] * taps[t]
            phases.append(acc * vp[r])
        spec = _forward(f_v, phases)
        for q in range(R):
            us_v[j, a, 2 * q], us_v[j, a, 2 * q + 1] = spec[q]

    def synthesise(a, j):
        ys = []
        for q in range(R):
            yr = yi = None
            for b in range(a + 1):
                ur, ui = us_v[j, a - b, 2 * q], us_v[j, a - b, 2 * q + 1]
                gr, gi = gs_v[j, b, 2 * q], gs_v[j, b, 2 * q + 1]
                tr, ti = gr * ur - gi * ui, gr * ui + gi * ur
                yr, yi = (tr, ti) if b == 0 else (yr + tr, yi + ti)
            ys.append((yr, yi))
        for r, pair in enumerate(_butterfly(ys, inverse=True)):
            spec = jnp.stack(pair, axis=1).reshape(2 * M, LANES).astype(BF16)
            y_v[j, pl.ds(a * C + r, M, stride=R), :] = _dot(_unpack(fi_v[r]), spec)

    def modulation(n):
        cc = c_v[...].astype(F32)
        sc = jnp.broadcast_to(cc * jax.nn.sigmoid(cc), (16, D)).astype(BF16)
        return _dot(sc, wmod_v[:, n * D:(n + 1) * D])[0:8]

    def scale(x, n):
        return (x.reshape(x.shape[0] // 8, 8, D) * mod_v[n]).reshape(x.shape)

    def shift(x, n):
        return (x.reshape(x.shape[0] // 8, 8, D) + mod_v[n]).reshape(x.shape)

    def prepare(i):
        def piece(r0):
            rs = slice(r0, r0 + PR)
            x = paced(q_v[rs, :].astype(F32))
            y = jnp.concatenate([y_v[j, rs, :] for j in range(NJ)], axis=1)
            x1 = x + shift(scale(_ln_rows(x), 0), 1) * y
            x1_v[rs, :] = x1
            h = shift(scale(_ln_rows(x1), 2), 3)
            h_v[r0 // 2:(r0 + PR) // 2, :] = _pack(h)
            last.append(h[:, -LANES:])

        return [functools.partial(piece, r0) for r0 in range(2 * i * T, 2 * (i + 1) * T, PR)]

    def split_left(dst, top, bottom, width, pace):
        last.clear()
        for r0 in range(0, top.shape[0], 8):
            blk = [src[r0:r0 + 8, k:k + width] for src in (top, bottom) for k in (0, width)]
            if pace:
                blk = [paced(w, width // LANES, list(last)) for w in blk]
            left = _strassen_left(*(_unpack(w).astype(F32) for w in blk))
            for n, val in enumerate(left):
                dst[n, 2 * r0:2 * r0 + 16, :] = val.astype(BF16)
            last[:] = [delayed(lax.bitcast_convert_type(left[0][:8, :LANES], U32))]

    def load_w_in(fh):
        for qh in range(2):
            for dst, src, n in ((0, qh * KO, KO), (KO, 2 * KO + qh * (HF - KO), HF - KO)):
                w_v[fh, qh, dst // 2:(dst + n) // 2] = _pack(win_v[fh * FH + src:fh * FH + src + n, :])
        split_left(wis_v.at[fh], w_v.at[fh, 0], w_v.at[fh, 1], KI, False)

    def project(i, fh):
        hs = [_unpack(h_v[(2 * i + hh) * T // 2:(2 * i + hh + 1) * T // 2, :]) for hh in range(2)]
        right = _strassen_right(*(h[:, k:k + KI] for k in (0, KI) for h in hs))
        return _strassen(lambda n: _dot_nt(wis_v[fh, n], right[n]),
                         lambda qh, hh: _dot_nt(_unpack(w_v[fh, qh, :, 2 * KI:]), hs[hh][:, 2 * KI:]))

    def activate(i):
        tot = {}
        for (qh, hh), z in project(i, 1):
            a2 = _gelu2(z)
            a2_v[i % 2, hh, qh * HF:(qh + 1) * HF, :] = a2
            part = jnp.sum(a2.reshape(HF // 8, 8, T), axis=0)
            tot[hh] = tot[hh] + part if hh in tot else part
            yield
        for hh in range(2):
            mean = jnp.sum(tot[hh], axis=0, keepdims=True) * (1.0 / FH)
            mean_v[i % 2, :, hh * T:(hh + 1) * T] = jnp.broadcast_to(mean, (8, T))

    def normalize(i):
        state = {}

        def centred(r0, n, mean):
            a2 = jnp.concatenate([a2_v[i % 2, hh, r0:r0 + n, :] for hh in range(2)], axis=1)
            return a2.reshape(n // 8, 8, 2 * T) - mean

        def var_piece(r0):
            d = centred(r0, NR, paced(mean_v[i % 2], 2))
            part = jnp.sum(d * d, axis=0)
            state["ss"] = part if r0 == 0 else state["ss"] + part
            last.append(delayed(state["ss"][:, :LANES]))
            if r0 + NR == FH:
                var = jnp.sum(state["ss"], axis=0, keepdims=True) * (1.0 / FH)
                state["rstd"] = jnp.broadcast_to(lax.rsqrt(var + 4.0 * EPS), (8, 2 * T))

        def out_piece(r0):
            mean = paced(mean_v[i % 2], 2)
            za, zb = (centred(r, NO, mean) * state["rstd"] for r in (r0, HF + r0))
            left = _strassen_left(za[..., :T], za[..., T:], zb[..., :T], zb[..., T:])
            for n, val in enumerate(left):
                zs_v[i % 2, n, r0:r0 + NO, :] = val.reshape(NO, T).astype(BF16)
            last.append(delayed(left[0][-1]))

        return ([functools.partial(var_piece, r0) for r0 in range(0, FH, NR)]
                + [functools.partial(out_piece, r0) for r0 in range(0, HF, NO)])

    def mix(i, extra=iter(())):
        def block(k0, th, sh):
            return jnp.concatenate(
                [wsp_v[i, (2 * k + th) * T:(2 * k + th + 1) * T, sh * T:(sh + 1) * T]
                 for k in range(k0, k0 + TW)], axis=0)

        for k0 in range(0, NB, TW):
            for pos, n in enumerate(ORDER):
                for _ in range(XAT.count(pos) if k0 == 0 else 0):
                    next(extra, None)
                right = _strassen_right(*(block(k0, th, sh) for sh in range(2) for th in range(2)))[n]
                m = _dot_nt(zs_v[i % 2, n], right)
                for k in range(TW):
                    at = (k0 + k, slice(n * HF, (n + 1) * HF))
                    part = m[:, k * T:(k + 1) * T]
                    acc_v[at] = acc_v[at] + part if i else part
        for _ in extra:
            pass

    def step_b(i):
        if i in SYNC:
            if i == SYNC[1]:
                split_code()
            for n in [n for n in SYNC if n > i][:1]:
                cp_step[n] = fetch_for_steps(n)
            wait(cp_step[i])
        extra = activate(i)
        if i == 1:
            run(normalize(0), chained=False)
            last.clear()
            for _ in extra:
                pass
        mix(i - 1, extra)
        run((prepare(i + 1) if i + 1 < NB else []) + normalize(i))

    def gate(i, zs):
        gates = dict(_strassen(lambda n: acc_v[i, n * HF:(n + 1) * HF]))
        ps = {}
        for (qh, hh), z in zs:
            bias = brow_v[:, (2 * i + hh) * T:(2 * i + hh + 1) * T]
            ps[qh, hh] = _gelu2(z) * (gates[qh, hh].reshape(HF // 8, 8, T) + bias).reshape(HF, T)
        for n, val in enumerate(_strassen_right(*(ps[qh, hh][:KO] for qh in range(2) for hh in range(2)))):
            p_v[i % 2, n] = val
        for hh in range(2):
            pr_v[i % 2, hh] = jnp.concatenate([ps[0, hh][KO:], ps[1, hh][KO:]], axis=0).astype(BF16)

    def project_out(i):
        for (dh, hh), o in _strassen(
                lambda n: _dot(wos_v[n], p_v[i % 2, n]),
                lambda dh, hh: _dot(_unpack(woutt_v[dh, :, 2 * KO:]), pr_v[i % 2, hh])):
            o_v[i % 2, hh, dh * HD:(dh + 1) * HD] = o

    cp_out = []

    def finish(i):
        for hh in range(2):
            rs = slice((2 * i + hh) * T, (2 * i + hh + 1) * T)
            out_v[rs, :] = (x1_v[rs, :] + scale(o_v[i % 2, hh].T, 4)).astype(out_v.dtype)
            cp_out.append(fetch_rows(out_v, out_h, 2 * i + hh, T))

    wait(cp_g[0])
    tap_v[KS] = jnp.broadcast_to(sd_v[...].astype(F32).reshape(1, D), (8, D))
    sk = sk_v[...].astype(F32)
    for t in range(KS):
        tap_v[t] = jnp.broadcast_to(sk[t:t + 1] * (1.0 / C), (8, D))
    for r in range(R):
        fi_v[r] = _pack(_unpack(f_v[r]).T)

    tiles = [(a, j) for a in range(NA) for j in range(NJ)]
    nt = len(tiles)
    needed = {a * NJ: cp_g[a] for a in range(1, NA)}
    needed.update({nt + a * NJ: cp_kv[a] for a in range(NA)})
    needed[2 * nt + 1] = cp_mod
    stages = ((transpose, 0), (filter_spectrum, 1), (widen, nt), (analyse, nt + 1), (synthesise, nt + 2))
    for n in range(2 * nt + 2):
        if n == 2 * nt + 1:
            sa, ca, ga, sb, cb = (modulation(m) for m in range(5))
            mod_v[0], mod_v[1], mod_v[2], mod_v[3] = ga * (1.0 + ca), ga * sa, 1.0 + cb, sb
            run(prepare(0), chained=False)
        for fn, lag in stages:
            if fn is synthesise and n + 1 in needed:
                wait(needed[n + 1])
            if 0 <= n - lag < nt:
                fn(*tiles[n - lag])

    wait(cp_proj)
    load_w_in(1)
    for _ in activate(0):
        pass
    run(prepare(1), chained=False)
    for i in range(1, NB):
        step_b(i)

    load_w_in(0)
    brow_v[...] = jnp.broadcast_to(bsp_v[...].astype(F32).reshape(1, S), (8, S))
    mod_v[4] = 0.5 * modulation(5)
    z_first = list(project(0, 0))
    mix(NB - 1)
    gate(0, z_first)
    woutt = _pack(wout_v[...].T)
    for dh in range(2):
        woutt_v[dh] = woutt[dh * HD // 2:(dh + 1) * HD // 2]
    split_left(wos_v, woutt_v.at[0], woutt_v.at[1], KO, True)

    for i in range(1, NB + 2):
        if i >= 2:
            finish(i - 2)
        if i < NB:
            gate(i, project(i, 0))
        if i <= NB:
            project_out(i - 1)
    wait(cp_out)


@jax.jit
def pallas_adaLN_cond__ssm_conv_h3__mixer_gmlp__prompt_kernel(
    A_q: jax.Array,
    A_k: jax.Array,
    A_v: jax.Array,
    A_shift_k: jax.Array,
    A_ssm_k: jax.Array,
    A_ssm_D: jax.Array,
    B_x: jax.Array,
    B_w_in: jax.Array,
    B_w_sp: jax.Array,
    B_b_sp: jax.Array,
    B_w_out: jax.Array,
    c: jax.Array,
    w_mod: jax.Array,
):
    del B_x
    B, S, D = A_q.shape
    FH = B_w_out.shape[0]
    KS = A_shift_k.shape[1]
    assert B == 1 and S % C == 0 and D % LANES == 0 and B_w_in.shape[1] == 2 * FH
    NA, NJ, NB = S // C, D // LANES, S // (2 * T)
    KI, KO = (D // (2 * LANES)) * LANES, (FH // (2 * LANES)) * LANES
    operands = (
        A_q.reshape(S, D), A_k.reshape(S, D), A_v.reshape(S, D), A_shift_k.T, A_ssm_k, A_ssm_D,
        B_w_in.T, B_w_sp, B_b_sp, B_w_out, c, w_mod, _np_pack(_dft_matrix()),
    )
    spectra = (NJ, NA, 2 * R, M // 8, 8, LANES)
    scratch = [pltpu.VMEM((NB, S, 2 * T) if o is B_w_sp else o.shape, o.dtype) for o in operands] + [
        pltpu.VMEM((R, M // 2, 2 * M), U32),
        pltpu.VMEM(spectra, F32),
        pltpu.VMEM(spectra, F32),
        pltpu.VMEM((NJ, C // 2, LANES), U32),
        pltpu.VMEM((NJ, HIST + C, LANES), F32),
        pltpu.VMEM((NJ, C, LANES), F32),
        pltpu.VMEM((KS + 1, 8, D), F32),
        pltpu.VMEM((NJ, S, LANES), F32),
        pltpu.VMEM((S, D), F32),
        pltpu.VMEM((5, 8, D), F32),
        pltpu.VMEM((S // 2, D), U32),
        pltpu.VMEM((2, 2, FH // 4, D), U32),
        pltpu.VMEM((2, 7, FH // 2, KI), BF16),
        pltpu.VMEM((2, 2, FH, T), F32),
        pltpu.VMEM((2, 8, 2 * T), F32),
        pltpu.VMEM((2, 7, FH // 2, T), BF16),
        pltpu.VMEM((NB, 7 * FH // 2 + 8, T), F32),
        pltpu.VMEM((8, S), F32),
        pltpu.VMEM((2, D // 4, FH), U32),
        pltpu.VMEM((7, D // 2, KO), BF16),
        pltpu.VMEM((2, 7, KO, T), BF16),
        pltpu.VMEM((2, 2, FH - 2 * KO, T), BF16),
        pltpu.VMEM((2, 2, D, T), F32),
        pltpu.VMEM((S, D), A_q.dtype),
        pltpu.SMEM((1,), jnp.int32),
        pltpu.SemaphoreType.DMA((16 + 3 * NA + 4 * NB,)),
    ]
    out = pl.pallas_call(
        _kernel,
        out_shape=jax.ShapeDtypeStruct((S, D), A_q.dtype),
        in_specs=[pl.BlockSpec(memory_space=pl.ANY)] * len(operands),
        out_specs=pl.BlockSpec(memory_space=pl.ANY),
        scratch_shapes=scratch,
        compiler_params=pltpu.CompilerParams(vmem_limit_bytes=124 * 2**20),
    )(*operands)
    return out.reshape(B, S, D)
```

```python
import functools

import numpy as np

import jax
import jax.numpy as jnp
from jax import lax
import jax.experimental.pallas as pl
import jax.experimental.pallas.tpu as pltpu

LANES = 128
R = 4
M = 128
C = R * M
HIST = 16
T = 128
EPS = 1e-5
GELU_C1 = float(np.sqrt(2.0 / np.pi))
GELU_C3 = float(np.sqrt(2.0 / np.pi) * 0.044715)

PR = 32
NR = 288
NO = 16
TW = 2
SYNC = (1, 2, 4, 6)
XAT = (0, 0, 2, 2)
ORDER = (1, 4, 2, 3, 0, 6, 5)
F32 = jnp.float32
BF16 = jnp.bfloat16
U32 = jnp.uint32
NT = (((1,), (1,)), ((), ()))


def _dft_matrix(r):
    def cis(steps):
        angle = (((steps + 2 * C) & (4 * C - 1)) - 2 * C).astype(F32) * (np.pi / (2 * C))
        return jnp.cos(angle), -jnp.sin(angle)

    n = lax.broadcasted_iota(jnp.int32, (8, M), 1) * R + r
    re, im = cis(n * (4 * lax.broadcasted_iota(jnp.int32, (8, M), 0) + 1))
    wr, wi = cis(n * 32)
    rows = []
    for _ in range(M // 8):
        rows += [re, im]
        re, im = re * wr - im * wi, re * wi + im * wr
    return jnp.concatenate(rows, axis=0)


def _pack(x):
    return pltpu.bitcast(x.astype(BF16), U32)


def _unpack(w):
    return pltpu.bitcast(w, BF16)


def _split_rows(w):
    return [lax.bitcast_convert_type(x, F32) for x in (w << 16, w & np.uint32(0xFFFF0000))]


def _dot(a, b):
    return jnp.dot(a, b, preferred_element_type=F32)


def _dot_nt(a, b):
    return lax.dot_general(a, b, NT, preferred_element_type=F32)


def _gelu2(x):
    t = jnp.tanh(x * (x * x * GELU_C3 + GELU_C1))
    return x * t + x


def _ln_rows(x):
    n = x.shape[-1]
    d = x - jnp.sum(x, axis=-1, keepdims=True) * (1.0 / n)
    var = jnp.sum(d * d, axis=-1, keepdims=True) * (1.0 / n)
    return d * lax.rsqrt(var + EPS)


def _strassen_left(a11, a12, a21, a22):
    return (a11 + a22, a21 + a22, a11, a22, a11 + a12, a21 - a11, a12 - a22)


def _strassen_right(b11, b12, b21, b22):
    f11, f12, f21, f22 = (b.astype(F32) for b in (b11, b12, b21, b22))
    return [b.astype(BF16) for b in (f11 + f22, b11, f12 - f22, f21 - f11, b22, f11 + f12, f21 + f22)]


def _strassen(product, rest=None):
    def block(row, col, value):
        return (row, col), value if rest is None else value + rest(row, col)

    m2, m4 = product(1), product(3)
    yield block(1, 0, m2 + m4)
    m5, m3 = product(4), product(2)
    yield block(0, 1, m3 + m5)
    m1, m7 = product(0), product(6)
    yield block(0, 0, (m4 - m5) + m1 + m7)
    yield block(1, 1, (m3 - m2) + m1 + product(5))


def _butterfly(x, inverse):
    (r0, i0), (r1, i1), (r2, i2), (r3, i3) = x
    ar, ai, br, bi = r0 + r2, i0 + i2, r0 - r2, i0 - i2
    cr, ci, dr, di = r1 + r3, i1 + i3, r1 - r3, i1 - i3
    lo, hi = (br + di, bi - dr), (br - di, bi + dr)
    if inverse:
        lo, hi = hi, lo
    return [(ar + cr, ai + ci), lo, (ar - cr, ai - ci), hi]


def _forward(f_v, phases):
    es = []
    for r in range(R):
        e = _dot(_unpack(f_v[r]), phases[r].astype(BF16)).reshape(M // 8, 2, 8, LANES)
        es.append((e[:, 0], e[:, 1]))
    return _butterfly(es, inverse=False)


def _kernel(q_h, k_h, v_h, sk_h, g_h, sd_h, win_h, wsp_h, bsp_h, wout_h, c_h, wmod_h,
            out_h,
            q_v, k_v, v_v, sk_v, g_v, sd_v, win_v, wsp_v, bsp_v, wout_v, c_v, wmod_v, f_v,
            fi_v, gs_v, us_v, gt_v, kf_v, vf_v, tap_v, y_v, x1_v, mod_v, h_v, w_v, wis_v, a2_v,
            mean_v, zs_v, acc_v, brow_v, woutt_v, wos_v, p_v, pr_v, o_v, out_v, flag_v, sems):
    S, D = q_v.shape
    FH = wout_v.shape[0]
    KS = sk_v.shape[0]
    NA, NJ, NB = S // C, D // LANES, S // (2 * T)
    HF, HD = FH // 2, D // 2
    KI, KO = wis_v.shape[-1], wos_v.shape[-1]

    n_sem = [0]

    def fetch(src, dst):
        cp = pltpu.make_async_copy(src, dst, sems.at[n_sem[0]])
        n_sem[0] += 1
        cp.start()
        return cp

    def fetch_rows(src, dst, i, n):
        return fetch(src.at[pl.ds(i * n, n)], dst.at[pl.ds(i * n, n)])

    def fetch_cols(src, dst, i, n):
        return fetch(src.at[:, pl.ds(i * n, n)], dst.at[:, pl.ds(i * n, n)])

    def wait(copies):
        for cp in copies:
            cp.wait()

    def fetch_for_steps(first):
        later = [n for n in SYNC if n > first]
        copies = []
        for i in range(first, (later + [NB + 1])[0]):
            if i + 1 < NB:
                copies.append(fetch_rows(q_h, q_v, i + 1, 2 * T))
            copies.append(fetch(wsp_h.at[:, pl.ds((i - 1) * 2 * T, 2 * T)], wsp_v.at[i - 1]))
        if not later:
            copies += [fetch_cols(wmod_h, wmod_v, 5, D), fetch_rows(win_h, win_v, 0, FH),
                       fetch(bsp_h, bsp_v), fetch(wout_h, wout_v)]
        return copies

    cp_g = [[fetch_cols(g_h, g_v, 0, C), fetch(sd_h, sd_v), fetch(sk_h, sk_v),
             fetch(c_h, c_v)]]
    cp_g += [[fetch_cols(g_h, g_v, a, C)] for a in range(1, NA)]
    cp_kv = [[fetch_rows(k_h, k_v, a, C), fetch_rows(v_h, v_v, a, C)] for a in range(NA)]
    cp_mod = [fetch_rows(q_h, q_v, 0, 2 * T), fetch_cols(wmod_h, wmod_v, 0, 5 * D)]
    cp_proj = [fetch_rows(win_h, win_v, 1, FH), fetch_rows(q_h, q_v, 1, 2 * T)]
    cp_step = {SYNC[0]: fetch_for_steps(SYNC[0])}

    flag_v[0] = 0

    def split_code():
        @pl.loop(0, 2)
        def _(n):
            acc_v[n, 7 * HF:] = jnp.zeros((8, T), F32)

    last = []

    def paced(x, tiles=1, token=last):
        if not token:
            return x
        dep = token.pop()
        n = min(dep.shape[0], x.shape[0])
        dep = jnp.concatenate([dep[:n]] * (x.shape[0] // n), axis=0)
        cols = [x[:, c:c + LANES] for c in range(0, x.shape[1], LANES)]
        return jnp.concatenate(
            [jnp.where(flag_v[0] > 0, dep, col) for col in cols[:tiles]] + cols[tiles:], axis=1)

    def delayed(x):
        return pltpu.roll(x, 1, 1)

    def run(pieces, chained=True):
        for piece in pieces:
            if not chained:
                last.clear()
            piece()

    def transpose(a, j):
        gt_v[j] = _pack(g_v[j * LANES:(j + 1) * LANES, a * C:(a + 1) * C].T)

    def filter_spectrum(a, j):
        spec = _forward(f_v, [ph for r in range(R // 2)
                              for ph in _split_rows(gt_v[j, pl.ds(r, M, stride=R // 2), :])])
        for q in range(R):
            re, im = spec[q]
            if a == 0:
                re = re + tap_v[KS, :, j * LANES:(j + 1) * LANES]
            else:
                pr, pi = gs_v[j, 0, 2 * q], gs_v[j, 0, 2 * q + 1]
                for b in range(1, a):
                    pr, pi = gs_v[j, b, 2 * q] + pi, gs_v[j, b, 2 * q + 1] - pr
                re, im = re - pi, im + pr
            gs_v[j, a, 2 * q], gs_v[j, a, 2 * q + 1] = re, im

    def widen(a, j):
        lanes = slice(j * LANES, (j + 1) * LANES)
        if a == 0:
            kf_v[j, 0:HIST, :] = jnp.zeros((HIST, LANES), F32)
            kf_v[j, HIST:, :] = k_v[0:C, lanes].astype(F32)
        else:
            kf_v[j] = k_v[a * C - HIST:(a + 1) * C, lanes].astype(F32)
        vf_v[j] = v_v[a * C:(a + 1) * C, lanes].astype(F32)

    def analyse(a, j):
        lanes = slice(j * LANES, (j + 1) * LANES)
        kp = {s: kf_v[j, pl.ds(HIST + s, M, stride=R), :] for s in range(1 - KS, R)}
        vp = [vf_v[j, pl.ds(r, M, stride=R), :] for r in range(R)]
        taps = [jnp.concatenate([tap_v[t, :, lanes]] * (M // 8), axis=0) for t in range(KS)]
        phases = []
        for r in range(R):
            acc = kp[r] * taps[0]
            for t in range(1, KS):
                acc = acc + kp[r - t] * taps[t]
            phases.append(acc * vp[r])
        spec = _forward(f_v, phases)
        for q in range(R):
            us_v[j, a, 2 * q], us_v[j, a, 2 * q + 1] = spec[q]

    def synthesise(a, j):
        ys = []
        for q in range(R):
            yr = yi = None
            for b in range(a + 1):
                ur, ui = us_v[j, a - b, 2 * q], us_v[j, a - b, 2 * q + 1]
                gr, gi = gs_v[j, b, 2 * q], gs_v[j, b, 2 * q + 1]
                tr, ti = gr * ur - gi * ui, gr * ui + gi * ur
                yr, yi = (tr, ti) if b == 0 else (yr + tr, yi + ti)
            ys.append((yr, yi))
        for r, pair in enumerate(_butterfly(ys, inverse=True)):
            spec = jnp.stack(pair, axis=1).reshape(2 * M, LANES).astype(BF16)
            y_v[j, pl.ds(a * C + r, M, stride=R), :] = _dot(_unpack(fi_v[r]), spec)

    def modulation(n):
        cc = c_v[...].astype(F32)
        sc = jnp.broadcast_to(cc * jax.nn.sigmoid(cc), (16, D)).astype(BF16)
        return _dot(sc, wmod_v[:, n * D:(n + 1) * D])[0:8]

    def scale(x, n):
        return (x.reshape(x.shape[0] // 8, 8, D) * mod_v[n]).reshape(x.shape)

    def shift(x, n):
        return (x.reshape(x.shape[0] // 8, 8, D) + mod_v[n]).reshape(x.shape)

    def prepare(i):
        def piece(r0):
            rs = slice(r0, r0 + PR)
            x = paced(q_v[rs, :].astype(F32))
            y = jnp.concatenate([y_v[j, rs, :] for j in range(NJ)], axis=1)
            x1 = x + shift(scale(_ln_rows(x), 0), 1) * y
            x1_v[rs, :] = x1
            h = shift(scale(_ln_rows(x1), 2), 3)
            h_v[r0 // 2:(r0 + PR) // 2, :] = _pack(h)
            last.append(h[:, -LANES:])

        return [functools.partial(piece, r0) for r0 in range(2 * i * T, 2 * (i + 1) * T, PR)]

    def split_left(dst, top, bottom, width, pace):
        last.clear()
        for r0 in range(0, top.shape[0], 8):
            blk = [src[r0:r0 + 8, k:k + width] for src in (top, bottom) for k in (0, width)]
            if pace:
                blk = [paced(w, width // LANES, list(last)) for w in blk]
            left = _strassen_left(*(_unpack(w).astype(F32) for w in blk))
            for n, val in enumerate(left):
                dst[n, 2 * r0:2 * r0 + 16, :] = val.astype(BF16)
            last[:] = [delayed(lax.bitcast_convert_type(left[0][:8, :LANES], U32))]

    def load_w_in(fh):
        for qh in range(2):
            for dst, src, n in ((0, qh * KO, KO), (KO, 2 * KO + qh * (HF - KO), HF - KO)):
                w_v[fh, qh, dst // 2:(dst + n) // 2] = _pack(win_v[fh * FH + src:fh * FH + src + n, :])
        split_left(wis_v.at[fh], w_v.at[fh, 0], w_v.at[fh, 1], KI, False)

    def project(i, fh):
        hs = [_unpack(h_v[(2 * i + hh) * T // 2:(2 * i + hh + 1) * T // 2, :]) for hh in range(2)]
        right = _strassen_right(*(h[:, k:k + KI] for k in (0, KI) for h in hs))
        return _strassen(lambda n: _dot_nt(wis_v[fh, n], right[n]),
                         lambda qh, hh: _dot_nt(_unpack(w_v[fh, qh, :, 2 * KI:]), hs[hh][:, 2 * KI:]))

    def activate(i):
        tot = {}
        for (qh, hh), z in project(i, 1):
            a2 = _gelu2(z)
            a2_v[i % 2, hh, qh * HF:(qh + 1) * HF, :] = a2
            part = jnp.sum(a2.reshape(HF // 8, 8, T), axis=0)
            tot[hh] = tot[hh] + part if hh in tot else part
            yield
        for hh in range(2):
            mean = jnp.sum(tot[hh], axis=0, keepdims=True) * (1.0 / FH)
            mean_v[i % 2, :, hh * T:(hh + 1) * T] = jnp.broadcast_to(mean, (8, T))

    def normalize(i):
        state = {}

        def centred(r0, n, mean):
            a2 = jnp.concatenate([a2_v[i % 2, hh, r0:r0 + n, :] for hh in range(2)], axis=1)
            return a2.reshape(n // 8, 8, 2 * T) - mean

        def var_piece(r0):
            d = centred(r0, NR, paced(mean_v[i % 2], 2))
            part = jnp.sum(d * d, axis=0)
            state["ss"] = part if r0 == 0 else state["ss"] + part
            last.append(delayed(state["ss"][:, :LANES]))
            if r0 + NR == FH:
                var = jnp.sum(state["ss"], axis=0, keepdims=True) * (1.0 / FH)
                state["rstd"] = jnp.broadcast_to(lax.rsqrt(var + 4.0 * EPS), (8, 2 * T))

        def out_piece(r0):
            mean = paced(mean_v[i % 2], 2)
            za, zb = (centred(r, NO, mean) * state["rstd"] for r in (r0, HF + r0))
            left = _strassen_left(za[..., :T], za[..., T:], zb[..., :T], zb[..., T:])
            for n, val in enumerate(left):
                zs_v[i % 2, n, r0:r0 + NO, :] = val.reshape(NO, T).astype(BF16)
            last.append(delayed(left[0][-1]))

        return ([functools.partial(var_piece, r0) for r0 in range(0, FH, NR)]
                + [functools.partial(out_piece, r0) for r0 in range(0, HF, NO)])

    def mix(i, extra=iter(())):
        def block(k0, th, sh):
            return jnp.concatenate(
                [wsp_v[i, (2 * k + th) * T:(2 * k + th + 1) * T, sh * T:(sh + 1) * T]
                 for k in range(k0, k0 + TW)], axis=0)

        for k0 in range(0, NB, TW):
            for pos, n in enumerate(ORDER):
                for _ in range(XAT.count(pos) if k0 == 0 else 0):
                    next(extra, None)
                right = _strassen_right(*(block(k0, th, sh) for sh in range(2) for th in range(2)))[n]
                m = _dot_nt(zs_v[i % 2, n], right)
                for k in range(TW):
                    at = (k0 + k, slice(n * HF, (n + 1) * HF))
                    part = m[:, k * T:(k + 1) * T]
                    acc_v[at] = acc_v[at] + part if i else part
        for _ in extra:
            pass

    def step_b(i):
        if i in SYNC:
            if i == SYNC[1]:
                split_code()
            for n in [n for n in SYNC if n > i][:1]:
                cp_step[n] = fetch_for_steps(n)
            wait(cp_step[i])
        extra = activate(i)
        if i == 1:
            run(normalize(0), chained=False)
            last.clear()
            for _ in extra:
                pass
        mix(i - 1, extra)
        run((prepare(i + 1) if i + 1 < NB else []) + normalize(i))

    def gate(i, zs):
        gates = dict(_strassen(lambda n: acc_v[i, n * HF:(n + 1) * HF]))
        ps = {}
        for (qh, hh), z in zs:
            bias = brow_v[:, (2 * i + hh) * T:(2 * i + hh + 1) * T]
            ps[qh, hh] = _gelu2(z) * (gates[qh, hh].reshape(HF // 8, 8, T) + bias).reshape(HF, T)
        for n, val in enumerate(_strassen_right(*(ps[qh, hh][:KO] for qh in range(2) for hh in range(2)))):
            p_v[i % 2, n] = val
        for hh in range(2):
            pr_v[i % 2, hh] = jnp.concatenate([ps[0, hh][KO:], ps[1, hh][KO:]], axis=0).astype(BF16)

    def project_out(i):
        for (dh, hh), o in _strassen(
                lambda n: _dot(wos_v[n], p_v[i % 2, n]),
                lambda dh, hh: _dot(_unpack(woutt_v[dh, :, 2 * KO:]), pr_v[i % 2, hh])):
            o_v[i % 2, hh, dh * HD:(dh + 1) * HD] = o

    cp_out = []

    def finish(i):
        for hh in range(2):
            rs = slice((2 * i + hh) * T, (2 * i + hh + 1) * T)
            out_v[rs, :] = (x1_v[rs, :] + scale(o_v[i % 2, hh].T, 4)).astype(out_v.dtype)
            cp_out.append(fetch_rows(out_v, out_h, 2 * i + hh, T))

    split_code()
    for r in range(R):
        f = _dft_matrix(r).astype(BF16)
        f_v[r], fi_v[r] = _pack(f), _pack(f.T)

    wait(cp_g[0])
    tap_v[KS] = jnp.broadcast_to(sd_v[...].astype(F32).reshape(1, D), (8, D))
    sk = sk_v[...].astype(F32)
    for t in range(KS):
        tap_v[t] = jnp.broadcast_to(sk[t:t + 1] * (1.0 / C), (8, D))

    tiles = [(a, j) for a in range(NA) for j in range(NJ)]
    nt = len(tiles)
    needed = {a * NJ: cp_g[a] for a in range(1, NA)}
    needed.update({nt + a * NJ: cp_kv[a] for a in range(NA)})
    needed[2 * nt + 1] = cp_mod
    stages = ((transpose, 0), (filter_spectrum, 1), (widen, nt), (analyse, nt + 1), (synthesise, nt + 2))
    for n in range(2 * nt + 2):
        if n == 2 * nt + 1:
            sa, ca, ga, sb, cb = (modulation(m) for m in range(5))
            mod_v[0], mod_v[1], mod_v[2], mod_v[3] = ga * (1.0 + ca), ga * sa, 1.0 + cb, sb
            run(prepare(0), chained=False)
        for fn, lag in stages:
            if fn is synthesise and n + 1 in needed:
                wait(needed[n + 1])
            if 0 <= n - lag < nt:
                fn(*tiles[n - lag])

    wait(cp_proj)
    load_w_in(1)
    for _ in activate(0):
        pass
    run(prepare(1), chained=False)
    for i in range(1, NB):
        step_b(i)

    load_w_in(0)
    brow_v[...] = jnp.broadcast_to(bsp_v[...].astype(F32).reshape(1, S), (8, S))
    mod_v[4] = 0.5 * modulation(5)
    z_first = list(project(0, 0))
    mix(NB - 1)
    gate(0, z_first)
    woutt = _pack(wout_v[...].T)
    for dh in range(2):
        woutt_v[dh] = woutt[dh * HD // 2:(dh + 1) * HD // 2]
    split_left(wos_v, woutt_v.at[0], woutt_v.at[1], KO, True)

    for i in range(1, NB + 2):
        if i >= 2:
            finish(i - 2)
        if i < NB:
            gate(i, project(i, 0))
        if i <= NB:
            project_out(i - 1)
    wait(cp_out)


@jax.jit
def pallas_adaLN_cond__ssm_conv_h3__mixer_gmlp__prompt_kernel(
    A_q: jax.Array,
    A_k: jax.Array,
    A_v: jax.Array,
    A_shift_k: jax.Array,
    A_ssm_k: jax.Array,
    A_ssm_D: jax.Array,
    B_x: jax.Array,
    B_w_in: jax.Array,
    B_w_sp: jax.Array,
    B_b_sp: jax.Array,
    B_w_out: jax.Array,
    c: jax.Array,
    w_mod: jax.Array,
):
    del B_x
    B, S, D = A_q.shape
    FH = B_w_out.shape[0]
    KS = A_shift_k.shape[1]
    assert B == 1 and S % C == 0 and D % LANES == 0 and B_w_in.shape[1] == 2 * FH
    NA, NJ, NB = S // C, D // LANES, S // (2 * T)
    KI, KO = (D // (2 * LANES)) * LANES, (FH // (2 * LANES)) * LANES
    operands = (
        A_q.reshape(S, D), A_k.reshape(S, D), A_v.reshape(S, D), A_shift_k.T, A_ssm_k, A_ssm_D,
        B_w_in.T, B_w_sp, B_b_sp, B_w_out, c, w_mod,
    )
    spectra = (NJ, NA, 2 * R, M // 8, 8, LANES)
    scratch = [pltpu.VMEM((NB, S, 2 * T) if o is B_w_sp else o.shape, o.dtype) for o in operands] + [
        pltpu.VMEM((R, M, M), U32),
        pltpu.VMEM((R, M // 2, 2 * M), U32),
        pltpu.VMEM(spectra, F32),
        pltpu.VMEM(spectra, F32),
        pltpu.VMEM((NJ, C // 2, LANES), U32),
        pltpu.VMEM((NJ, HIST + C, LANES), F32),
        pltpu.VMEM((NJ, C, LANES), F32),
        pltpu.VMEM((KS + 1, 8, D), F32),
        pltpu.VMEM((NJ, S, LANES), F32),
        pltpu.VMEM((S, D), F32),
        pltpu.VMEM((5, 8, D), F32),
        pltpu.VMEM((S // 2, D), U32),
        pltpu.VMEM((2, 2, FH // 4, D), U32),
        pltpu.VMEM((2, 7, FH // 2, KI), BF16),
        pltpu.VMEM((2, 2, FH, T), F32),
        pltpu.VMEM((2, 8, 2 * T), F32),
        pltpu.VMEM((2, 7, FH // 2, T), BF16),
        pltpu.VMEM((NB, 7 * FH // 2 + 8, T), F32),
        pltpu.VMEM((8, S), F32),
        pltpu.VMEM((2, D // 4, FH), U32),
        pltpu.VMEM((7, D // 2, KO), BF16),
        pltpu.VMEM((2, 7, KO, T), BF16),
        pltpu.VMEM((2, 2, FH - 2 * KO, T), BF16),
        pltpu.VMEM((2, 2, D, T), F32),
        pltpu.VMEM((S, D), A_q.dtype),
        pltpu.SMEM((1,), jnp.int32),
        pltpu.SemaphoreType.DMA((16 + 3 * NA + 4 * NB,)),
    ]
    out = pl.pallas_call(
        _kernel,
        out_shape=jax.ShapeDtypeStruct((S, D), A_q.dtype),
        in_specs=[pl.BlockSpec(memory_space=pl.ANY)] * len(operands),
        out_specs=pl.BlockSpec(memory_space=pl.ANY),
        scratch_shapes=scratch,
        compiler_params=pltpu.CompilerParams(vmem_limit_bytes=124 * 2**20),
    )(*operands)
    return out.reshape(B, S, D)
```

```python
import functools

import numpy as np

import jax
import jax.numpy as jnp
from jax import lax
import jax.experimental.pallas as pl
import jax.experimental.pallas.tpu as pltpu

LANES = 128
R = 4
M = 128
C = R * M
HIST = 16
T = 128
EPS = 1e-5
GELU_C1 = float(np.sqrt(2.0 / np.pi))
GELU_C3 = float(np.sqrt(2.0 / np.pi) * 0.044715)

PR = 32
NR = 288
NO = 16
TW = 2
SYNC = (1, 2, 4, 6)
XAT = (0, 0, 2, 2)
ORDER = (1, 4, 2, 3, 0, 6, 5)

F32 = jnp.float32
BF16 = jnp.bfloat16
U32 = jnp.uint32
NT = (((1,), (1,)), ((), ()))


def _dft_matrix(r):
    def cis(steps):
        angle = (((steps + 2 * C) & (4 * C - 1)) - 2 * C).astype(F32) * (np.pi / (2 * C))
        return jnp.cos(angle), -jnp.sin(angle)

    n = lax.broadcasted_iota(jnp.int32, (8, M), 1) * R + r
    re, im = cis(n * (4 * lax.broadcasted_iota(jnp.int32, (8, M), 0) + 1))
    wr, wi = cis(n * 32)
    rows = []
    for _ in range(M // 8):
        rows += [re, im]
        re, im = re * wr - im * wi, re * wi + im * wr
    return jnp.concatenate(rows, axis=0)


def _pack(x):
    return pltpu.bitcast(x.astype(BF16), U32)


def _unpack(w):
    return pltpu.bitcast(w, BF16)


def _split_rows(w):
    return [lax.bitcast_convert_type(x, F32) for x in (w << 16, w & np.uint32(0xFFFF0000))]


def _dot(a, b):
    return jnp.dot(a, b, preferred_element_type=F32)


def _dot_nt(a, b):
    return lax.dot_general(a, b, NT, preferred_element_type=F32)


def _gelu2(x):
    t = jnp.tanh(x * (x * x * GELU_C3 + GELU_C1))
    return x * t + x


def _ln_rows(x):
    n = x.shape[-1]
    d = x - jnp.sum(x, axis=-1, keepdims=True) * (1.0 / n)
    var = jnp.sum(d * d, axis=-1, keepdims=True) * (1.0 / n)
    return d * lax.rsqrt(var + EPS)


def _strassen_left(a11, a12, a21, a22):
    return (a11 + a22, a21 + a22, a11, a22, a11 + a12, a21 - a11, a12 - a22)


def _strassen_right(b11, b12, b21, b22):
    f11, f12, f21, f22 = (b.astype(F32) for b in (b11, b12, b21, b22))
    return [b.astype(BF16) for b in (f11 + f22, b11, f12 - f22, f21 - f11, b22, f11 + f12, f21 + f22)]


def _strassen(product, rest=None):
    def block(row, col, value):
        return (row, col), value if rest is None else value + rest(row, col)

    m2, m4 = product(1), product(3)
    yield block(1, 0, m2 + m4)
    m5, m3 = product(4), product(2)
    yield block(0, 1, m3 + m5)
    m1, m7 = product(0), product(6)
    yield block(0, 0, (m4 - m5) + m1 + m7)
    yield block(1, 1, (m3 - m2) + m1 + product(5))


def _butterfly(x, inverse):
    (r0, i0), (r1, i1), (r2, i2), (r3, i3) = x
    ar, ai, br, bi = r0 + r2, i0 + i2, r0 - r2, i0 - i2
    cr, ci, dr, di = r1 + r3, i1 + i3, r1 - r3, i1 - i3
    lo, hi = (br + di, bi - dr), (br - di, bi + dr)
    if inverse:
        lo, hi = hi, lo
    return [(ar + cr, ai + ci), lo, (ar - cr, ai - ci), hi]


def _forward(f_v, phases):
    es = []
    for r in range(R):
        e = _dot(_unpack(f_v[r]), phases[r].astype(BF16)).reshape(M // 8, 2, 8, LANES)
        es.append((e[:, 0], e[:, 1]))
    return _butterfly(es, inverse=False)


def _kernel(q_h, k_h, v_h, sk_h, g_h, sd_h, win_h, wsp_h, bsp_h, wout_h, c_h, wmod_h,
            out_h,
            q_v, k_v, v_v, sk_v, g_v, sd_v, win_v, wsp_v, bsp_v, wout_v, c_v, wmod_v, f_v,
            fi_v, gs_v, us_v, gt_v, kf_v, vf_v, tap_v, y_v, x1_v, mod_v, h_v, w_v, wis_v, a2_v,
            mean_v, zs_v, acc_v, brow_v, woutt_v, wos_v, p_v, pr_v, o_v, out_v, flag_v, sems):
    S, D = q_v.shape
    FH = wout_v.shape[0]
    KS = sk_v.shape[0]
    NA, NJ, NB = S // C, D // LANES, S // (2 * T)
    HF, HD = FH // 2, D // 2
    KI, KO = wis_v.shape[-1], wos_v.shape[-1]

    n_sem = [0]

    def fetch(src, dst):
        cp = pltpu.make_async_copy(src, dst, sems.at[n_sem[0]])
        n_sem[0] += 1
        cp.start()
        return cp

    def fetch_rows(src, dst, i, n):
        return fetch(src.at[pl.ds(i * n, n)], dst.at[pl.ds(i * n, n)])

    def fetch_cols(src, dst, i, n):
        return fetch(src.at[:, pl.ds(i * n, n)], dst.at[:, pl.ds(i * n, n)])

    def wait(copies):
        for cp in copies:
            cp.wait()

    def fetch_for_steps(first):
        later = [n for n in SYNC if n > first]
        copies = []
        for i in range(first, (later + [NB + 1])[0]):
            if i + 1 < NB:
                copies.append(fetch_rows(q_h, q_v, i + 1, 2 * T))
            copies.append(fetch(wsp_h.at[:, pl.ds((i - 1) * 2 * T, 2 * T)], wsp_v.at[i - 1]))
        if not later:
            copies += [fetch_cols(wmod_h, wmod_v, 5, D), fetch_rows(win_h, win_v, 0, FH),
                       fetch(bsp_h, bsp_v), fetch(wout_h, wout_v)]
        return copies

    cp_g = [[fetch_cols(g_h, g_v, 0, C), fetch(sd_h, sd_v), fetch(sk_h, sk_v),
             fetch(c_h, c_v)]]
    cp_g += [[fetch_cols(g_h, g_v, a, C)] for a in range(1, NA)]
    cp_kv = [[fetch_rows(k_h, k_v, a, C), fetch_rows(v_h, v_v, a, C)] for a in range(NA)]
    cp_mod = [fetch_rows(q_h, q_v, 0, 2 * T), fetch_cols(wmod_h, wmod_v, 0, 5 * D)]
    cp_proj = [fetch_rows(win_h, win_v, 1, FH), fetch_rows(q_h, q_v, 1, 2 * T)]
    cp_step = {SYNC[0]: fetch_for_steps(SYNC[0])}

    flag_v[0] = 0

    def split_code():
        @pl.loop(0, 2)
        def _(n):
            acc_v[n, 7 * HF:] = jnp.zeros((8, T), F32)

    last = []

    def paced(x, tiles=1, token=last):
        if not token:
            return x
        dep = token.pop()
        n = min(dep.shape[0], x.shape[0])
        dep = jnp.concatenate([dep[:n]] * (x.shape[0] // n), axis=0)
        cols = [x[:, c:c + LANES] for c in range(0, x.shape[1], LANES)]
        return jnp.concatenate(
            [jnp.where(flag_v[0] > 0, dep, col) for col in cols[:tiles]] + cols[tiles:], axis=1)

    def delayed(x):
        return pltpu.roll(x, 1, 1)

    def run(pieces, chained=True):
        for piece in pieces:
            if not chained:
                last.clear()
            piece()

    def transpose(a, j):
        gt_v[j, :C // 2, :] = _pack(g_v[j * LANES:(j + 1) * LANES, a * C:(a + 1) * C].T)

    def filter_spectrum(a, j):
        spec = _forward(f_v, [ph for r in range(R // 2)
                              for ph in _split_rows(gt_v[j, pl.ds(r, M, stride=R // 2), :])])
        for q in range(R):
            re, im = spec[q]
            if a == 0:
                re = re + tap_v[KS, :, j * LANES:(j + 1) * LANES]
            else:
                pr, pi = gs_v[j, 0, 2 * q], gs_v[j, 0, 2 * q + 1]
                for b in range(1, a):
                    pr, pi = gs_v[j, b, 2 * q] + pi, gs_v[j, b, 2 * q + 1] - pr
                re, im = re - pi, im + pr
            gs_v[j, a, 2 * q], gs_v[j, a, 2 * q + 1] = re, im

    def widen(a, j):
        lanes = slice(j * LANES, (j + 1) * LANES)
        if a == 0:
            kf_v[j, 0:HIST, :] = jnp.zeros((HIST, LANES), F32)
            kf_v[j, HIST:HIST + C, :] = k_v[0:C, lanes].astype(F32)
        else:
            kf_v[j, :HIST + C, :] = k_v[a * C - HIST:(a + 1) * C, lanes].astype(F32)
        vf_v[j, :C, :] = v_v[a * C:(a + 1) * C, lanes].astype(F32)

    def analyse(a, j):
        lanes = slice(j * LANES, (j + 1) * LANES)
        kp = {s: kf_v[j, pl.ds(HIST + s, M, stride=R), :] for s in range(1 - KS, R)}
        vp = [vf_v[j, pl.ds(r, M, stride=R), :] for r in range(R)]
        taps = [jnp.concatenate([tap_v[t, :, lanes]] * (M // 8), axis=0) for t in range(KS)]
        phases = []
        for r in range(R):
            acc = kp[r] * taps[0]
            for t in range(1, KS):
                acc = acc + kp[r - t] * taps[t]
            phases.append(acc * vp[r])
        spec = _forward(f_v, phases)
        for q in range(R):
            us_v[j, a, 2 * q], us_v[j, a, 2 * q + 1] = spec[q]

    def synthesise(a, j):
        ys = []
        for q in range(R):
            yr = yi = None
            for b in range(a + 1):
                ur, ui = us_v[j, a - b, 2 * q], us_v[j, a - b, 2 * q + 1]
                gr, gi = gs_v[j, b, 2 * q], gs_v[j, b, 2 * q + 1]
                tr, ti = gr * ur - gi * ui, gr * ui + gi * ur
                yr, yi = (tr, ti) if b == 0 else (yr + tr, yi + ti)
            ys.append((yr, yi))
        for r, pair in enumerate(_butterfly(ys, inverse=True)):
            spec = jnp.stack(pair, axis=1).reshape(2 * M, LANES).astype(BF16)
            y_v[j, pl.ds(a * C + r, M, stride=R), :] = _dot(_unpack(fi_v[r]), spec)

    def modulation(n):
        cc = c_v[...].astype(F32)
        sc = jnp.broadcast_to(cc * jax.nn.sigmoid(cc), (16, D)).astype(BF16)
        return _dot(sc, wmod_v[:, n * D:(n + 1) * D])[0:8]

    def scale(x, n):
        return (x.reshape(x.shape[0] // 8, 8, D) * mod_v[n]).reshape(x.shape)

    def shift(x, n):
        return (x.reshape(x.shape[0] // 8, 8, D) + mod_v[n]).reshape(x.shape)

    def prepare(i):
        def piece(r0):
            rs = slice(r0, r0 + PR)
            x = paced(q_v[rs, :].astype(F32))
            y = jnp.concatenate([y_v[j, rs, :] for j in range(NJ)], axis=1)
            x1 = x + shift(scale(_ln_rows(x), 0), 1) * y
            x1_v[rs, :] = x1
            h = shift(scale(_ln_rows(x1), 2), 3)
            h_v[r0 // 2:(r0 + PR) // 2, :] = _pack(h)
            last.append(h[:, -LANES:])

        return [functools.partial(piece, r0) for r0 in range(2 * i * T, 2 * (i + 1) * T, PR)]

    def split_left(dst, top, bottom, width, pace):
        last.clear()
        for r0 in range(0, top.shape[0], 8):
            blk = [src[r0:r0 + 8, k:k + width] for src in (top, bottom) for k in (0, width)]
            if pace:
                blk = [paced(w, width // LANES, list(last)) for w in blk]
            left = _strassen_left(*(_unpack(w).astype(F32) for w in blk))
            for n, val in enumerate(left):
                dst[n, 2 * r0:2 * r0 + 16, :] = val.astype(BF16)
            last[:] = [delayed(lax.bitcast_convert_type(left[0][:8, :LANES], U32))]

    def load_w_in(fh):
        for qh in range(2):
            for dst, src, n in ((0, qh * KO, KO), (KO, 2 * KO + qh * (HF - KO), HF - KO)):
                w_v[fh, qh, dst // 2:(dst + n) // 2] = _pack(win_v[fh * FH + src:fh * FH + src + n, :])
        split_left(wis_v.at[fh], w_v.at[fh, 0], w_v.at[fh, 1], KI, False)

    def project(i, fh):
        hs = [_unpack(h_v[(2 * i + hh) * T // 2:(2 * i + hh + 1) * T // 2, :]) for hh in range(2)]
        right = _strassen_right(*(h[:, k:k + KI] for k in (0, KI) for h in hs))
        return _strassen(lambda n: _dot_nt(wis_v[fh, n], right[n]),
                         lambda qh, hh: _dot_nt(_unpack(w_v[fh, qh, :, 2 * KI:]), hs[hh][:, 2 * KI:]))

    def activate(i):
        tot = {}
        for (qh, hh), z in project(i, 1):
            a2 = _gelu2(z)
            a2_v[i % 2, hh, qh * HF:(qh + 1) * HF, :] = a2
            part = jnp.sum(a2.reshape(HF // 8, 8, T), axis=0)
            tot[hh] = tot[hh] + part if hh in tot else part
            yield
        for hh in range(2):
            mean = jnp.sum(tot[hh], axis=0, keepdims=True) * (1.0 / FH)
            mean_v[i % 2, :, hh * T:(hh + 1) * T] = jnp.broadcast_to(mean, (8, T))

    def normalize(i):
        state = {}

        def centred(r0, n, mean):
            a2 = jnp.concatenate([a2_v[i % 2, hh, r0:r0 + n, :] for hh in range(2)], axis=1)
            return a2.reshape(n // 8, 8, 2 * T) - mean

        def var_piece(r0):
            d = centred(r0, NR, paced(mean_v[i % 2], 2))
            part = jnp.sum(d * d, axis=0)
            state["ss"] = part if r0 == 0 else state["ss"] + part
            last.append(delayed(state["ss"][:, :LANES]))
            if r0 + NR == FH:
                var = jnp.sum(state["ss"], axis=0, keepdims=True) * (1.0 / FH)
                state["rstd"] = jnp.broadcast_to(lax.rsqrt(var + 4.0 * EPS), (8, 2 * T))

        def out_piece(r0):
            mean = paced(mean_v[i % 2], 2)
            za, zb = (centred(r, NO, mean) * state["rstd"] for r in (r0, HF + r0))
            left = _strassen_left(za[..., :T], za[..., T:], zb[..., :T], zb[..., T:])
            for n, val in enumerate(left):
                zs_v[i % 2, n, r0:r0 + NO, :] = val.reshape(NO, T).astype(BF16)
            last.append(delayed(left[0][-1]))

        return ([functools.partial(var_piece, r0) for r0 in range(0, FH, NR)]
                + [functools.partial(out_piece, r0) for r0 in range(0, HF, NO)])

    def mix(i, extra=iter(())):
        def block(k0, th, sh):
            return jnp.concatenate(
                [wsp_v[i, (2 * k + th) * T:(2 * k + th + 1) * T, sh * T:(sh + 1) * T]
                 for k in range(k0, k0 + TW)], axis=0)

        for k0 in range(0, NB, TW):
            for pos, n in enumerate(ORDER):
                for _ in range(XAT.count(pos) if k0 == 0 else 0):
                    next(extra, None)
                right = _strassen_right(*(block(k0, th, sh) for sh in range(2) for th in range(2)))[n]
                m = _dot_nt(zs_v[i % 2, n], right)
                for k in range(TW):
                    at = (k0 + k, slice(n * HF, (n + 1) * HF))
                    part = m[:, k * T:(k + 1) * T]
                    acc_v[at] = acc_v[at] + part if i else part
        for _ in extra:
            pass

    def step_b(i):
        if i in SYNC:
            if i == SYNC[1]:
                split_code()
            for n in [n for n in SYNC if n > i][:1]:
                cp_step[n] = fetch_for_steps(n)
            wait(cp_step[i])
        extra = activate(i)
        if i == 1:
            run(normalize(0), chained=False)
            last.clear()
            for _ in extra:
                pass
        mix(i - 1, extra)
        run((prepare(i + 1) if i + 1 < NB else []) + normalize(i))

    def gate(i, zs):
        gates = dict(_strassen(lambda n: acc_v[i, n * HF:(n + 1) * HF]))
        ps = {}
        for (qh, hh), z in zs:
            bias = brow_v[:, (2 * i + hh) * T:(2 * i + hh + 1) * T]
            ps[qh, hh] = _gelu2(z) * (gates[qh, hh].reshape(HF // 8, 8, T) + bias).reshape(HF, T)
        for n, val in enumerate(_strassen_right(*(ps[qh, hh][:KO] for qh in range(2) for hh in range(2)))):
            p_v[i % 2, n] = val
        for hh in range(2):
            pr_v[i % 2, hh] = jnp.concatenate([ps[0, hh][KO:], ps[1, hh][KO:]], axis=0).astype(BF16)

    def project_out(i):
        for (dh, hh), o in _strassen(
                lambda n: _dot(wos_v[n], p_v[i % 2, n]),
                lambda dh, hh: _dot(_unpack(woutt_v[dh, :, 2 * KO:]), pr_v[i % 2, hh])):
            o_v[i % 2, hh, dh * HD:(dh + 1) * HD] = o

    cp_out = []

    def finish(i):
        for hh in range(2):
            rs = slice((2 * i + hh) * T, (2 * i + hh + 1) * T)
            out_v[rs, :] = (x1_v[rs, :] + scale(o_v[i % 2, hh].T, 4)).astype(out_v.dtype)
            cp_out.append(fetch_rows(out_v, out_h, 2 * i + hh, T))

    split_code()
    for r in range(R):
        f = _dft_matrix(r).astype(BF16)
        f_v[r], fi_v[r] = _pack(f), _pack(f.T)

    wait(cp_g[0])
    tap_v[KS] = jnp.broadcast_to(sd_v[...].astype(F32).reshape(1, D), (8, D))
    sk = sk_v[...].astype(F32)
    for t in range(KS):
        tap_v[t] = jnp.broadcast_to(sk[t:t + 1] * (1.0 / C), (8, D))

    tiles = [(a, j) for a in range(NA) for j in range(NJ)]
    nt = len(tiles)
    needed = {a * NJ: cp_g[a] for a in range(1, NA)}
    needed.update({nt + a * NJ: cp_kv[a] for a in range(NA)})
    needed[2 * nt + 1] = cp_mod
    stages = ((transpose, 0), (filter_spectrum, 1), (widen, nt), (analyse, nt + 1), (synthesise, nt + 2))
    for n in range(2 * nt + 2):
        if n == 2 * nt + 1:
            sa, ca, ga, sb, cb = (modulation(m) for m in range(5))
            mod_v[0], mod_v[1], mod_v[2], mod_v[3] = ga * (1.0 + ca), ga * sa, 1.0 + cb, sb
            run(prepare(0), chained=False)
        for fn, lag in stages:
            if fn is synthesise and n + 1 in needed:
                wait(needed[n + 1])
            if 0 <= n - lag < nt:
                fn(*tiles[n - lag])

    wait(cp_proj)
    load_w_in(1)
    for _ in activate(0):
        pass
    run(prepare(1), chained=False)
    for i in range(1, NB):
        step_b(i)

    load_w_in(0)
    brow_v[...] = jnp.broadcast_to(bsp_v[...].astype(F32).reshape(1, S), (8, S))
    mod_v[4] = 0.5 * modulation(5)
    z_first = list(project(0, 0))
    mix(NB - 1)
    gate(0, z_first)
    woutt = _pack(wout_v[...].T)
    for dh in range(2):
        woutt_v[dh] = woutt[dh * HD // 2:(dh + 1) * HD // 2]
    split_left(wos_v, woutt_v.at[0], woutt_v.at[1], KO, True)

    for i in range(1, NB + 2):
        if i >= 2:
            finish(i - 2)
        if i < NB:
            gate(i, project(i, 0))
        if i <= NB:
            project_out(i - 1)
    wait(cp_out)


@jax.jit
def pallas_adaLN_cond__ssm_conv_h3__mixer_gmlp__prompt_kernel(
    A_q: jax.Array,
    A_k: jax.Array,
    A_v: jax.Array,
    A_shift_k: jax.Array,
    A_ssm_k: jax.Array,
    A_ssm_D: jax.Array,
    B_x: jax.Array,
    B_w_in: jax.Array,
    B_w_sp: jax.Array,
    B_b_sp: jax.Array,
    B_w_out: jax.Array,
    c: jax.Array,
    w_mod: jax.Array,
):
    del B_x
    B, S, D = A_q.shape
    FH = B_w_out.shape[0]
    KS = A_shift_k.shape[1]
    assert B == 1 and S % C == 0 and D % LANES == 0 and B_w_in.shape[1] == 2 * FH
    NA, NJ, NB = S // C, D // LANES, S // (2 * T)
    KI, KO = (D // (2 * LANES)) * LANES, (FH // (2 * LANES)) * LANES
    operands = (
        A_q.reshape(S, D), A_k.reshape(S, D), A_v.reshape(S, D), A_shift_k.T, A_ssm_k, A_ssm_D,
        B_w_in.T, B_w_sp, B_b_sp, B_w_out, c, w_mod,
    )
    spectra = (NJ, NA, 2 * R, M // 8, 8, LANES)
    scratch = [pltpu.VMEM((NB, S, 2 * T) if o is B_w_sp else o.shape, o.dtype) for o in operands] + [
        pltpu.VMEM((R, M, M), U32),
        pltpu.VMEM((R, M // 2, 2 * M), U32),
        pltpu.VMEM(spectra, F32),
        pltpu.VMEM(spectra, F32),
        pltpu.VMEM((NJ, C // 2 + 8, LANES), U32),
        pltpu.VMEM((NJ, HIST + C + 8, LANES), F32),
        pltpu.VMEM((NJ, C + 8, LANES), F32),
        pltpu.VMEM((KS + 1, 8, D), F32),
        pltpu.VMEM((NJ, S + 8, LANES), F32),
        pltpu.VMEM((S, D), F32),
        pltpu.VMEM((5, 8, D), F32),
        pltpu.VMEM((S // 2, D), U32),
        pltpu.VMEM((2, 2, FH // 4, D), U32),
        pltpu.VMEM((2, 7, FH // 2, KI), BF16),
        pltpu.VMEM((2, 2, FH, T), F32),
        pltpu.VMEM((2, 8, 2 * T), F32),
        pltpu.VMEM((2, 7, FH // 2, T), BF16),
        pltpu.VMEM((NB, 7 * FH // 2 + 8, T), F32),
        pltpu.VMEM((8, S), F32),
        pltpu.VMEM((2, D // 4, FH), U32),
        pltpu.VMEM((7, D // 2, KO), BF16),
        pltpu.VMEM((2, 7, KO, T), BF16),
        pltpu.VMEM((2, 2, FH - 2 * KO, T), BF16),
        pltpu.VMEM((2, 2, D, T), F32),
        pltpu.VMEM((S, D), A_q.dtype),
        pltpu.SMEM((1,), jnp.int32),
        pltpu.SemaphoreType.DMA((16 + 3 * NA + 4 * NB,)),
    ]
    out = pl.pallas_call(
        _kernel,
        out_shape=jax.ShapeDtypeStruct((S, D), A_q.dtype),
        in_specs=[pl.BlockSpec(memory_space=pl.ANY)] * len(operands),
        out_specs=pl.BlockSpec(memory_space=pl.ANY),
        scratch_shapes=scratch,
        compiler_params=pltpu.CompilerParams(vmem_limit_bytes=124 * 2**20),
    )(*operands)
    return out.reshape(B, S, D)
```
